```python
import os as _os
_os.environ.setdefault("JAX_PLATFORMS", "cpu")
import jax
import jax.numpy as jnp

def _softmax(x, axis=-1):
    return jax.nn.softmax(x, axis=axis)
def _gelu(x):
    return jax.nn.gelu(x, approximate=True)
def _silu(x):
    return jax.nn.silu(x)
def _sigmoid(x):
    return jax.nn.sigmoid(x)
def _layernorm(x, axis=-1, eps=1e-5):
    m = jnp.mean(x, axis=axis, keepdims=True)
    v = jnp.var(x, axis=axis, keepdims=True)
    return (x - m) / jnp.sqrt(v + eps)
def _scatter_add(tgt, idx, src, axis=0):
    return tgt.at[idx].add(src)
def _segment_sum(src, seg, n):
    return jax.ops.segment_sum(src, seg, n)
class _Rng:
    def __init__(self, key):
        self._k = key
    def _next(self):
        self._k, sub = jax.random.split(self._k)
        return sub
    def normal(self, shape):
        return jax.random.normal(self._next(), shape, dtype=jnp.bfloat16)
    def randint(self, lo, hi, shape):
        return jax.random.randint(self._next(), shape, lo, hi, dtype=jnp.int32)
    def uniform(self, shape, lo=0.0, hi=1.0):
        return jax.random.uniform(self._next(), shape, jnp.bfloat16, lo, hi)
    def permutation(self, n):
        return jax.random.permutation(self._next(), n)


kernel_name = 'interleave_layers__spectral_gfnet__mixer_token_mlp__prompt'

def setup_inputs():
    _rng = _Rng(jax.random.key(int.from_bytes(__import__("os").urandom(4), "little")))
    _w = (lambda a: (lambda t: t.astype(jnp.bfloat16) if jnp.issubdtype(t.dtype, jnp.floating) else t)(jnp.asarray(a)))
    def _A_setup():
        B, S, D = 1, 2048, 640
        Df = D // 2 + 1
        return {
            "x": _w((lambda *s: _rng.normal(s) * 0.05)(B, S, D)),
            "w_r": _w((lambda *s: _rng.normal(s) * 0.2)(S, Df) * 0.02),
            "w_i": _w((lambda *s: _rng.normal(s) * 0.2)(S, Df) * 0.02),
        }
    _A_in = _A_setup()

    def _B_setup():
        B, S, D, F = 1, 2048, 640, 1728
        return {
            "x": _w((lambda *s: _rng.normal(s) * 0.05)(B, S, D)),
            "w1": _w((lambda *s: _rng.normal(s) * 0.1)(S, F) * (S ** -0.5)),
            "b1": _w((lambda *s: _rng.normal(s) * 0.1)(F) * 0.02),
            "w2": _w((lambda *s: _rng.normal(s) * 0.1)(F, S) * (F ** -0.5)),
            "b2": _w((lambda *s: _rng.normal(s) * 0.1)(S) * 0.02),
        }
    _B_in = _B_setup()

    return {
        "A_x": _A_in["x"],
        "A_w_r": _A_in["w_r"],
        "A_w_i": _A_in["w_i"],
        "B_x": _B_in["x"],
        "B_w1": _B_in["w1"],
        "B_b1": _B_in["b1"],
        "B_w2": _B_in["w2"],
        "B_b2": _B_in["b2"],
    }

def reference(A_x, A_w_r, A_w_i, B_x, B_w1, B_b1, B_w2, B_b2):
    def _A_ref(x, w_r, w_i):
        B, S, D = x.shape
        X = (lambda x, axes=(-2,-1): jnp.fft.rfft2(x.astype(jnp.float32), axes=axes))(x, axes=(-2, -1))
        W = w_r + 1j * w_i
        X = X * W
        y = (lambda x, s, axes=(-2,-1): jnp.fft.irfft2(x, s=s, axes=axes).astype(jnp.bfloat16))(X, (S, D), axes=(-2, -1))
        return y

    def _B_ref(x, w1, b1, w2, b2):
        B, S, D = x.shape
        h = _layernorm(x, axis=-1)
        u = jnp.einsum("bsd,sf->bdf", h, w1) + b1
        u = _gelu(u)
        y = jnp.einsum("bdf,fs->bds", u, w2) + b2
        return (lambda x, *d: x.transpose(*d))(y, 0, 2, 1)

    x = A_x
    x = x + _A_ref(_layernorm(x, axis=-1), A_w_r, A_w_i)
    x = x + _B_ref(_layernorm(x, axis=-1), B_w1, B_b1, B_w2, B_b2)
    x = x + _A_ref(_layernorm(x, axis=-1), A_w_r, A_w_i)
    x = x + _B_ref(_layernorm(x, axis=-1), B_w1, B_b1, B_w2, B_b2)
    return x
```

```python
import numpy as np
import jax
import jax.numpy as jnp
from jax import lax
import jax.experimental.pallas as pl
import jax.experimental.pallas.tpu as pltpu

S, D, F = 2048, 640, 1728
DF = D // 2 + 1
R = 336
NG = 41
CH = 256
NCH = S // CH
EPS = 1e-5
F32 = jnp.float32
BF16 = jnp.bfloat16
U32 = jnp.uint32

_S1 = float(np.sin(2 * np.pi / 5))
_S2 = float(np.sin(4 * np.pi / 5))
_C5 = float((np.cos(2 * np.pi / 5) - np.cos(4 * np.pi / 5)) / 2)
_CLASS_OFF = (0, 1, 4, 2, 3)
_RH = float(np.sqrt(0.5))


def _pack_rows(a):
    u = np.asarray(a, np.float32).view(np.uint32)
    u = (u + 0x7FFF + ((u >> 16) & 1)) >> 16
    return (u[..., 0::2, :] | (u[..., 1::2, :] << 16)).astype(np.uint32)


def _tables():
    q = np.arange(128)
    t = np.arange(32)
    j5 = np.concatenate([10 * t, 5 + 10 * t])
    sig = np.concatenate([np.ones(64), -np.ones(64)])

    def cs(k):
        th = 2 * np.pi * np.outer(k, q) / D
        return np.cos(th), np.sin(th)

    c0, s0 = cs(j5)
    cn, _ = cs(np.array([D // 2]))
    sc = 2.0 / (D * S)
    nyq = np.zeros((16, 128))
    nyq[0] = cn[0]
    i0 = np.concatenate([c0, -s0]).T * sc
    i0[:, 0] *= 0.5
    i0[:, 64] = cn[0] * 0.5 * sc
    fwd, inv = [nyq, c0, -s0], [i0]
    for ca, cb in ((1, 4), (2, 3)):
        cA, sA = cs(ca + j5)
        cB, sB = cs(cb + j5)
        P = np.concatenate([cA, cB])
        Q = np.concatenate([sA, -sB])
        fwd += [P, (-Q - P) * sig[:, None], P - Q]
        inv += [P.T * sc, (Q.T - P.T) * sc, (P.T + Q.T) * sig[None, :] * sc]
    b = np.arange(128)
    th = 2 * np.pi * np.outer(b, b) / 128
    tt = 2 * np.pi * np.outer(np.arange(16), b) / S
    ft = np.concatenate([np.cos(th), -np.sin(th), np.cos(tt), -np.sin(tt)])
    return (_pack_rows(np.concatenate(fwd)), _pack_rows(np.concatenate(inv)), ft.astype(np.float32))


def _bfly4(a, b, c, d):
    s0r, s0i = a[0] + c[0], a[1] + c[1]
    d0r, d0i = a[0] - c[0], a[1] - c[1]
    s1r, s1i = b[0] + d[0], b[1] + d[1]
    d1r, d1i = b[0] - d[0], b[1] - d[1]
    return ((s0r + s1r, s0i + s1i), (d0r + d1i, d0i - d1r),
            (s0r - s1r, s0i - s1i), (d0r - d1i, d0i + d1r))


def _tw16(z, e):
    r, i = z
    if e == 0:
        return z
    if e == 4:
        return (i, -r)
    if e == 2:
        return ((r + i) * _RH, (i - r) * _RH)
    if e == 6:
        return ((i - r) * _RH, (r + i) * (-_RH))
    c, s = float(np.cos(2 * np.pi * e / 16)), float(np.sin(2 * np.pi * e / 16))
    return (r * c + i * s, i * c - r * s)


def _dft16(x):
    t = []
    for a0 in range(4):
        o = _bfly4(x[a0], x[4 + a0], x[8 + a0], x[12 + a0])
        t.append([_tw16(o[r0], a0 * r0) for r0 in range(4)])
    out = [None] * 16
    for r0 in range(4):
        o = _bfly4(t[0][r0], t[1][r0], t[2][r0], t[3][r0])
        for r1 in range(4):
            out[r0 + 4 * r1] = o[r1]
    return out


def _dot(a, b):
    return jnp.dot(a, b, preferred_element_type=F32)


def _dot_t(a, b):
    return lax.dot_general(a, b, (((1,), (1,)), ((), ())), preferred_element_type=F32)


def _gelu(u):
    return 0.5 * u * (1.0 + jnp.tanh(0.7978845608028654 * (u + 0.044715 * (u * u * u))))


def _cols(off, width):
    if isinstance(off, int):
        return pl.ds(off, width)
    return pl.ds(pl.multiple_of(off, 128), width)


def _bf(u):
    return pltpu.bitcast(u, BF16)


def _pk(v):
    return pltpu.bitcast(v.astype(BF16), U32)


def _kernel(x_hbm, wr_hbm, wi_hbm, w1_hbm, b1_hbm, w2_hbm, b2_hbm, fwd_hbm, inv_hbm, ft_hbm,
            out_hbm,
            xin, wraw, wnyq, wn, w1, w2, b1_ref, b2_ref, fwd_ref, inv_ref, ft_ref,
            b1f, b2f, st, xa, xb, yr, yi, tb, tp, yb, hb, gb, wt, g3, ost,
            sem_x, sem_w, sem_m, sem_o, sem_c):
    def x_copy(j):
        return pltpu.make_async_copy(x_hbm.at[pl.ds(j * CH, CH), :], xin.at[pl.ds(j * CH, CH), :], sem_x.at[j])

    def o_copy(j):
        return pltpu.make_async_copy(ost.at[pl.ds(j * CH, CH), :], out_hbm.at[pl.ds(j * CH, CH), :], sem_o.at[j])

    w_copies = []
    for ri, src in enumerate((wr_hbm, wi_hbm)):
        w_copies.append(pltpu.make_async_copy(src.at[pl.ds(0, 320), :], wraw.at[pl.ds(320 * ri, 320), :], sem_w.at[2 * ri]))
        w_copies.append(pltpu.make_async_copy(src.at[pl.ds(320, 1), :], wnyq.at[ri], sem_w.at[2 * ri + 1]))
    w1_copy = pltpu.make_async_copy(w1_hbm, w1, sem_m.at[0])
    w2_copy = pltpu.make_async_copy(w2_hbm, w2, sem_m.at[1])
    c_pairs = ((fwd_hbm, fwd_ref), (ft_hbm, ft_ref), (inv_hbm, inv_ref), (b1_hbm, b1_ref), (b2_hbm, b2_ref))
    c_copies = [pltpu.make_async_copy(a, b, sem_c.at[i]) for i, (a, b) in enumerate(c_pairs)]

    c_copies[0].start()

    def start_x(j, c):
        x_copy(j).start()
        return c
    lax.fori_loop(0, NCH, start_x, 0)
    c_copies[1].start()

    yi[320:336, :] = jnp.zeros((16, S), F32)
    tb[:, 320:336, :] = jnp.zeros((16, 16, 384), BF16)

    def put_stats(gcols, xn):
        dlt = jnp.sum(xn, axis=0, keepdims=True) * (1.0 / D)
        msq = jnp.sum(xn * xn, axis=0, keepdims=True) * (1.0 / D)
        return dlt, jnp.maximum(msq - dlt * dlt, 0.0)

    def col_pre(buf, loff, goff):
        lc, gc = _cols(loff, 128), _cols(goff, 128)
        r = lax.rsqrt(st[2:3, gc] + EPS)
        rs1, rs2, rc, d5 = r * (-_S1), r * (-_S2), r * _C5, st[1:2, gc] * r * 5.0
        x0, x1, x2, x3, x4 = [buf[128 * p:128 * (p + 1), lc] for p in range(5)]
        t1, t2, t3, t4 = x1 + x4, x2 + x3, x1 - x4, x2 - x3
        u = (t1 + t2) * r
        x0 = x0 * r
        m = x0 - 0.25 * u
        n = (t1 - t2) * rc
        a1, a2 = m + n, m - n
        b1_ = t3 * rs1 + t4 * rs2
        b2_ = t3 * rs2 - t4 * rs1
        return [v.astype(BF16) for v in (x0 + u - d5, a1 + b1_, a1, b1_, a2 + b2_, a2, b2_)]

    def col_dft(goff, a):
        cols = _cols(goff, 128)
        o0 = _dot(_bf(fwd_ref[0:72, :]), a[0])
        yr[320:336, cols] = o0[0:16]
        yr[0:64, cols] = o0[16:80]
        yi[0:64, cols] = o0[80:144]
        for c in range(2):
            k1, k2, k3 = [_dot(_bf(fwd_ref[72 + 64 * (3 * c + i):72 + 64 * (3 * c + i + 1), :]), a[1 + 3 * c + i])
                          for i in range(3)]
            r0 = 64 + 128 * c
            yr[r0:r0 + 128, cols] = k1 - k3
            yi[r0:r0 + 64, cols] = k2[0:64] + k1[0:64]
            yi[r0 + 64:r0 + 128, cols] = k2[64:128] - k1[64:128]

    def col_fwd(buf, loff, goff):
        a0 = col_pre(buf, loff, goff)
        a1 = col_pre(buf, loff + 128, goff + 128)
        col_dft(goff, a0)
        col_dft(goff + 128, a1)

    def radix_fwd(g, c):
        rows = pl.ds(pl.multiple_of(g * 8, 8), 8)
        x = [(yr[rows, 128 * a:128 * (a + 1)], yi[rows, 128 * a:128 * (a + 1)]) for a in range(16)]
        o = _dft16(x)
        for m1 in range(16):
            tb[m1, rows, :] = jnp.concatenate([o[m1][0] + o[m1][1], o[m1][0], o[m1][1]], axis=1).astype(BF16)
        return c

    def gen_g(m1):
        tr = ft_ref[256 + m1:257 + m1, :]
        ti = ft_ref[272 + m1:273 + m1, :]
        fr = ft_ref[0:128, :]
        fi = ft_ref[128:256, :]
        gr = fr * tr - fi * ti
        gi = fr * ti + fi * tr
        g3[m1, 0] = _pk(gr)
        g3[m1, 1] = _pk(gi - gr)
        g3[m1, 2] = _pk(gr + gi)

    def unpack(v):
        return pltpu.bitcast(v << 16, F32), pltpu.bitcast(v & jnp.uint32(0xFFFF0000), F32)

    def load_wt(m1):
        nq = unpack(wt[m1, 320:336, :])
        res = []
        for ri in range(2):
            h = [unpack(wt[m1, pl.ds(160 * ri + w0, 32, stride=5), :]) for w0 in range(5)]
            parts = []
            for cl in _CLASS_OFF:
                parts += [h[cl // 2][cl % 2], h[(cl + 5) // 2][(cl + 5) % 2]]
            res.append(jnp.concatenate(parts + [nq[ri]], axis=0))
        return res

    def spec_fwd(m1):
        k1 = _dot_t(tb[m1, :, 0:128], _bf(g3[m1, 0]))
        k2 = _dot_t(tb[m1, :, 128:256], _bf(g3[m1, 1]))
        k3 = _dot_t(tb[m1, :, 256:384], _bf(g3[m1, 2]))
        return k1 - k3, k1 + k2

    def spec_mul(m1, xr, xi):
        wr_, wi_ = load_wt(m1)
        zr = xr * wr_ - xi * wi_
        zi = xr * wi_ + xi * wr_
        return (zr + zi).astype(BF16), zi.astype(BF16), zr.astype(BF16)

    def spec_inv(m1, z):
        q1 = _dot(z[0], _bf(g3[m1, 0]))
        q2 = _dot(z[1], _bf(g3[m1, 1]))
        q3 = _dot(z[2], _bf(g3[m1, 2]))
        tp[m1, :, 0:128] = q1 + q2
        tp[m1, :, 128:256] = q1 - q3

    def spectral():
        z = spec_mul(0, *spec_fwd(0))
        for m1 in range(16):
            zn = spec_mul(m1 + 1, *spec_fwd(m1 + 1)) if m1 + 1 < 16 else None
            spec_inv(m1, z)
            z = zn

    def spectral_first():
        def fwd_store(m1):
            gen_g(m1)
            xr, xi = spec_fwd(m1)
            tp[m1, :, 0:128] = xr
            tp[m1, :, 128:256] = xi

        wu = wraw.bitcast(U32)

        def prep1(j):
            cols = pl.ds(j * 128, 128)
            wn[0, cols, :] = wu[0:128, cols].T
            wn[1, cols, :] = wu[128:256, cols].T
            wn[2, cols, 0:80] = wu[256:336, cols].T

        def prep2(m1):
            wt[m1, 0:128, :] = wn[0, pl.ds(m1, 128, stride=16), :].T
            wt[m1, 128:256, :] = wn[1, pl.ds(m1, 128, stride=16), :].T
            wt[m1, 256:336, :] = wn[2, pl.ds(m1, 128, stride=16), :].T[0:80]

        c_copies[1].wait()
        with jax.named_scope("s1_fwdA"):
            for m1 in range(8):
                fwd_store(m1)
        with jax.named_scope("s1_wait"):
            for cp in w_copies:
                cp.wait()
        with jax.named_scope("s1_fwdB"):
            wraw[640:672, :] = jnp.concatenate(
                [wnyq[0].astype(F32), wnyq[1].astype(F32), jnp.zeros((30, S), F32)], axis=0).astype(BF16)
            for m1 in range(8, 16):
                fwd_store(m1)
                prep1(2 * (m1 - 8))
                prep1(2 * (m1 - 8) + 1)
        with jax.named_scope("s1_inv"):
            for m1 in range(16):
                prep2(m1)
                spec_inv(m1, spec_mul(m1, tp[m1, :, 0:128], tp[m1, :, 128:256]))

    def idft_group(rows):
        x = [(tp[m1, rows, 128:256], tp[m1, rows, 0:128]) for m1 in range(16)]
        o = _dft16(x)
        return [o[a][1] for a in range(16)], [o[a][0] for a in range(16)]

    def row_bf16(vals):
        return jnp.concatenate(vals, axis=1).astype(BF16)

    def radix_inv0(g, c):
        re, im = idft_group(pl.ds(pl.multiple_of(g * 8, 8), 8))
        yb[pl.ds(pl.multiple_of(g * 8, 8), 8), :] = row_bf16(re)
        yb[pl.ds(pl.multiple_of(64 + g * 8, 8), 8), :] = row_bf16(im)
        return c

    def radix_inv(g0, base, sign):
        def body(g, c):
            re, im = idft_group(pl.ds(pl.multiple_of(g * 8, 8), 8))
            sm = [(a + b if sign > 0 else a - b) for a, b in zip(re, im)]
            o = base + (g - g0) * 8
            yb[pl.ds(pl.multiple_of(o, 8), 8), :] = row_bf16(sm)
            yb[pl.ds(pl.multiple_of(o + 128, 8), 8), :] = row_bf16(re)
            yb[pl.ds(pl.multiple_of(o + 256, 8), 8), :] = row_bf16(im)
            return c
        return body

    def radix_inv_all():
        re0, im0 = idft_group(pl.ds(0, 8))
        ren, _ = idft_group(pl.ds(320, 8))
        first = lax.broadcasted_iota(jnp.int32, (8, 128), 0) == 0
        yb[0:8, :] = row_bf16(re0)
        yb[64:72, :] = row_bf16([jnp.where(first, a, b) for a, b in zip(ren, im0)])
        lax.fori_loop(1, 8, radix_inv0, 0)
        lax.fori_loop(8, 16, radix_inv(8, 128, 1), 0)
        lax.fori_loop(16, 24, radix_inv(8, 128, -1), 0)
        lax.fori_loop(24, 32, radix_inv(24, 512, 1), 0)
        lax.fori_loop(32, 40, radix_inv(24, 512, -1), 0)

    def inv_dots(goff):
        cols = _cols(goff, 128)
        v = [_dot(_bf(inv_ref[0:64, :]), yb[0:128, cols])]
        for c in range(2):
            j1, j2, j3 = [_dot(_bf(inv_ref[64 * (1 + 3 * c + i):64 * (2 + 3 * c + i), :]),
                               yb[128 * (1 + 3 * c + i):128 * (2 + 3 * c + i), cols]) for i in range(3)]
            v += [j1 - j3, j1 + j2]
        return v

    def inv_post(buf, loff, goff, v):
        lc, gc = _cols(loff, 128), _cols(goff, 128)
        dold = st[1:2, gc]
        st[0:1, gc] = st[0:1, gc] + dold
        v0, v1r, v1i, v2r, v2i = v
        v0 = v0 - dold
        t1 = v1r + v2r
        m = v0 - 0.25 * t1
        n = _C5 * (v1r - v2r)
        a, b = m + n, m - n
        cc = _S1 * v1i + _S2 * v2i
        dd = _S2 * v1i - _S1 * v2i
        ys = (v0 + t1, a - cc, b - dd, b + dd, a + cc)
        xn = buf[:, lc] + jnp.concatenate(ys, axis=0)
        buf[:, lc] = xn
        dlt, var = put_stats(gc, xn)
        r1 = lax.rsqrt(var + EPS)
        rr = r1 * lax.rsqrt(var * r1 * r1 + EPS)
        hb[:, gc] = _pk(buf[:, lc] * rr - dlt * rr)

    def col_inv_all():
        v = inv_dots(0)
        for blk in range(16):
            vn = inv_dots(128 * (blk + 1)) if blk + 1 < 16 else None
            j = blk // 2
            inv_post((xa, xb)[j % 2], (j // 2) * CH + 128 * (blk % 2), 128 * blk, v)
            v = vn

    def mlp_up():
        def one(cols):
            u = _dot_t(_bf(hb[...]), w1[cols, :]) + b1f[:, cols]
            gb[:, cols] = _pk(_gelu(u))

        def body(j, c):
            one(_cols(j * 512, 256))
            one(_cols(j * 512 + 256, 256))
            return c
        lax.fori_loop(0, 3, body, 0)
        one(pl.ds(1536, F - 1536))

    def down_y(gc):
        return _dot(_bf(gb[...]), w2[:, gc])

    def mlp_down_mid():
        def step(cur, loff, goff, prev, ploff, pgoff):
            lc, gc = _cols(loff, CH), _cols(goff, CH)
            xy = cur[:, lc] + down_y(gc)
            row0 = xy[0:1]
            xn = xy - row0
            cur[:, lc] = xn
            col_fwd(prev, ploff, pgoff)
            dlt, var = put_stats(gc, xn)
            st[0:1, gc] = st[0:1, gc] + row0 + b2f[:, gc]
            st[1:2, gc] = dlt
            st[2:3, gc] = var

        def body(i, c):
            ip = (i + 3) % 4
            step(xa, i * CH, 2 * i * CH, xb, ip * CH, (2 * ip + 1) * CH)
            step(xb, i * CH, (2 * i + 1) * CH, xa, i * CH, 2 * i * CH)
            return c
        lax.fori_loop(0, NCH // 2, body, 0)
        col_fwd(xb, 3 * CH, 7 * CH)

    def mlp_down_last():
        def step(cur, loff, goff):
            lc, gc = _cols(loff, CH), _cols(goff, CH)
            xn = cur[:, lc] + down_y(gc) + (st[0:1, gc] + b2f[:, gc])
            ost[gc, :] = xn.T.astype(BF16)

        def body(i, c):
            step(xa, i * CH, 2 * i * CH)
            step(xb, i * CH, (2 * i + 1) * CH)
            o_copy(2 * i).start()
            o_copy(2 * i + 1).start()
            return c
        lax.fori_loop(0, NCH // 2, body, 0)

    c_copies[0].wait()
    with jax.named_scope("first_cols"):
        for j in range(NCH):
            x_copy(j).wait()
            if j == 2:
                for cp in w_copies:
                    cp.start()
                for cp in c_copies[2:]:
                    cp.start()
            buf, loff = (xa, xb)[j % 2], (j // 2) * CH
            gc = pl.ds(j * CH, CH)
            xt = xin[gc, :].astype(F32).T
            pilot = xt[0:1]
            xn = xt - pilot
            buf[:, pl.ds(loff, CH)] = xn
            dlt, var = put_stats(gc, xn)
            st[0:1, gc] = pilot
            st[1:2, gc] = dlt
            st[2:3, gc] = var
            if j > 0:
                col_fwd((xa, xb)[(j - 1) % 2], ((j - 1) // 2) * CH, (j - 1) * CH)
        col_fwd(xb, 3 * CH, 7 * CH)
    w1_copy.start()
    w2_copy.start()
    with jax.named_scope("radix_fwd"):
        lax.fori_loop(0, NG, radix_fwd, 0)
    spectral_first()
    for cp in c_copies[2:]:
        cp.wait()
    b1f[...] = b1_ref[...].reshape(1, F).astype(F32)
    b2f[...] = b2_ref[...].reshape(1, S).astype(F32)

    def layer(l, c):
        with jax.named_scope("radix_inv"):
            radix_inv_all()
        with jax.named_scope("col_inv"):
            col_inv_all()

        @pl.when(l == 0)
        def _():
            w1_copy.wait()

        with jax.named_scope("mlp_up"):
            mlp_up()

        @pl.when(l == 0)
        def _():
            w2_copy.wait()
            with jax.named_scope("mlp_down"):
                mlp_down_mid()
            with jax.named_scope("radix_fwd"):
                lax.fori_loop(0, NG, radix_fwd, 0)
            with jax.named_scope("spectral"):
                spectral()

        @pl.when(l == 1)
        def _():
            with jax.named_scope("mlp_down_last"):
                mlp_down_last()
        return c

    lax.fori_loop(0, 2, layer, 0)
    for j in range(NCH):
        o_copy(j).wait()


@jax.jit
def pallas_interleave_layers__spectral_gfnet__mixer_token_mlp__prompt_kernel(A_x, A_w_r, A_w_i, B_x, B_w1, B_b1, B_w2, B_b2):
    del B_x
    fwd, inv, ft = _tables()
    hbm = pl.BlockSpec(memory_space=pltpu.HBM)
    out = pl.pallas_call(
        _kernel,
        out_shape=jax.ShapeDtypeStruct((S, D), BF16),
        in_specs=[hbm] * 10,
        out_specs=hbm,
        scratch_shapes=[
            pltpu.VMEM((S, D), BF16),
            pltpu.VMEM((672, S), BF16),
            pltpu.VMEM((2, 1, S), BF16),
            pltpu.VMEM((3, S, 128), U32),
            pltpu.VMEM((F, S), BF16),
            pltpu.VMEM((F, S), BF16),
            pltpu.VMEM((F,), BF16),
            pltpu.VMEM((S,), BF16),
            pltpu.VMEM(fwd.shape, U32),
            pltpu.VMEM(inv.shape, U32),
            pltpu.VMEM(ft.shape, F32),
            pltpu.VMEM((1, F), F32),
            pltpu.VMEM((1, S), F32),
            pltpu.VMEM((8, S), F32),
            pltpu.VMEM((D, S // 2), F32),
            pltpu.VMEM((D, S // 2), F32),
            pltpu.VMEM((R, S), F32),
            pltpu.VMEM((R, S), F32),
            pltpu.VMEM((16, R, 384), BF16),
            pltpu.VMEM((16, R, 256), F32),
            pltpu.VMEM((896, S), BF16),
            pltpu.VMEM((D // 2, S), U32),
            pltpu.VMEM((D // 2, F), U32),
            pltpu.VMEM((16, R, 128), U32),
            pltpu.VMEM((16, 3, 64, 128), U32),
            pltpu.VMEM((S, D), BF16),
            pltpu.SemaphoreType.DMA((NCH,)),
            pltpu.SemaphoreType.DMA((4,)),
            pltpu.SemaphoreType.DMA((2,)),
            pltpu.SemaphoreType.DMA((NCH,)),
            pltpu.SemaphoreType.DMA((5,)),
        ],
        compiler_params=pltpu.CompilerParams(vmem_limit_bytes=110 * 1024 * 1024),
    )(A_x.reshape(S, D), A_w_r.T, A_w_i.T, B_w1.T, B_b1, B_w2, B_b2,
      jnp.asarray(fwd), jnp.asarray(inv), jnp.asarray(ft))
    return out.reshape(1, S, D)
```

```python
import os
import numpy as np
import jax
import jax.numpy as jnp
from jax import lax
import jax.experimental.pallas as pl
import jax.experimental.pallas.tpu as pltpu

S, D, F = 2048, 640, 1728
DF = D // 2 + 1
R = 336
NG = 41
CH = 256
NCH = S // CH
EPS = 1e-5
F32 = jnp.float32
BF16 = jnp.bfloat16
U32 = jnp.uint32

_S1 = float(np.sin(2 * np.pi / 5))
_S2 = float(np.sin(4 * np.pi / 5))
_C5 = float((np.cos(2 * np.pi / 5) - np.cos(4 * np.pi / 5)) / 2)
_RHO = _S2 / _S1
_TILE_CLASS = ((4, -1), (2, 1), (1, 1), (3, -1))
_PAIRS = ((0, 5), (2, 7), (4, 9), (6, 1), (8, 3))
_RH = float(np.sqrt(0.5))


def _pack_rows(a):
    u = np.asarray(a, np.float32).view(np.uint32)
    u = (u + 0x7FFF + ((u >> 16) & 1)) >> 16
    return (u[..., 0::2, :] | (u[..., 1::2, :] << 16)).astype(np.uint32)


_DC_SCALE = float((_pack_rows(np.full((2, 1), 1.0 / (D * S))) << 16).view(np.float32)[0, 0])


def _tables():
    q = np.arange(64)
    j10 = 10 * np.arange(32)

    def cs(k):
        th = 2 * np.pi * np.outer(k, q) / D
        return np.cos(th), np.sin(th)

    sc = 2.0 / (D * S)
    z = np.zeros((32, 64))
    c0, s0 = cs(j10)
    c5, s5 = cs(5 + j10)
    cn, _ = cs(np.array([D // 2]))
    nyq = np.zeros((16, 128))
    nyq[0, :64] = cn[0]
    m0 = np.block([[c0, z], [z, c5], [-s0, z], [z, -s5]])
    i0 = m0.T * sc
    i0[:, 0] *= 0.5
    i0[:, 64] = nyq[0] * 0.5 * sc
    fwd, inv = [nyq, m0], [i0]
    for c, sgn in _TILE_CLASS:
        cA, sA = cs(c + j10)
        cB, sB = cs(10 - c + j10)
        m = np.block([[cA, sA], [cB, -sB], [-sA, cA], [-sB, -cB]])
        colscale = np.concatenate([np.ones(64), -sgn * _S1 * np.ones(64)])
        rowscale = np.concatenate([np.ones(64), sgn * _S1 * np.ones(64)])
        fwd.append(m * colscale[None, :])
        inv.append(m.T * sc * rowscale[:, None])
    b = np.arange(128)
    th = 2 * np.pi * np.outer(b, b) / 128
    tt = 2 * np.pi * np.outer(np.arange(16), b) / S
    ft = np.concatenate([np.cos(th), -np.sin(th), np.cos(tt), -np.sin(tt)])
    kperm = np.stack([np.arange(64), 64 + np.arange(64)], axis=1).reshape(-1)
    return (_pack_rows(np.concatenate(fwd)[:, kperm]), _pack_rows(np.concatenate(inv)[:, kperm]), ft.astype(np.float32))


def _bfly4(a, b, c, d):
    s0r, s0i = a[0] + c[0], a[1] + c[1]
    d0r, d0i = a[0] - c[0], a[1] - c[1]
    s1r, s1i = b[0] + d[0], b[1] + d[1]
    d1r, d1i = b[0] - d[0], b[1] - d[1]
    return ((s0r + s1r, s0i + s1i), (d0r + d1i, d0i - d1r),
            (s0r - s1r, s0i - s1i), (d0r - d1i, d0i + d1r))


def _tw16(z, e):
    r, i = z
    if e == 0:
        return z
    if e == 4:
        return (i, -r)
    if e == 2:
        return ((r + i) * _RH, (i - r) * _RH)
    if e == 6:
        return ((i - r) * _RH, (r + i) * (-_RH))
    c, s = float(np.cos(2 * np.pi * e / 16)), float(np.sin(2 * np.pi * e / 16))
    return (r * c + i * s, i * c - r * s)


def _dft16(x):
    t = []
    for a0 in range(4):
        o = _bfly4(x[a0], x[4 + a0], x[8 + a0], x[12 + a0])
        t.append([_tw16(o[r0], a0 * r0) for r0 in range(4)])
    out = [None] * 16
    for r0 in range(4):
        o = _bfly4(t[0][r0], t[1][r0], t[2][r0], t[3][r0])
        for r1 in range(4):
            out[r0 + 4 * r1] = o[r1]
    return out


def _dot(a, b):
    return jnp.dot(a, b, preferred_element_type=F32)


def _dot_t(a, b):
    return lax.dot_general(a, b, (((1,), (1,)), ((), ())), preferred_element_type=F32)


def _gelu(u):
    return 0.5 * u * (1.0 + jnp.tanh(0.7978845608028654 * (u + 0.044715 * (u * u * u))))


def _cols(off, width):
    if isinstance(off, int):
        return pl.ds(off, width)
    return pl.ds(pl.multiple_of(off, 128), width)


def _bf(u):
    return pltpu.bitcast(u, BF16)


def _pk(v):
    return pltpu.bitcast(v.astype(BF16), U32)


def _pk2(lo, hi):
    return pltpu.pack_elementwise([lo, hi], packed_dtype=BF16)


_PIECES = []
_r = 0
for _k in (0, 5, None) + tuple(v for c, _ in _TILE_CLASS for v in (c, 10 - c)):
    if _k is None:
        _PIECES.append((_r, 16, None, None))
        _r += 16
    else:
        _PIECES.append((_r, 32, _k // 2, _k % 2))
        _r += 32
EARLY = int(os.environ.get('EARLY', '2'))
LATE = int(os.environ.get('LATE', '3'))
SLF = int(os.environ.get('SLF', '8'))
SLI = int(os.environ.get('SLI', '8'))
DM_MODE = int(os.environ.get('DM_MODE', '3'))
F_MODE = int(os.environ.get('F_MODE', '5'))
PAD = int(os.environ.get('PAD', '128'))
PY = int(os.environ.get('PY', '0'))
UP_MODE = int(os.environ.get('UP_MODE', '2'))
PW = int(os.environ.get('PW', '128'))
PB = int(os.environ.get('PB', '128'))
PA = int(os.environ.get('PA', '0'))
S1_SPLIT = int(os.environ.get('SPLIT', '176'))
UN = int(os.environ.get('UN', '512'))
F0 = 3 * UN
W1_PIECES = ((F0, F - F0), (0, UN), (UN, UN), (2 * UN, UN))


def _groups(lo, hi):
    return [g for g in range(lo // 8, hi // 8) if g != 9]


def _kernel(x_hbm, wr_hbm, wi_hbm, w1_hbm, b1_hbm, w2_hbm, b2_hbm, fwd_hbm, inv_hbm, ft_hbm,
            out_hbm,
            xin, wraw, wnyq, wn, w1, w2, b1_ref, b2_ref, fwd_ref, inv_ref, ft_ref,
            b1f, b2f, st, xa, xb, ab, al, yr, yi, tb, tp, yb, hb, gb, vraw, uat, wt, g3, ost, flag,
            sem_x, sem_w, sem_m, sem_o, sem_c):
    def x_copy(j):
        return pltpu.make_async_copy(x_hbm.at[pl.ds(j * CH, CH), :], xin.at[pl.ds(j * CH, CH), :], sem_x.at[j])

    def o_copy(j):
        return pltpu.make_async_copy(ost.at[pl.ds(j * 128, 128), :], out_hbm.at[pl.ds(j * 128, 128), :], sem_o.at[0])

    w_half = [[], []]
    for ri, src in enumerate((wr_hbm, wi_hbm)):
        for h in range(2):
            w_half[h].append(pltpu.make_async_copy(
                src.at[pl.ds(0, 320), pl.ds(1024 * h, 1024)],
                wraw.at[pl.ds(320 * ri, 320), pl.ds(1024 * h, 1024)], sem_w.at[3 * ri + h]))
        w_half[0].append(pltpu.make_async_copy(src.at[pl.ds(320, 1), :], wnyq.at[ri], sem_w.at[3 * ri + 2]))

    def w1_copy(i):
        if isinstance(i, int):
            rows = pl.ds(*W1_PIECES[i])
        else:
            rows = pl.ds(pl.multiple_of((i - 1) * UN, 128), UN)
        return pltpu.make_async_copy(w1_hbm.at[rows, :], w1.at[rows, pl.ds(0, S)], sem_m.at[i])

    w2_copy = pltpu.make_async_copy(w2_hbm, w2.at[:, pl.ds(0, S)], sem_m.at[4])
    c_pairs = ((fwd_hbm, fwd_ref), (ft_hbm, ft_ref), (inv_hbm, inv_ref), (b1_hbm, b1_ref), (b2_hbm, b2_ref))
    c_copies = [pltpu.make_async_copy(a, b, sem_c.at[i]) for i, (a, b) in enumerate(c_pairs)]

    c_copies[1].start()

    def start_x(j, c):
        x_copy(j).start()

        @pl.when(j == 0)
        def _():
            c_copies[0].start()
        return c
    lax.fori_loop(0, NCH, start_x, 0)

    flag[0] = 1
    yi[64:80, 0:S] = jnp.zeros((16, S), F32)
    tb[:, 64:80, :] = jnp.zeros((16, 16, 384), BF16)

    def block(name, fn):
        with jax.named_scope(name):
            pl.when(flag[0] == 1)(fn)

    def fold8(v):
        out = v[0:8]
        for i in range(1, v.shape[0] // 8):
            out = out + v[8 * i:8 * (i + 1)]
        return out

    def acc_stats(acc, xn):
        a1, a2 = fold8(xn), fold8(xn * xn)
        return (a1, a2) if acc is None else (acc[0] + a1, acc[1] + a2)

    def fin_stats(acc):
        dlt = jnp.sum(acc[0], axis=0, keepdims=True) * (1.0 / D)
        msq = jnp.sum(acc[1], axis=0, keepdims=True) * (1.0 / D)
        return dlt, jnp.maximum(msq - dlt * dlt, 0.0)

    def col_pre(buf, loff, goff, slot, slabs=None, width=CH, sub=0):
        lc, gc, ac = _cols(loff + sub, width), _cols(goff + sub, width), pl.ds(CH * slot + sub, width)
        slabs = range(64 // SLF) if slabs is None else slabs
        r = lax.rsqrt(st[2:3, gc] + EPS)
        rc, rr, d10 = r * _C5, r * _RHO, st[1:2, gc] * r * 10.0

        def radix5(x0, x1, x2, x3, x4):
            t1, t2, t3, t4 = x1 + x4, x2 + x3, x1 - x4, x2 - x3
            u = (t1 + t2) * r
            x0 = x0 * r
            m = x0 - 0.25 * u
            n = (t1 - t2) * rc
            return x0 + u, m + n, t3 * r + t4 * rr, m - n, t3 * rr - t4 * r

        for sl in slabs:
            sm, df = [], []
            for pa, pb in _PAIRS:
                va = buf[64 * pa + SLF * sl:64 * pa + SLF * (sl + 1), lc]
                vb = buf[64 * pb + SLF * sl:64 * pb + SLF * (sl + 1), lc]
                sm.append(va + vb)
                df.append(va - vb)
            s0, s1r, s1i, s2r, s2i = radix5(*sm)
            d0, d1r, d1i, d2r, d2i = radix5(*df)
            for t, pair in enumerate(((s0 - d10, d0), (s1r, s1i), (s2r, s2i), (d1r, d1i), (d2r, d2i))):
                if t < LATE:
                    ab[64 * t + SLF * sl:64 * t + SLF * (sl + 1), ac] = _pk2(*pair)
                else:
                    al[64 * (t - LATE) + SLF * sl:64 * (t - LATE) + SLF * (sl + 1), gc] = _pk2(*pair)

    def col_dft(goff, slot, halves=range(2)):
        for h in halves:
            cols = _cols(goff + 128 * h, 128)
            ac = pl.ds(CH * slot + 128 * h, 128)
            o = _dot(_bf(fwd_ref[0:72, :]), _bf(ab[0:64, ac]))
            yr[64:80, cols] = o[0:16]
            yr[0:64, cols] = o[16:80]
            yi[0:64, cols] = o[80:144]
            for t in range(1, LATE):
                dft_tile(t, cols, ab[64 * t:64 * (t + 1), ac])

    def dft_tile(t, cols, operand):
        o = _dot(_bf(fwd_ref[8 + 64 * t:72 + 64 * t, :]), _bf(operand))
        yr[16 + 64 * t:80 + 64 * t, cols] = o[0:64]
        yi[16 + 64 * t:80 + 64 * t, cols] = o[64:128]

    def dft_late(blk):
        cols = pl.ds(128 * blk, 128)
        for t in range(LATE, 5):
            dft_tile(t, cols, al[64 * (t - LATE):64 * (t - LATE + 1), cols])

    def col_fwd(buf, loff, goff, slot):
        col_pre(buf, loff, goff, slot)
        col_dft(goff, slot)

    def rf(g):
        rows = pl.ds(g * 8, 8)
        x = [(yr[rows, 128 * a:128 * (a + 1)], yi[rows, 128 * a:128 * (a + 1)]) for a in range(16)]
        o = _dft16(x)
        for m1 in range(16):
            tb[m1, rows, :] = jnp.concatenate([o[m1][0] + o[m1][1], o[m1][0], o[m1][1]], axis=1).astype(BF16)

    def idft(g):
        rows = pl.ds(g * 8, 8)
        x = [(tp[m1, rows, 128:256], tp[m1, rows, 0:128]) for m1 in range(16)]
        o = _dft16(x)
        return [o[a][1] for a in range(16)], [o[a][0] for a in range(16)]

    def row_bf16(vals):
        return jnp.concatenate(vals, axis=1).astype(BF16)

    def ri(g):
        if g == 8:
            return
        re, im = idft(g)
        if g == 0:
            ren, _ = idft(8)
            first = lax.broadcasted_iota(jnp.int32, (8, 128), 0) == 0
            im = [jnp.where(first, a, b) for a, b in zip(ren, im)]
        gg = g if g < 8 else g - 2
        for a in range(16):
            yb[pl.ds(8 * gg, 8), 128 * a:128 * (a + 1)] = _pk2(re[a], im[a])

    def gmat(m1, i):
        return _bf(g3[:, 128 * (3 * m1 + i):128 * (3 * m1 + i + 1)])

    def gen_g(m1):
        tr = ft_ref[256 + m1:257 + m1, :]
        ti = ft_ref[272 + m1:273 + m1, :]
        fr = ft_ref[0:128, :]
        fi = ft_ref[128:256, :]
        gr = fr * tr - fi * ti
        gi = fr * ti + fi * tr
        g3[:, 384 * m1:384 * (m1 + 1)] = _pk(jnp.concatenate([gr, gi - gr, gr + gi], axis=1))

    def half(v, h):
        return pltpu.bitcast(v << 16 if h == 0 else v & jnp.uint32(0xFFFF0000), F32)

    def load_wt(m1, lo, hi):
        res = []
        for c in range(2):
            ps = []
            for (r0, n, w0, h) in _PIECES:
                a, b = max(lo, r0), min(hi, r0 + n)
                if a >= b:
                    continue
                if w0 is None:
                    ps.append(half(wt[m1, 320 + a - r0:320 + b - r0, :], c))
                else:
                    ps.append(half(wt[m1, pl.ds(160 * c + w0 + 5 * (a - r0), b - a, stride=5), :], h))
            res.append(jnp.concatenate(ps, axis=0))
        return res

    def spec_fwd(m1, lo, hi):
        k1, k2, k3 = [_dot_t(tb[m1, lo:hi, 128 * i:128 * (i + 1)], gmat(m1, i)) for i in range(3)]
        return k1 - k3, k1 + k2

    def spec_mul(m1, lo, hi, xr, xi):
        wr_, wi_ = load_wt(m1, lo, hi)
        zr = xr * wr_ - xi * wi_
        zi = xr * wi_ + xi * wr_
        return (zr + zi).astype(BF16), zi.astype(BF16), zr.astype(BF16)

    def spec_inv(m1, lo, hi, z):
        q1, q2, q3 = [_dot(z[i], gmat(m1, i)) for i in range(3)]
        tp[m1, lo:hi, 0:128] = q1 + q2
        tp[m1, lo:hi, 128:256] = q1 - q3

    def spread(side, m1):
        n = len(side)
        for fn, arg in side[(m1 * n) // 16:((m1 + 1) * n) // 16]:
            fn(arg)

    def run_all(side):
        def fn():
            for f, arg in side:
                f(arg)
        return fn

    def merge(a, b):
        keyed = [((i + 0.5) / len(b), 0, w) for i, w in enumerate(b)] + [((i + 0.75) / len(a), 1, w) for i, w in enumerate(a)]
        return [w for _, _, w in sorted(keyed, key=lambda t: t[:2])]

    A, B = (0, S1_SPLIT), (S1_SPLIT, R)

    def prep1(j):
        cols = pl.ds(j * 128, 128)
        wn[0, cols, :] = pltpu.bitcast(wraw[0:256, cols], U32).T
        wn[1, cols, :] = pltpu.bitcast(wraw[256:512, cols], U32).T
        wn[2, cols, 0:80] = pltpu.bitcast(wraw[512:672, cols], U32).T

    def prep2(m1):
        wt[m1, 0:128, :] = wn[0, pl.ds(m1, 128, stride=16), :].T
        wt[m1, 128:256, :] = wn[1, pl.ds(m1, 128, stride=16), :].T
        wt[m1, 256:336, :] = wn[2, pl.ds(m1, 128, stride=16), :].T[0:80]

    def fwd_pass(rows, side):
        def fn():
            for m1 in range(16):
                spread(side, m1)
                xr, xi = spec_fwd(m1, *rows)
                tp[m1, rows[0]:rows[1], 0:128] = xr
                tp[m1, rows[0]:rows[1], 128:256] = xi
        return fn

    def inv_pass(rows, side, pre):
        lo, hi = rows

        def fn():
            for m1 in range(16):
                if m1 in pre:
                    prep2(m1)
                spread(side, m1)
                spec_inv(m1, lo, hi, spec_mul(m1, lo, hi, tp[m1, lo:hi, 0:128], tp[m1, lo:hi, 128:256]))
        return fn

    def spectral_mid_first():
        with jax.named_scope("wait_w0"):
            for cp in w_half[0]:
                cp.wait()
        for cp in c_copies[2:]:
            cp.start()
        w1_copy(0).start()
        wraw[640:672, :] = jnp.concatenate(
            [wnyq[0].astype(F32), wnyq[1].astype(F32), jnp.zeros((30, S), F32)], axis=0).astype(BF16)
        side = [(rf, g) for g in _groups(*B)]
        side = merge(side, [(prep1, j) for j in range(8)])
        block("s1_fwdA", fwd_pass(A, side))
        with jax.named_scope("wait_w1"):
            for cp in w_half[1]:
                cp.wait()
        w1_copy(1).start()
        block("s1_fwdB", fwd_pass(B, [(prep1, j) for j in range(8, 16)] + [(prep2, m) for m in range(5)]))
        block("s1_invA", inv_pass(A, [], range(5, 16)))
        w1_copy(2).start()
        for cp in c_copies[2:]:
            cp.wait()
        w1_copy(0).wait()
        b1f[...] = b1_ref[...].reshape(1, F).astype(F32)
        b2f[...] = b2_ref[...].reshape(1, S).astype(F32)

    def spectral_mid_second():
        block("s2_fwdA", fwd_pass(A, [(rf, g) for g in _groups(*B)]))

        def rest():
            fwd_pass(B, [])()
            inv_pass(A, [], ())()
        block("s2_fwdB_invA", rest)

    def inv_dot(t, cols):
        return _dot(_bf(inv_ref[64 * t:64 * (t + 1), :]), _bf(yb[64 * t:64 * (t + 1), cols]))

    def inv_early(blk):
        cols = pl.ds(128 * blk, 128)
        for t in range(EARLY):
            vraw[128 * t:128 * (t + 1), cols] = inv_dot(t, cols)

    def inv_dots(goff):
        cols = _cols(goff, 128)
        return [None if t < EARLY else inv_dot(t, cols) for t in range(5)]

    def inv_post(buf, loff, goff, v):
        lc, gc = _cols(loff, 128), _cols(goff, 128)
        shift = st[1:2, gc] + half(yb[0:1, gc], 0) * _DC_SCALE
        st[0:1, gc] = st[0:1, gc] + shift

        def iradix5(v0, v1r, v1i, v2r, v2i):
            t1 = v1r + v2r
            m = v0 - 0.25 * t1
            n = _C5 * (v1r - v2r)
            a, b = m + n, m - n
            cc = v1i + _RHO * v2i
            dd = _RHO * v1i - v2i
            return v0 + t1, a - cc, b - dd, b + dd, a + cc

        acc = None
        for sl in range(64 // SLI):
            lo, hi = slice(SLI * sl, SLI * (sl + 1)), slice(64 + SLI * sl, 64 + SLI * (sl + 1))
            def get(t, rs):
                if t < EARLY:
                    return vraw[128 * t + rs.start:128 * t + rs.stop, gc]
                return v[t][rs]
            ys = iradix5(get(0, lo) - shift, get(1, lo), get(1, hi), get(2, lo), get(2, hi))
            yd = iradix5(get(0, hi), get(3, lo), get(3, hi), get(4, lo), get(4, hi))
            for (pa, pb), a, b in zip(_PAIRS, ys, yd):
                for p, y in ((pa, a + b), (pb, a - b)):
                    rows = slice(64 * p + SLI * sl, 64 * p + SLI * (sl + 1))
                    xn = buf[rows, lc] + y
                    buf[rows, lc] = xn
                    sq = fold8(xn * xn)
                    acc = sq if acc is None else acc + sq
        var = jnp.sum(acc, axis=0, keepdims=True) * (1.0 / D)
        r1 = lax.rsqrt(var + EPS)
        return (r1 * lax.rsqrt(var * r1 * r1 + EPS),)

    def inv_norm(buf, loff, goff, rr):
        lc, gc = _cols(loff, 128), _cols(goff, 128)
        for sl in range(20):
            hb[16 * sl:16 * (sl + 1), gc] = _pk(buf[32 * sl:32 * (sl + 1), lc] * rr)

    def col_inv_up():
        f0 = W1_PIECES[0][0]

        def up(t):
            kc = pl.ds(t * CH, CH)
            if UP_MODE == 0:
                d = _dot_t(_bf(hb[:, kc]), w1[f0:F, kc])
                if t == 0:
                    uacc[...] = d
                elif t + 1 < NCH:
                    uacc[...] += d
                else:
                    gb[:, f0:F] = _pk(_gelu(uacc[...] + d + b1f[:, f0:F]))
                return
            d = _dot_t(w1[f0:F, kc], _bf(hb[:, kc]))
            if t == 0:
                uat[:, 0:D] = d
            elif t + 1 < NCH or UP_MODE == 2:
                uat[:, 0:D] += d
            else:
                u = (uat[:, 0:D] + d).T
                gb[:, f0:F] = _pk(_gelu(u + b1f[:, f0:F]))

        def where(blk):
            j = blk // 2
            return (xa, xb)[j % 2], (j // 2) * CH + 128 * (blk % 2), 128 * blk

        nlag, ulag = int(os.environ.get('NLAG', '1')), int(os.environ.get('ULAG', '2'))
        v = inv_dots(0)
        sc = {}
        done = 0
        for blk in range(16 + nlag):
            if blk < 16:
                vn = inv_dots(128 * (blk + 1)) if blk + 1 < 16 else None
                sc[blk] = inv_post(*where(blk), v)
                v = vn
            nb = blk - nlag
            if nb >= 0:
                inv_norm(*where(nb), *sc[nb])
            while 2 * done + 1 + ulag <= nb:
                up(done)
                done += 1
        while done < NCH:
            up(done)
            done += 1

    def mlp_up(l):
        def one(cols):
            u = _dot_t(_bf(hb[:, 0:S]), w1[cols, 0:S]) + b1f[:, cols]
            gb[:, cols] = _pk(_gelu(u))

        def body(j, c):
            @pl.when(l == 0)
            def _():
                w1_copy(j + 1).wait()

            first = 256 if UN == 512 else 128
            one(_cols(j * UN, first))
            off = jnp.minimum(j * 256, D - 256)
            u = uat[:, pl.ds(pl.multiple_of(off, 128), 256)].T
            gb[pl.ds(pl.multiple_of(off // 2, 64), 128), F0:F] = _pk(_gelu(u + b1f[:, F0:F]))
            one(_cols(j * UN + first, 256))
            return c
        lax.fori_loop(0, 3, body, 0)

    def down_y(gc):
        return _dot(_bf(gb[...]), w2[:, gc])

    def mlp_down_mid():
        def step(cur, loff, goff, prev, ploff, pgoff, slot):
            lc, gc = _cols(loff, CH), _cols(goff, CH)
            pre = lambda sl: col_pre(prev, ploff, pgoff, slot, sl)
            dft = lambda h: col_dft(pgoff, slot, h)
            plans = {
                3: (2, {0: [lambda: pre(None)], 1: [lambda: dft(range(2))]}),
                4: (4, {0: [lambda: pre(range(4))], 1: [lambda: pre(range(4, 8))], 2: [lambda: dft([0])], 3: [lambda: dft([1])]}),
                5: (4, {1: [lambda: pre(range(4))], 2: [lambda: pre(range(4, 8))], 3: [lambda: dft(range(2))]}),
                6: (5, {0: [lambda: pre(range(3))], 1: [lambda: pre(range(3, 6))], 2: [lambda: pre(range(6, 8))], 3: [lambda: dft([0])], 4: [lambda: dft([1])]}),
                7: (2, {0: [lambda: pre(range(8))], 2: [lambda: dft(range(2))]}),
                8: (4, {0: [lambda: pre(range(8))], 2: [lambda: dft(range(2))]}),
            }
            nb, plan = plans[DM_MODE]
            mb = D // nb
            acc = None
            row0 = None
            for b in range(nb + 1):
                for fn in plan.get(b, []):
                    fn()
                if b == nb:
                    break
                y = _dot(_bf(gb[mb // 2 * b:mb // 2 * (b + 1), :]), w2[:, gc])
                if b == 0:
                    row0 = cur[0:1, lc] + y[0:1]
                for sl in range(mb // 16):
                    rows = slice(mb * b + 16 * sl, mb * b + 16 * (sl + 1))
                    xn = cur[rows, lc] + (y[16 * sl:16 * (sl + 1)] - row0)
                    cur[rows, lc] = xn
                    acc = acc_stats(acc, xn)
            dlt, var = fin_stats(acc)
            st[0:1, gc] = st[0:1, gc] + row0 + b2f[:, gc]
            st[1:2, gc] = dlt
            st[2:3, gc] = var

        def body(i, c):
            ip = (i + 3) % 4
            step(xa, i * CH, 2 * i * CH, xb, ip * CH, (2 * ip + 1) * CH, 0)
            step(xb, i * CH, (2 * i + 1) * CH, xa, i * CH, 2 * i * CH, 1)
            return c
        lax.fori_loop(0, NCH // 2, body, 0)
        for h in range(2):
            col_pre(xb, 3 * CH, 7 * CH, 0, width=128, sub=128 * h)
            col_dft(7 * CH, 0, [h])

    def mlp_down_last():
        def step(cur, loff, j):
            y = down_y(_cols(j * CH, CH))
            for h in range(2):
                gc = _cols(j * CH + 128 * h, 128)
                xn = cur[:, _cols(loff + 128 * h, 128)] + y[:, 128 * h:128 * (h + 1)] + (st[0:1, gc] + b2f[:, gc])
                ost[gc, :] = xn.T.astype(BF16)
                o_copy(2 * j + h).start()

        def body(i, c):
            step(xa, i * CH, 2 * i)
            step(xb, i * CH, 2 * i + 1)
            return c
        lax.fori_loop(0, NCH // 2, body, 0)

    def loc(j):
        return (xa, xb)[j % 2], (j // 2) * CH

    def stage_t(j):
        buf, loff = loc(j)
        gc = pl.ds(j * CH, CH)
        xt = xin[gc, :].astype(F32).T
        pilot = xt[0:1]
        acc = None
        for sl in range(40):
            rows = slice(16 * sl, 16 * (sl + 1))
            xn = xt[rows] - pilot
            buf[rows, pl.ds(loff, CH)] = xn
            acc = acc_stats(acc, xn)
        dlt, var = fin_stats(acc)
        st[0:1, gc] = pilot
        st[1:2, gc] = dlt
        st[2:3, gc] = var

    def stage_p(j):
        buf, loff = loc(j)
        col_pre(buf, loff, j * CH, j % 2)

    def stage_d(j):
        col_dft(j * CH, j % 2)

    def stage_pd(j):
        buf, loff = loc(j)
        for h in range(2):
            col_pre(buf, loff, j * CH, j % 2, width=128, sub=128 * h)
            col_dft(j * CH, j % 2, [h])

    c_copies[1].wait()
    with jax.named_scope("gen_g"):
        for m1 in range(16):
            gen_g(m1)
    def dma_hooks(j):
        x_copy(j).wait()
        if j == 1:
            c_copies[0].wait()
        if j == 5:
            for cp in w_half[0]:
                cp.start()
        if j == 7:
            for cp in w_half[1]:
                cp.start()

    def seq(*items):
        def fn():
            for f, j in items:
                if 0 <= j < NCH:
                    f(j)
        return fn

    if F_MODE == 0:
        for j in range(NCH):
            dma_hooks(j)
            block("f_step", seq((stage_d, j - 2), (stage_t, j), (stage_p, j - 1)))
        block("f_tail1", seq((stage_d, NCH - 2), (stage_p, NCH - 1)))
        block("f_tail2", seq((stage_d, NCH - 1)))
    elif F_MODE == 1:
        for j in range(NCH):
            dma_hooks(j)
            block("f_step", seq((stage_d, j - 1), (stage_t, j), (stage_p, j)))
        block("f_tail2", seq((stage_d, NCH - 1)))
    elif F_MODE == 2:
        for j in range(NCH):
            dma_hooks(j)
            block("f_step", seq((stage_p, j - 1), (stage_d, j - 1), (stage_t, j)))
        block("f_tail2", seq((stage_p, NCH - 1), (stage_d, NCH - 1)))
    elif F_MODE == 5:
        for j in range(NCH):
            dma_hooks(j)
            block("f_step", seq((stage_pd, j - 1), (stage_t, j)))
        block("f_tail2", seq((stage_pd, NCH - 1)))
    elif F_MODE == 3:
        dma_hooks(0)
        block("f_step", seq((stage_t, 0)))
        for j in range(1, NCH, 2):
            dma_hooks(j)
            if j + 1 < NCH:
                dma_hooks(j + 1)
            block("f_step", seq((stage_p, j - 2), (stage_d, j - 2), (stage_p, j - 1), (stage_d, j - 1), (stage_t, j), (stage_t, j + 1)))
        block("f_tail2", seq((stage_p, NCH - 1), (stage_d, NCH - 1)))
    elif F_MODE == 4:
        for j in range(NCH):
            dma_hooks(j)
            block("f_step", seq((stage_d, j - 2), (stage_t, j), (stage_p, j - 1)))
        block("f_tail1", seq((stage_d, NCH - 2), (stage_p, NCH - 1), (stage_d, NCH - 1)))

    def layer(l, c):
        block("s_rf", run_all(merge([(rf, g) for g in _groups(*A)], [(dft_late, b) for b in range(16)] if LATE < 5 else [])))
        pl.when(l == 0)(spectral_mid_first)
        pl.when(l == 1)(spectral_mid_second)
        block("s_invB", inv_pass(B, [(ri, g) for g in _groups(*A)], ()))
        block("s_ri", run_all(merge([(ri, g) for g in _groups(*B)], [(inv_early, b) for b in range(16)] if EARLY else [])))
        with jax.named_scope("col_inv_up"):
            col_inv_up()

        @pl.when(l == 0)
        def _():
            w1_copy(3).start()
            w2_copy.start()

        with jax.named_scope("mlp_up"):
            mlp_up(l)

        @pl.when(l == 0)
        def _():
            w2_copy.wait()
            with jax.named_scope("mlp_down"):
                mlp_down_mid()

        @pl.when(l == 1)
        def _():
            with jax.named_scope("mlp_down_last"):
                mlp_down_last()
        return c

    lax.fori_loop(0, 2, layer, 0)
    with jax.named_scope("final_wait"):
        pltpu.make_async_copy(ost, out_hbm, sem_o.at[0]).wait()


@jax.jit
def pallas_interleave_layers__spectral_gfnet__mixer_token_mlp__prompt_kernel(A_x, A_w_r, A_w_i, B_x, B_w1, B_b1, B_w2, B_b2):
    del B_x
    fwd, inv, ft = _tables()
    hbm = pl.BlockSpec(memory_space=pltpu.HBM)
    out = pl.pallas_call(
        _kernel,
        out_shape=jax.ShapeDtypeStruct((S, D), BF16),
        in_specs=[hbm] * 10,
        out_specs=hbm,
        scratch_shapes=[
            pltpu.VMEM((S, D), BF16),
            pltpu.VMEM((672, S), BF16),
            pltpu.VMEM((2, 1, S), BF16),
            pltpu.VMEM((3, S, 128), U32),
            pltpu.VMEM((F, S + PW), BF16),
            pltpu.VMEM((F, S + PW), BF16),
            pltpu.VMEM((F,), BF16),
            pltpu.VMEM((S,), BF16),
            pltpu.VMEM(fwd.shape, U32),
            pltpu.VMEM(inv.shape, U32),
            pltpu.VMEM(ft.shape, F32),
            pltpu.VMEM((1, F), F32),
            pltpu.VMEM((1, S), F32),
            pltpu.VMEM((8, S), F32),
            pltpu.VMEM((D, S // 2 + PAD), F32),
            pltpu.VMEM((D, S // 2 + PB), F32),
            pltpu.VMEM((320, 512 + PA), U32),
            pltpu.VMEM((192, S + PAD), U32),
            pltpu.VMEM((R, S + PY), F32),
            pltpu.VMEM((R, S + PY), F32),
            pltpu.VMEM((16, R, 384), BF16),
            pltpu.VMEM((16, R, 256), F32),
            pltpu.VMEM((D // 2, S + PAD), U32),
            pltpu.VMEM((D // 2, S + PAD), U32),
            pltpu.VMEM((D // 2, F), U32),
            pltpu.VMEM((384, S + PAD), F32),
            pltpu.VMEM((F - F0, D), F32),
            pltpu.VMEM((16, R, 128), U32),
            pltpu.VMEM((64, 48 * 128), U32),
            pltpu.VMEM((S, D), BF16),
            pltpu.SMEM((1,), jnp.int32),
            pltpu.SemaphoreType.DMA((NCH,)),
            pltpu.SemaphoreType.DMA((6,)),
            pltpu.SemaphoreType.DMA((5,)),
            pltpu.SemaphoreType.DMA((1,)),
            pltpu.SemaphoreType.DMA((5,)),
        ],
        compiler_params=pltpu.CompilerParams(vmem_limit_bytes=110 * 1024 * 1024,
                                             disable_bounds_checks=bool(int(os.environ.get('NOCHK', '1'))),
                                             disable_semaphore_checks=bool(int(os.environ.get('NOCHK', '1')))),
    )(A_x.reshape(S, D), A_w_r.T, A_w_i.T, B_w1.T, B_b1, B_w2, B_b2,
      jnp.asarray(fwd), jnp.asarray(inv), jnp.asarray(ft))
    return out.reshape(1, S, D)
```

```python
import numpy as np
import jax
import jax.numpy as jnp
from jax import lax
import jax.experimental.pallas as pl
import jax.experimental.pallas.tpu as pltpu

S, D, F = 2048, 640, 1728
R = 336
CH = 256
NCH = S // CH
PAD = 128
EPS = 1e-5
F32 = jnp.float32
BF16 = jnp.bfloat16
U32 = jnp.uint32

SPLIT = 176
LATE = 3
EARLY = 2
F0 = 1536
NU = 2
UN = F0 // NU
W1_PIECES = ((F0, F - F0),) + tuple((UN * i, UN) for i in range(NU))

_S1 = float(np.sin(2 * np.pi / 5))
_S2 = float(np.sin(4 * np.pi / 5))
_C5 = float((np.cos(2 * np.pi / 5) - np.cos(4 * np.pi / 5)) / 2)
_RHO = _S2 / _S1
_RH = float(np.sqrt(0.5))
_TILE_CLASS = ((4, -1), (2, 1), (1, 1), (3, -1))
_PAIRS = ((0, 5), (2, 7), (4, 9), (6, 1), (8, 3))

_PIECES = []
for _k in (0, 5, None) + tuple(v for c, _ in _TILE_CLASS for v in (c, 10 - c)):
    _r0 = _PIECES[-1][0] + _PIECES[-1][1] if _PIECES else 0
    _PIECES.append((_r0, 16, None, None) if _k is None else (_r0, 32, _k // 2, _k % 2))


def _pack_rows(a):
    u = np.ascontiguousarray(a, np.float32).view(np.uint32)
    u = (u + 0x7FFF + ((u >> 16) & 1)) >> 16
    return (u[0::2] | (u[1::2] << 16)).astype(np.uint32)


_DC_SCALE = float((_pack_rows(np.full((2, 1), 1.0 / (D * S))) << 16).view(np.float32)[0, 0])


def _tables():
    q = np.arange(64)
    j10 = 10 * np.arange(32)

    def cs(k):
        th = 2 * np.pi * np.outer(k, q) / D
        return np.cos(th), np.sin(th)

    sc = 2.0 / (D * S)
    z = np.zeros((32, 64))
    c0, s0 = cs(j10)
    c5, s5 = cs(5 + j10)
    nyq = np.zeros((16, 128))
    nyq[0, :64] = cs(np.array([D // 2]))[0][0]
    m0 = np.block([[c0, z], [z, c5], [-s0, z], [z, -s5]])
    i0 = m0.T * sc
    i0[:, 0] *= 0.5
    i0[:, 64] = nyq[0] * 0.5 * sc
    fwd, inv = [nyq, m0], [i0]
    for c, sgn in _TILE_CLASS:
        cA, sA = cs(c + j10)
        cB, sB = cs(10 - c + j10)
        m = np.block([[cA, sA], [cB, -sB], [-sA, cA], [-sB, -cB]])
        scale = np.concatenate([np.ones(64), sgn * _S1 * np.ones(64)])
        fwd.append(m * np.concatenate([np.ones(64), -scale[64:]])[None, :])
        inv.append(m.T * sc * scale[:, None])
    kperm = np.stack([np.arange(64), 64 + np.arange(64)], axis=1).reshape(-1)
    b = np.arange(128)
    th = 2 * np.pi * np.outer(b, b) / 128
    tt = 2 * np.pi * np.outer(np.arange(16), b) / S
    ft = np.concatenate([np.cos(th), -np.sin(th), np.cos(tt), -np.sin(tt)])
    return (_pack_rows(np.concatenate(fwd)[:, kperm]), _pack_rows(np.concatenate(inv)[:, kperm]),
            ft.astype(np.float32))


def _bfly4(a, b, c, d):
    s0r, s0i = a[0] + c[0], a[1] + c[1]
    d0r, d0i = a[0] - c[0], a[1] - c[1]
    s1r, s1i = b[0] + d[0], b[1] + d[1]
    d1r, d1i = b[0] - d[0], b[1] - d[1]
    return ((s0r + s1r, s0i + s1i), (d0r + d1i, d0i - d1r),
            (s0r - s1r, s0i - s1i), (d0r - d1i, d0i + d1r))


def _tw16(z, e):
    r, i = z
    if e == 0:
        return z
    if e == 4:
        return (i, -r)
    if e == 2:
        return ((r + i) * _RH, (i - r) * _RH)
    if e == 6:
        return ((i - r) * _RH, (r + i) * (-_RH))
    c, s = float(np.cos(2 * np.pi * e / 16)), float(np.sin(2 * np.pi * e / 16))
    return (r * c + i * s, i * c - r * s)


def _dft16(x):
    t = []
    for a0 in range(4):
        o = _bfly4(x[a0], x[4 + a0], x[8 + a0], x[12 + a0])
        t.append([_tw16(o[r0], a0 * r0) for r0 in range(4)])
    out = [None] * 16
    for r0 in range(4):
        o = _bfly4(t[0][r0], t[1][r0], t[2][r0], t[3][r0])
        for r1 in range(4):
            out[r0 + 4 * r1] = o[r1]
    return out


def _dot(a, b):
    return jnp.dot(a, b, preferred_element_type=F32)


def _dot_t(a, b):
    return lax.dot_general(a, b, (((1,), (1,)), ((), ())), preferred_element_type=F32)


def _gelu(u):
    return 0.5 * u * (1.0 + jnp.tanh(0.7978845608028654 * (u + 0.044715 * (u * u * u))))


def _cols(off, width):
    if isinstance(off, int):
        return pl.ds(off, width)
    return pl.ds(pl.multiple_of(off, 128), width)


def _bf(u):
    return pltpu.bitcast(u, BF16)


def _pk(v):
    return pltpu.bitcast(v.astype(BF16), U32)


def _pk2(lo, hi):
    return pltpu.pack_elementwise([lo, hi], packed_dtype=BF16)


def _half(v, h):
    return pltpu.bitcast(v << 16 if h == 0 else v & jnp.uint32(0xFFFF0000), F32)


def _fold8(v):
    out = v[0:8]
    for i in range(1, v.shape[0] // 8):
        out = out + v[8 * i:8 * (i + 1)]
    return out


def _acc_stats(acc, xn):
    a1, a2 = _fold8(xn), _fold8(xn * xn)
    return (a1, a2) if acc is None else (acc[0] + a1, acc[1] + a2)


def _fin_stats(acc):
    dlt = jnp.sum(acc[0], axis=0, keepdims=True) * (1.0 / D)
    msq = jnp.sum(acc[1], axis=0, keepdims=True) * (1.0 / D)
    return dlt, jnp.maximum(msq - dlt * dlt, 0.0)


def _groups(lo, hi):
    return [g for g in range(lo // 8, hi // 8) if g != 9]


def _merge(a, b):
    keyed = ([((i + 0.5) / len(b), 0, w) for i, w in enumerate(b)]
             + [((i + 0.75) / len(a), 1, w) for i, w in enumerate(a)])
    return [w for _, _, w in sorted(keyed, key=lambda t: t[:2])]


def _run_all(work):
    def fn():
        for f, arg in work:
            f(arg)
    return fn


def _spread(work, m1):
    n = len(work)
    for fn, arg in work[(m1 * n) // 16:((m1 + 1) * n) // 16]:
        fn(arg)


def _kernel(x_hbm, wr_hbm, wi_hbm, w1_hbm, b1_hbm, w2_hbm, b2_hbm, fwd_hbm, inv_hbm, ft_hbm,
            out_hbm,
            xin, wraw, wnyq, wn, w1, w2, b1_ref, b2_ref, fwd_ref, inv_ref, ft_ref,
            b1f, b2f, st, xa, xb, ab, al, yr, yi, tb, tp, yb, hb, gb, vraw, uat, wt, g3, ost, flag,
            sem_x, sem_w, sem_m, sem_o, sem_c):

    def x_copy(j):
        return pltpu.make_async_copy(x_hbm.at[pl.ds(j * CH, CH), :], xin.at[pl.ds(j * CH, CH), :], sem_x.at[j])

    def o_copy(k):
        return pltpu.make_async_copy(ost.at[pl.ds(k * 128, 128), :], out_hbm.at[pl.ds(k * 128, 128), :],
                                     sem_o.at[0])

    w_half = [[], []]
    for ri, src in enumerate((wr_hbm, wi_hbm)):
        for h in range(2):
            w_half[h].append(pltpu.make_async_copy(
                src.at[pl.ds(0, 320), pl.ds(1024 * h, 1024)],
                wraw.at[pl.ds(320 * ri, 320), pl.ds(1024 * h, 1024)], sem_w.at[3 * ri + h]))
        w_half[0].append(pltpu.make_async_copy(src.at[pl.ds(320, 1), :], wnyq.at[ri], sem_w.at[3 * ri + 2]))

    def w1_copy(i):
        if isinstance(i, int):
            rows = pl.ds(*W1_PIECES[i])
        else:
            rows = pl.ds(pl.multiple_of((i - 1) * UN, 128), UN)
        return pltpu.make_async_copy(w1_hbm.at[rows, :], w1.at[rows, pl.ds(0, S)], sem_m.at[i])

    w2_copy = pltpu.make_async_copy(w2_hbm, w2.at[:, pl.ds(0, S)], sem_m.at[NU + 1])
    fwd_copy = pltpu.make_async_copy(fwd_hbm, fwd_ref, sem_c.at[0])
    ft_copy = pltpu.make_async_copy(ft_hbm, ft_ref, sem_c.at[1])
    misc_copies = [pltpu.make_async_copy(a, b, sem_c.at[2 + i])
                   for i, (a, b) in enumerate(((inv_hbm, inv_ref), (b1_hbm, b1_ref), (b2_hbm, b2_ref)))]

    ft_copy.start()

    def start_x(j, c):
        x_copy(j).start()

        @pl.when(j == 0)
        def _():
            fwd_copy.start()
        return c
    lax.fori_loop(0, NCH, start_x, 0)

    flag[0] = 1
    yi[64:80, :] = jnp.zeros((16, S), F32)
    tb[:, 64:80, :] = jnp.zeros((16, 16, 384), BF16)

    def block(fn):
        pl.when(flag[0] == 1)(fn)

    def col_pre(buf, loff, goff, slot, width, late):
        lc, gc, ac = _cols(loff, width), _cols(goff, width), pl.ds(128 * slot, width)
        r = lax.rsqrt(st[2:3, gc] + EPS)
        rc, rr, d10 = r * _C5, r * _RHO, st[1:2, gc] * r * 10.0

        def radix5(x0, x1, x2, x3, x4):
            t1, t2, t3, t4 = x1 + x4, x2 + x3, x1 - x4, x2 - x3
            u = (t1 + t2) * r
            x0 = x0 * r
            m = x0 - 0.25 * u
            n = (t1 - t2) * rc
            return x0 + u, m + n, t3 * r + t4 * rr, m - n, t3 * rr - t4 * r

        for sl in range(8):
            sm, df = [], []
            for pa, pb in _PAIRS:
                va = buf[64 * pa + 8 * sl:64 * pa + 8 * (sl + 1), lc]
                vb = buf[64 * pb + 8 * sl:64 * pb + 8 * (sl + 1), lc]
                sm.append(va + vb)
                df.append(va - vb)
            s0, s1r, s1i, s2r, s2i = radix5(*sm)
            d0, d1r, d1i, d2r, d2i = radix5(*df)
            for t, pair in enumerate(((s0 - d10, d0), (s1r, s1i), (s2r, s2i), (d1r, d1i), (d2r, d2i))):
                if t < late:
                    ab[64 * t + 8 * sl:64 * t + 8 * (sl + 1), ac] = _pk2(*pair)
                else:
                    al[64 * (t - LATE) + 8 * sl:64 * (t - LATE) + 8 * (sl + 1), gc] = _pk2(*pair)

    def dft_tile(t, cols, operand):
        o = _dot(_bf(fwd_ref[8 + 64 * t:72 + 64 * t, :]), _bf(operand))
        yr[16 + 64 * t:80 + 64 * t, cols] = o[0:64]
        yi[16 + 64 * t:80 + 64 * t, cols] = o[64:128]

    def col_dft(goff, slot, late):
        cols, ac = _cols(goff, 128), pl.ds(128 * slot, 128)
        o = _dot(_bf(fwd_ref[0:72, :]), _bf(ab[0:64, ac]))
        yr[64:80, cols] = o[0:16]
        yr[0:64, cols] = o[16:80]
        yi[0:64, cols] = o[80:144]
        for t in range(1, late):
            dft_tile(t, cols, ab[64 * t:64 * (t + 1), ac])

    def dft_late(blk):
        cols = pl.ds(128 * blk, 128)
        for t in range(LATE, 5):
            dft_tile(t, cols, al[64 * (t - LATE):64 * (t - LATE + 1), cols])

    def col_fwd(buf, loff, goff, slot, late):
        for h in range(2):
            col_pre(buf, loff + 128 * h, goff + 128 * h, slot + h, 128, late)
            col_dft(goff + 128 * h, slot + h, late)

    def rf(g):
        rows = pl.ds(g * 8, 8)
        o = _dft16([(yr[rows, 128 * a:128 * (a + 1)], yi[rows, 128 * a:128 * (a + 1)]) for a in range(16)])
        for m1 in range(16):
            tb[m1, rows, :] = jnp.concatenate([o[m1][0] + o[m1][1], o[m1][0], o[m1][1]], axis=1).astype(BF16)

    def idft(g):
        rows = pl.ds(g * 8, 8)
        o = _dft16([(tp[m1, rows, 128:256], tp[m1, rows, 0:128]) for m1 in range(16)])
        return [o[a][1] for a in range(16)], [o[a][0] for a in range(16)]

    def ri(g):
        if g == 8:
            return
        re, im = idft(g)
        if g == 0:
            ren, _ = idft(8)
            first = lax.broadcasted_iota(jnp.int32, (8, 128), 0) == 0
            im = [jnp.where(first, a, b) for a, b in zip(ren, im)]
        gg = g if g < 8 else g - 2
        for a in range(16):
            yb[pl.ds(8 * gg, 8), 128 * a:128 * (a + 1)] = _pk2(re[a], im[a])

    def gen_g(m1):
        tr, ti = ft_ref[256 + m1:257 + m1, :], ft_ref[272 + m1:273 + m1, :]
        fr, fi = ft_ref[0:128, :], ft_ref[128:256, :]
        gr = fr * tr - fi * ti
        gi = fr * ti + fi * tr
        g3[:, 384 * m1:384 * (m1 + 1)] = _pk(jnp.concatenate([gr, gi - gr, gr + gi], axis=1))

    def gmat(m1, i):
        return _bf(g3[:, 128 * (3 * m1 + i):128 * (3 * m1 + i + 1)])

    def load_wt(m1, lo, hi):
        res = []
        for c in range(2):
            ps = []
            for (r0, n, w0, h) in _PIECES:
                a, b = max(lo, r0), min(hi, r0 + n)
                if a >= b:
                    continue
                if w0 is None:
                    ps.append(_half(wt[m1, 320 + a - r0:320 + b - r0, :], c))
                else:
                    ps.append(_half(wt[m1, pl.ds(160 * c + w0 + 5 * (a - r0), b - a, stride=5), :], h))
            res.append(jnp.concatenate(ps, axis=0))
        return res

    def prep1(j):
        cols = pl.ds(j * 128, 128)
        wn[0, cols, :] = pltpu.bitcast(wraw[0:256, cols], U32).T
        wn[1, cols, :] = pltpu.bitcast(wraw[256:512, cols], U32).T
        wn[2, cols, 0:80] = pltpu.bitcast(wraw[512:672, cols], U32).T

    def prep2(m1):
        wt[m1, 0:128, :] = wn[0, pl.ds(m1, 128, stride=16), :].T
        wt[m1, 128:256, :] = wn[1, pl.ds(m1, 128, stride=16), :].T
        wt[m1, 256:336, :] = wn[2, pl.ds(m1, 128, stride=16), :].T[0:80]

    def fwd_pass(rows, side):
        lo, hi = rows

        def fn():
            for m1 in range(16):
                _spread(side, m1)
                k1, k2, k3 = [_dot_t(tb[m1, lo:hi, 128 * i:128 * (i + 1)], gmat(m1, i)) for i in range(3)]
                tp[m1, lo:hi, 0:128] = k1 - k3
                tp[m1, lo:hi, 128:256] = k1 + k2
        return fn

    def inv_pass(rows, side, pre=()):
        lo, hi = rows

        def fn():
            for m1 in range(16):
                if m1 in pre:
                    prep2(m1)
                xr, xi = tp[m1, lo:hi, 0:128], tp[m1, lo:hi, 128:256]
                wr_, wi_ = load_wt(m1, lo, hi)
                zr = xr * wr_ - xi * wi_
                zi = xr * wi_ + xi * wr_
                q1, q2, q3 = [_dot(z.astype(BF16), gmat(m1, i)) for i, z in enumerate((zr + zi, zi, zr))]
                tp[m1, lo:hi, 0:128] = q1 + q2
                tp[m1, lo:hi, 128:256] = q1 - q3
                _spread(side, m1)
        return fn

    A, B = (0, SPLIT), (SPLIT, R)
    rf_a, rf_b = [(rf, g) for g in _groups(*A)], [(rf, g) for g in _groups(*B)]

    def spectral_head_first():
        block(_run_all(rf_a))
        for cp in w_half[0]:
            cp.wait()
        for cp in misc_copies:
            cp.start()
        w1_copy(0).start()
        wraw[640:672, :] = jnp.concatenate(
            [wnyq[0].astype(F32), wnyq[1].astype(F32), jnp.zeros((30, S), F32)], axis=0).astype(BF16)
        block(fwd_pass(A, _merge(rf_b, [(prep1, j) for j in range(8)])))
        for cp in w_half[1]:
            cp.wait()
        w1_copy(1).start()
        block(fwd_pass(B, [(prep1, j) for j in range(8, 16)] + [(prep2, m) for m in range(5)]))
        block(inv_pass(A, [], range(5, 16)))
        w1_copy(2).start()
        for cp in misc_copies:
            cp.wait()
        w1_copy(0).wait()
        b1f[...] = b1_ref[...].reshape(1, F).astype(F32)
        b2f[...] = b2_ref[...].reshape(1, S).astype(F32)

    def spectral_head_second():
        block(_run_all(_merge(rf_a, [(dft_late, b) for b in range(16)])))
        block(fwd_pass(A, rf_b))

        def rest():
            fwd_pass(B, [])()
            inv_pass(A, [])()
        block(rest)

    def inv_dot(t, cols):
        return _dot(_bf(inv_ref[64 * t:64 * (t + 1), :]), _bf(yb[64 * t:64 * (t + 1), cols]))

    def inv_early(blk):
        cols = pl.ds(128 * blk, 128)
        for t in range(EARLY):
            vraw[128 * t:128 * (t + 1), cols] = inv_dot(t, cols)

    def inv_dots(blk):
        return [None if t < EARLY else inv_dot(t, pl.ds(128 * blk, 128)) for t in range(5)]

    def where(blk):
        j = blk // 2
        return (xa, xb)[j % 2], pl.ds((j // 2) * CH + 128 * (blk % 2), 128), pl.ds(128 * blk, 128)

    def inv_post(blk, v):
        buf, lc, gc = where(blk)
        shift = st[1:2, gc] + _half(yb[0:1, gc], 0) * _DC_SCALE
        st[0:1, gc] = st[0:1, gc] + shift

        def get(t, r0):
            if t < EARLY:
                return vraw[128 * t + r0:128 * t + r0 + 8, gc]
            return v[t][r0:r0 + 8]

        def iradix5(v0, v1r, v1i, v2r, v2i):
            t1 = v1r + v2r
            m = v0 - 0.25 * t1
            n = _C5 * (v1r - v2r)
            a, b = m + n, m - n
            cc = v1i + _RHO * v2i
            dd = _RHO * v1i - v2i
            return v0 + t1, a - cc, b - dd, b + dd, a + cc

        acc = None
        for sl in range(8):
            lo, hi = 8 * sl, 64 + 8 * sl
            ys = iradix5(get(0, lo) - shift, get(1, lo), get(1, hi), get(2, lo), get(2, hi))
            yd = iradix5(get(0, hi), get(3, lo), get(3, hi), get(4, lo), get(4, hi))
            for (pa, pb), a, b in zip(_PAIRS, ys, yd):
                for p, y in ((pa, a + b), (pb, a - b)):
                    rows = slice(64 * p + lo, 64 * p + lo + 8)
                    xn = buf[rows, lc] + y
                    buf[rows, lc] = xn
                    acc = xn * xn if acc is None else acc + xn * xn
        var = jnp.sum(acc, axis=0, keepdims=True) * (1.0 / D)
        r1 = lax.rsqrt(var + EPS)
        return r1 * lax.rsqrt(var * r1 * r1 + EPS)

    def inv_norm(blk, rr):
        buf, lc, gc = where(blk)
        for sl in range(20):
            hb[16 * sl:16 * (sl + 1), gc] = _pk(buf[32 * sl:32 * (sl + 1), lc] * rr)

    def col_inv_up():
        def up(t):
            kc = pl.ds(t * CH, CH)
            d = _dot_t(w1[F0:F, kc], _bf(hb[:, kc]))
            if t == 0:
                uat[...] = d
            else:
                uat[...] += d

        v = inv_dots(0)
        scale = {}
        done = 0
        for blk in range(17):
            if blk < 16:
                vn = inv_dots(blk + 1) if blk + 1 < 16 else None
                scale[blk] = inv_post(blk, v)
                v = vn
            if blk >= 1:
                inv_norm(blk - 1, scale[blk - 1])
            while 2 * done + 4 <= blk:
                up(done)
                done += 1
        for t in range(done, NCH):
            up(t)

    def mlp_up(l):
        def body(j, c):
            @pl.when(l == 0)
            def _():
                w1_copy(j + 1).wait()

            off = jnp.minimum(j * 384, D - 384)
            for i in range(UN // 256):
                cols = _cols(j * UN + 256 * i, 256)
                u = _dot_t(_bf(hb[:, 0:S]), w1[cols, 0:S]) + b1f[:, cols]
                gb[:, cols] = _pk(_gelu(u))
                if i == 0:
                    u = uat[:, pl.ds(pl.multiple_of(off, 128), 384)].T
                    gb[pl.ds(pl.multiple_of(off // 2, 64), 192), F0:F] = _pk(_gelu(u + b1f[:, F0:F]))
            return c
        lax.fori_loop(0, NU, body, 0)

    def mlp_down_mid():
        def step(cur, loff, goff, prev, ploff, pgoff, slot):
            lc, gc = _cols(loff, CH), _cols(goff, CH)
            col_pre(prev, ploff, pgoff, slot, CH, LATE)
            acc = row0 = None
            for b in range(2):
                y = _dot(_bf(gb[160 * b:160 * (b + 1), :]), w2[:, gc])
                if b == 0:
                    row0 = cur[0:1, lc] + y[0:1]
                for sl in range(20):
                    rows = slice(320 * b + 16 * sl, 320 * b + 16 * (sl + 1))
                    xn = cur[rows, lc] + (y[16 * sl:16 * (sl + 1)] - row0)
                    cur[rows, lc] = xn
                    acc = _acc_stats(acc, xn)
                if b == 0:
                    col_dft(pgoff, slot, LATE)
                    col_dft(pgoff + 128, slot + 1, LATE)
            dlt, var = _fin_stats(acc)
            st[0:1, gc] = st[0:1, gc] + row0 + b2f[:, gc]
            st[1:2, gc] = dlt
            st[2:3, gc] = var

        def body(i, c):
            ip = (i + 3) % 4
            step(xa, i * CH, 2 * i * CH, xb, ip * CH, (2 * ip + 1) * CH, 0)
            step(xb, i * CH, (2 * i + 1) * CH, xa, i * CH, 2 * i * CH, 2)
            return c
        lax.fori_loop(0, NCH // 2, body, 0)
        col_fwd(xb, 3 * CH, 7 * CH, 0, LATE)

    def mlp_down_last():
        def step(cur, loff, j):
            y = _dot(_bf(gb[...]), w2[:, _cols(j * CH, CH)])
            for h in range(2):
                gc = _cols(j * CH + 128 * h, 128)
                xn = (cur[:, _cols(loff + 128 * h, 128)] + y[:, 128 * h:128 * (h + 1)]
                      + (st[0:1, gc] + b2f[:, gc]))
                ost[gc, :] = xn.T.astype(BF16)
                o_copy(2 * j + h).start()

        def body(i, c):
            step(xa, i * CH, 2 * i)
            step(xb, i * CH, 2 * i + 1)
            return c
        lax.fori_loop(0, NCH // 2, body, 0)

    def load_chunk(j):
        buf, lc, gc = (xa, xb)[j % 2], pl.ds((j // 2) * CH, CH), pl.ds(j * CH, CH)
        xt = xin[gc, :].astype(F32).T
        pilot = xt[0:1]
        acc = None
        for sl in range(40):
            rows = slice(16 * sl, 16 * (sl + 1))
            xn = xt[rows] - pilot
            buf[rows, lc] = xn
            acc = _acc_stats(acc, xn)
        dlt, var = _fin_stats(acc)
        st[0:1, gc] = pilot
        st[1:2, gc] = dlt
        st[2:3, gc] = var

    def first_fwd(j):
        col_fwd((xa, xb)[j % 2], (j // 2) * CH, j * CH, 2 * (j % 2), 5)

    ft_copy.wait()
    for m1 in range(16):
        gen_g(m1)
    for j in range(NCH):
        x_copy(j).wait()
        if j == 1:
            fwd_copy.wait()
        if j in (5, 7):
            for cp in w_half[j // 6]:
                cp.start()
        block(_run_all(([(first_fwd, j - 1)] if j else []) + [(load_chunk, j)]))
    block(lambda: first_fwd(NCH - 1))

    def layer(l, c):
        pl.when(l == 0)(spectral_head_first)
        pl.when(l == 1)(spectral_head_second)
        block(inv_pass(B, [(ri, g) for g in _groups(*A)]))
        block(_run_all(_merge([(ri, g) for g in _groups(*B)], [(inv_early, b) for b in range(16)])))
        col_inv_up()

        @pl.when(l == 0)
        def _():
            w2_copy.start()

        mlp_up(l)

        @pl.when(l == 0)
        def _():
            w2_copy.wait()
            mlp_down_mid()

        pl.when(l == 1)(mlp_down_last)
        return c

    lax.fori_loop(0, 2, layer, 0)
    pltpu.make_async_copy(ost, out_hbm, sem_o.at[0]).wait()


@jax.jit
def pallas_interleave_layers__spectral_gfnet__mixer_token_mlp__prompt_kernel(A_x, A_w_r, A_w_i, B_x, B_w1, B_b1, B_w2, B_b2):
    del B_x
    fwd, inv, ft = _tables()
    hbm = pl.BlockSpec(memory_space=pltpu.HBM)
    out = pl.pallas_call(
        _kernel,
        out_shape=jax.ShapeDtypeStruct((S, D), BF16),
        in_specs=[hbm] * 10,
        out_specs=hbm,
        scratch_shapes=[
            pltpu.VMEM((S, D), BF16),
            pltpu.VMEM((672, S), BF16),
            pltpu.VMEM((2, 1, S), BF16),
            pltpu.VMEM((3, S, 128), U32),
            pltpu.VMEM((F, S + PAD), BF16),
            pltpu.VMEM((F, S + PAD), BF16),
            pltpu.VMEM((F,), BF16),
            pltpu.VMEM((S,), BF16),
            pltpu.VMEM(fwd.shape, U32),
            pltpu.VMEM(inv.shape, U32),
            pltpu.VMEM(ft.shape, F32),
            pltpu.VMEM((1, F), F32),
            pltpu.VMEM((1, S), F32),
            pltpu.VMEM((8, S), F32),
            pltpu.VMEM((D, S // 2 + PAD), F32),
            pltpu.VMEM((D, S // 2 + PAD), F32),
            pltpu.VMEM((320, 512), U32),
            pltpu.VMEM((64 * (5 - LATE), S + PAD), U32),
            pltpu.VMEM((R, S), F32),
            pltpu.VMEM((R, S), F32),
            pltpu.VMEM((16, R, 384), BF16),
            pltpu.VMEM((16, R, 256), F32),
            pltpu.VMEM((D // 2, S + PAD), U32),
            pltpu.VMEM((D // 2, S + PAD), U32),
            pltpu.VMEM((D // 2, F), U32),
            pltpu.VMEM((128 * EARLY, S + PAD), F32),
            pltpu.VMEM((F - F0, D), F32),
            pltpu.VMEM((16, R, 128), U32),
            pltpu.VMEM((64, 48 * 128), U32),
            pltpu.VMEM((S, D), BF16),
            pltpu.SMEM((1,), jnp.int32),
            pltpu.SemaphoreType.DMA((NCH,)),
            pltpu.SemaphoreType.DMA((6,)),
            pltpu.SemaphoreType.DMA((NU + 2,)),
            pltpu.SemaphoreType.DMA((1,)),
            pltpu.SemaphoreType.DMA((5,)),
        ],
        compiler_params=pltpu.CompilerParams(
            vmem_limit_bytes=110 * 1024 * 1024,
            disable_bounds_checks=True,
            disable_semaphore_checks=True),
    )(A_x.reshape(S, D), A_w_r.T, A_w_i.T, B_w1.T, B_b1, B_w2, B_b2,
      jnp.asarray(fwd), jnp.asarray(inv), jnp.asarray(ft))
    return out.reshape(1, S, D)
```

```python
import numpy as np
import jax
import jax.numpy as jnp
from jax import lax
import jax.experimental.pallas as pl
import jax.experimental.pallas.tpu as pltpu

S, D, F = 2048, 640, 1728
R = 336
CH = 256
NCH = S // CH
PAD = 128
EPS = 1e-5
F32 = jnp.float32
BF16 = jnp.bfloat16
U32 = jnp.uint32

SPLIT = 176
LATE = 3
EARLY = 2
F0 = 1536
NU = 2
WP = 24
UN = F0 // NU
W1_PIECES = ((F0, F - F0),) + tuple((UN * i, UN) for i in range(NU))

_S1 = float(np.sin(2 * np.pi / 5))
_S2 = float(np.sin(4 * np.pi / 5))
_C5 = float((np.cos(2 * np.pi / 5) - np.cos(4 * np.pi / 5)) / 2)
_RHO = _S2 / _S1
_RH = float(np.sqrt(0.5))
_TILE_CLASS = ((4, -1), (2, 1), (1, 1), (3, -1))
_PAIRS = ((0, 5), (2, 7), (4, 9), (6, 1), (8, 3))

_PIECES = []
for _k in (0, 5, None) + tuple(v for c, _ in _TILE_CLASS for v in (c, 10 - c)):
    _r0 = _PIECES[-1][0] + _PIECES[-1][1] if _PIECES else 0
    _PIECES.append((_r0, 16, None, None) if _k is None else (_r0, 32, _k // 2, _k % 2))


def _pack_rows(a):
    u = np.ascontiguousarray(a, np.float32).view(np.uint32)
    u = (u + 0x7FFF + ((u >> 16) & 1)) >> 16
    return (u[0::2] | (u[1::2] << 16)).astype(np.uint32)


_DC_SCALE = float((_pack_rows(np.full((2, 1), 1.0 / (D * S))) << 16).view(np.float32)[0, 0])


def _tables():
    q = np.arange(64)
    j10 = 10 * np.arange(32)

    def cs(k):
        th = 2 * np.pi * np.outer(k, q) / D
        return np.cos(th), np.sin(th)

    sc = 2.0 / (D * S)
    z = np.zeros((32, 64))
    c0, s0 = cs(j10)
    c5, s5 = cs(5 + j10)
    nyq = np.zeros((16, 128))
    nyq[0, :64] = cs(np.array([D // 2]))[0][0]
    m0 = np.block([[c0, z], [z, c5], [-s0, z], [z, -s5]])
    i0 = m0.T * sc
    i0[:, 0] *= 0.5
    i0[:, 64] = nyq[0] * 0.5 * sc
    fwd, inv = [nyq, m0], [i0]
    for c, sgn in _TILE_CLASS:
        cA, sA = cs(c + j10)
        cB, sB = cs(10 - c + j10)
        m = np.block([[cA, sA], [cB, -sB], [-sA, cA], [-sB, -cB]])
        scale = np.concatenate([np.ones(64), sgn * _S1 * np.ones(64)])
        fwd.append(m * np.concatenate([np.ones(64), -scale[64:]])[None, :])
        inv.append(m.T * sc * scale[:, None])
    kperm = np.arange(128).reshape(2, 8, 8).transpose(1, 0, 2).reshape(-1)
    b = np.arange(128)
    th = 2 * np.pi * np.outer(b, b) / 128
    tt = 2 * np.pi * np.outer(np.arange(16), b) / S
    ft = np.concatenate([np.cos(th), -np.sin(th), np.cos(tt), -np.sin(tt)])
    return (_pack_rows(np.concatenate(fwd)[:, kperm]), _pack_rows(np.concatenate(inv)[:, kperm]),
            ft.astype(np.float32))


def _bfly4(a, b, c, d):
    s0r, s0i = a[0] + c[0], a[1] + c[1]
    d0r, d0i = a[0] - c[0], a[1] - c[1]
    s1r, s1i = b[0] + d[0], b[1] + d[1]
    d1r, d1i = b[0] - d[0], b[1] - d[1]
    return ((s0r + s1r, s0i + s1i), (d0r + d1i, d0i - d1r),
            (s0r - s1r, s0i - s1i), (d0r - d1i, d0i + d1r))


def _tw16(z, e):
    r, i = z
    if e == 0:
        return z
    if e == 4:
        return (i, -r)
    if e == 2:
        return ((r + i) * _RH, (i - r) * _RH)
    if e == 6:
        return ((i - r) * _RH, (r + i) * (-_RH))
    c, s = float(np.cos(2 * np.pi * e / 16)), float(np.sin(2 * np.pi * e / 16))
    return (r * c + i * s, i * c - r * s)


def _dft16(x):
    t = []
    for a0 in range(4):
        o = _bfly4(x[a0], x[4 + a0], x[8 + a0], x[12 + a0])
        t.append([_tw16(o[r0], a0 * r0) for r0 in range(4)])
    out = [None] * 16
    for r0 in range(4):
        o = _bfly4(t[0][r0], t[1][r0], t[2][r0], t[3][r0])
        for r1 in range(4):
            out[r0 + 4 * r1] = o[r1]
    return out


def _dot(a, b):
    return jnp.dot(a, b, preferred_element_type=F32)


def _dot_t(a, b):
    return lax.dot_general(a, b, (((1,), (1,)), ((), ())), preferred_element_type=F32)


def _gelu(u):
    return 0.5 * u * (1.0 + jnp.tanh(0.7978845608028654 * (u + 0.044715 * (u * u * u))))


def _cols(off, width):
    if isinstance(off, int):
        return pl.ds(off, width)
    return pl.ds(pl.multiple_of(off, 128), width)


def _bf(u):
    return pltpu.bitcast(u, BF16)


def _pk(v):
    return pltpu.bitcast(v.astype(BF16), U32)


def _pk2(lo, hi):
    return _pk(jnp.concatenate([lo, hi], axis=0))


def _half(v, h):
    return pltpu.bitcast(v << 16 if h == 0 else v & jnp.uint32(0xFFFF0000), F32)


def _fold8(v):
    out = v[0:8]
    for i in range(1, v.shape[0] // 8):
        out = out + v[8 * i:8 * (i + 1)]
    return out


def _acc_stats(acc, xn):
    a1, a2 = _fold8(xn), _fold8(xn * xn)
    return (a1, a2) if acc is None else (acc[0] + a1, acc[1] + a2)


def _fin_stats(acc):
    dlt = jnp.sum(acc[0], axis=0, keepdims=True) * (1.0 / D)
    msq = jnp.sum(acc[1], axis=0, keepdims=True) * (1.0 / D)
    return dlt, jnp.maximum(msq - dlt * dlt, 0.0)


def _groups(lo, hi):
    return [g for g in range(lo // 8, hi // 8) if g != 9]


def _merge(a, b):
    keyed = ([((i + 0.5) / len(b), 0, w) for i, w in enumerate(b)]
             + [((i + 0.75) / len(a), 1, w) for i, w in enumerate(a)])
    return [w for _, _, w in sorted(keyed, key=lambda t: t[:2])]


def _run_all(work):
    def fn():
        for f, arg in work:
            f(arg)
    return fn


def _spread(work, m1):
    n = len(work)
    for fn, arg in work[(m1 * n) // 16:((m1 + 1) * n) // 16]:
        fn(arg)


def _kernel(x_hbm, wr_hbm, wi_hbm, w1_hbm, b1_hbm, w2_hbm, b2_hbm, fwd_hbm, inv_hbm, ft_hbm,
            out_hbm,
            xin, wraw, wnyq, wn, w1, w2, b1_ref, b2_ref, fwd_ref, inv_ref, ft_ref,
            b1f, b2f, st, xa, xb, ab, al, yr, yi, tb, tp, yb, hb, gb, vraw, uat, wt, g3, ost, flag,
            sem_x, sem_w, sem_m, sem_o, sem_c):

    def x_copy(j):
        return pltpu.make_async_copy(x_hbm.at[pl.ds(j * CH, CH), :], xin.at[pl.ds(j * CH, CH), :], sem_x.at[j])

    def o_copy(k):
        return pltpu.make_async_copy(ost.at[pl.ds(k * 128, 128), :], out_hbm.at[pl.ds(k * 128, 128), :],
                                     sem_o.at[0])

    w_half = [[], []]
    for ri, src in enumerate((wr_hbm, wi_hbm)):
        for h in range(2):
            w_half[h].append(pltpu.make_async_copy(
                src.at[pl.ds(0, 320), pl.ds(1024 * h, 1024)],
                wraw.at[pl.ds(320 * ri, 320), pl.ds(1024 * h, 1024)], sem_w.at[3 * ri + h]))
        w_half[0].append(pltpu.make_async_copy(src.at[pl.ds(320, 1), :], wnyq.at[ri], sem_w.at[3 * ri + 2]))

    def w1_copy(i):
        if isinstance(i, int):
            rows = pl.ds(*W1_PIECES[i])
        else:
            rows = pl.ds(pl.multiple_of((i - 1) * UN, 128), UN)
        return pltpu.make_async_copy(w1_hbm.at[rows, :], w1.at[rows, pl.ds(0, S)], sem_m.at[i])

    w2_copy = pltpu.make_async_copy(w2_hbm, w2.at[:, pl.ds(0, S)], sem_m.at[NU + 1])
    fwd_copy = pltpu.make_async_copy(fwd_hbm, fwd_ref, sem_c.at[0])
    ft_copy = pltpu.make_async_copy(ft_hbm, ft_ref, sem_c.at[1])
    misc_copies = [pltpu.make_async_copy(a, b, sem_c.at[2 + i])
                   for i, (a, b) in enumerate(((inv_hbm, inv_ref), (b1_hbm, b1_ref), (b2_hbm, b2_ref)))]

    ft_copy.start()

    def start_x(j, c):
        x_copy(j).start()

        @pl.when(j == 0)
        def _():
            fwd_copy.start()
        return c
    lax.fori_loop(0, NCH, start_x, 0)

    flag[0] = 1
    yi[64:80, :] = jnp.zeros((16, S), F32)
    tb[:, 64:80, :] = jnp.zeros((16, 16, 384), BF16)
    wn[2, :, 80:128] = jnp.zeros((128 * WP, 48), U32)

    def block(fn):
        pl.when(flag[0] == 1)(fn)

    def col_pre(buf, loff, goff, slot, width, late):
        lc, gc, ac = _cols(loff, width), _cols(goff, width), pl.ds(128 * slot, width)
        r = lax.rsqrt(st[2:3, gc] + EPS)
        rc, rr, d10 = r * _C5, r * _RHO, st[1:2, gc] * r * 10.0

        def radix5(x0, x1, x2, x3, x4):
            t1, t2, t3, t4 = x1 + x4, x2 + x3, x1 - x4, x2 - x3
            u = (t1 + t2) * r
            x0 = x0 * r
            m = x0 - 0.25 * u
            n = (t1 - t2) * rc
            return x0 + u, m + n, t3 * r + t4 * rr, m - n, t3 * rr - t4 * r

        for sl in range(8):
            sm, df = [], []
            for pa, pb in _PAIRS:
                va = buf[64 * pa + 8 * sl:64 * pa + 8 * (sl + 1), lc]
                vb = buf[64 * pb + 8 * sl:64 * pb + 8 * (sl + 1), lc]
                sm.append(va + vb)
                df.append(va - vb)
            s0, s1r, s1i, s2r, s2i = radix5(*sm)
            d0, d1r, d1i, d2r, d2i = radix5(*df)
            for t, pair in enumerate(((s0 - d10, d0), (s1r, s1i), (s2r, s2i), (d1r, d1i), (d2r, d2i))):
                if t < late:
                    ab[64 * t + 8 * sl:64 * t + 8 * (sl + 1), ac] = _pk2(*pair)
                else:
                    al[64 * (t - LATE) + 8 * sl:64 * (t - LATE) + 8 * (sl + 1), gc] = _pk2(*pair)

    def dft_tile(t, cols, operand):
        o = _dot(_bf(fwd_ref[8 + 64 * t:72 + 64 * t, :]), _bf(operand))
        yr[16 + 64 * t:80 + 64 * t, cols] = o[0:64]
        yi[16 + 64 * t:80 + 64 * t, cols] = o[64:128]

    def col_dft(goff, slot, late):
        cols, ac = _cols(goff, 128), pl.ds(128 * slot, 128)
        o = _dot(_bf(fwd_ref[0:72, :]), _bf(ab[0:64, ac]))
        yr[64:80, cols] = o[0:16]
        yr[0:64, cols] = o[16:80]
        yi[0:64, cols] = o[80:144]
        for t in range(1, late):
            dft_tile(t, cols, ab[64 * t:64 * (t + 1), ac])

    def dft_late(blk):
        cols = pl.ds(128 * blk, 128)
        for t in range(LATE, 5):
            dft_tile(t, cols, al[64 * (t - LATE):64 * (t - LATE + 1), cols])

    def col_fwd(buf, loff, goff, slot, late):
        for h in range(2):
            col_pre(buf, loff + 128 * h, goff + 128 * h, slot + h, 128, late)
            col_dft(goff + 128 * h, slot + h, late)

    def rf(g):
        rows = pl.ds(g * 8, 8)
        o = _dft16([(yr[rows, 128 * a:128 * (a + 1)], yi[rows, 128 * a:128 * (a + 1)]) for a in range(16)])
        for m1 in range(16):
            tb[m1, rows, :] = jnp.concatenate([o[m1][0] + o[m1][1], o[m1][0], o[m1][1]], axis=1).astype(BF16)

    def idft(g):
        rows = pl.ds(g * 8, 8)
        o = _dft16([(tp[m1, rows, 128:256], tp[m1, rows, 0:128]) for m1 in range(16)])
        return [o[a][1] for a in range(16)], [o[a][0] for a in range(16)]

    def ri(g):
        if g == 8:
            return
        re, im = idft(g)
        if g == 0:
            ren, _ = idft(8)
            first = lax.broadcasted_iota(jnp.int32, (8, 128), 0) == 0
            im = [jnp.where(first, a, b) for a, b in zip(ren, im)]
        gg = g if g < 8 else g - 2
        for a in range(16):
            yb[pl.ds(8 * gg, 8), 128 * a:128 * (a + 1)] = _pk2(re[a], im[a])

    def gen_g(m1):
        tr, ti = ft_ref[256 + m1:257 + m1, :], ft_ref[272 + m1:273 + m1, :]
        fr, fi = ft_ref[0:128, :], ft_ref[128:256, :]
        gr = fr * tr - fi * ti
        gi = fr * ti + fi * tr
        g3[:, 384 * m1:384 * (m1 + 1)] = _pk(jnp.concatenate([gr, gi - gr, gr + gi], axis=1))

    def gmat(m1, i):
        return _bf(g3[:, 128 * (3 * m1 + i):128 * (3 * m1 + i + 1)])

    def load_wt(m1, lo, hi):
        res = []
        for c in range(2):
            ps = []
            for (r0, n, w0, h) in _PIECES:
                a, b = max(lo, r0), min(hi, r0 + n)
                if a >= b:
                    continue
                if w0 is None:
                    ps.append(_half(wt[m1, 320 + a - r0:320 + b - r0, :], c))
                else:
                    ps.append(_half(wt[m1, pl.ds(160 * c + w0 + 5 * (a - r0), b - a, stride=5), :], h))
            res.append(jnp.concatenate(ps, axis=0))
        return res

    def prep1(j):
        cols = pl.ds(j * 128, 128)
        for blk, (r0, r1) in enumerate(((0, 256), (256, 512), (512, 672))):
            v = pltpu.bitcast(wraw[r0:r1, cols], U32).T
            for t in range(8):
                wn[blk, pl.ds(WP * (8 * j + t), 16), 0:(r1 - r0) // 2] = v[16 * t:16 * (t + 1)]

    def prep2(m1):
        wt[m1, 0:128, :] = wn[0, pl.ds(m1, 128, stride=WP), :].T
        wt[m1, 128:256, :] = wn[1, pl.ds(m1, 128, stride=WP), :].T
        wt[m1, 256:336, :] = wn[2, pl.ds(m1, 128, stride=WP), :].T[0:80]

    def fwd_pass(rows, side):
        lo, hi = rows

        def fn():
            for m1 in range(16):
                _spread(side, m1)
                k1, k2, k3 = [_dot_t(tb[m1, lo:hi, 128 * i:128 * (i + 1)], gmat(m1, i)) for i in range(3)]
                tp[m1, lo:hi, 0:128] = k1 - k3
                tp[m1, lo:hi, 128:256] = k1 + k2
        return fn

    def inv_pass(rows, side, pre=()):
        lo, hi = rows

        def fn():
            for m1 in range(16):
                if m1 in pre:
                    prep2(m1)
                xr, xi = tp[m1, lo:hi, 0:128], tp[m1, lo:hi, 128:256]
                wr_, wi_ = load_wt(m1, lo, hi)
                zr = xr * wr_ - xi * wi_
                zi = xr * wi_ + xi * wr_
                q1, q2, q3 = [_dot(z.astype(BF16), gmat(m1, i)) for i, z in enumerate((zr + zi, zi, zr))]
                tp[m1, lo:hi, 0:128] = q1 + q2
                tp[m1, lo:hi, 128:256] = q1 - q3
                _spread(side, m1)
        return fn

    A, B = (0, SPLIT), (SPLIT, R)
    rf_a, rf_b = [(rf, g) for g in _groups(*A)], [(rf, g) for g in _groups(*B)]

    def spectral_head_first():
        block(_run_all(rf_a))
        for cp in w_half[0]:
            cp.wait()
        for cp in misc_copies:
            cp.start()
        w1_copy(0).start()
        wraw[640:672, :] = jnp.concatenate(
            [wnyq[0].astype(F32), wnyq[1].astype(F32), jnp.zeros((30, S), F32)], axis=0).astype(BF16)
        block(fwd_pass(A, _merge(rf_b, [(prep1, j) for j in range(8)])))
        for cp in w_half[1]:
            cp.wait()
        w1_copy(1).start()
        block(fwd_pass(B, [(prep1, j) for j in range(8, 16)] + [(prep2, m) for m in range(5)]))
        block(inv_pass(A, [], range(5, 16)))
        w1_copy(2).start()
        for cp in misc_copies:
            cp.wait()
        w1_copy(0).wait()
        b1f[...] = b1_ref[...].reshape(1, F).astype(F32)
        b2f[...] = b2_ref[...].reshape(1, S).astype(F32)

    def spectral_head_second():
        block(_run_all(_merge(rf_a, [(dft_late, b) for b in range(16)])))
        block(fwd_pass(A, rf_b))

        def rest():
            fwd_pass(B, [])()
            inv_pass(A, [])()
        block(rest)

    def inv_dot(t, cols):
        return _dot(_bf(inv_ref[64 * t:64 * (t + 1), :]), _bf(yb[64 * t:64 * (t + 1), cols]))

    def inv_early(blk):
        cols = pl.ds(128 * blk, 128)
        for t in range(EARLY):
            vraw[128 * t:128 * (t + 1), cols] = inv_dot(t, cols)

    def inv_dots(blk):
        return [None if t < EARLY else inv_dot(t, pl.ds(128 * blk, 128)) for t in range(5)]

    def where(blk):
        j = blk // 2
        return (xa, xb)[j % 2], pl.ds((j // 2) * CH + 128 * (blk % 2), 128), pl.ds(128 * blk, 128)

    def inv_post(blk, v):
        buf, lc, gc = where(blk)
        shift = st[1:2, gc] + _half(yb[0:1, gc], 0) * _DC_SCALE
        st[0:1, gc] = st[0:1, gc] + shift

        def get(t, r0):
            if t < EARLY:
                return vraw[128 * t + r0:128 * t + r0 + 8, gc]
            return v[t][r0:r0 + 8]

        def iradix5(v0, v1r, v1i, v2r, v2i):
            t1 = v1r + v2r
            m = v0 - 0.25 * t1
            n = _C5 * (v1r - v2r)
            a, b = m + n, m - n
            cc = v1i + _RHO * v2i
            dd = _RHO * v1i - v2i
            return v0 + t1, a - cc, b - dd, b + dd, a + cc

        acc = None
        for sl in range(8):
            lo, hi = 8 * sl, 64 + 8 * sl
            ys = iradix5(get(0, lo) - shift, get(1, lo), get(1, hi), get(2, lo), get(2, hi))
            yd = iradix5(get(0, hi), get(3, lo), get(3, hi), get(4, lo), get(4, hi))
            for (pa, pb), a, b in zip(_PAIRS, ys, yd):
                for p, y in ((pa, a + b), (pb, a - b)):
                    rows = slice(64 * p + lo, 64 * p + lo + 8)
                    xn = buf[rows, lc] + y
                    buf[rows, lc] = xn
                    acc = xn * xn if acc is None else acc + xn * xn
        var = jnp.sum(acc, axis=0, keepdims=True) * (1.0 / D)
        r1 = lax.rsqrt(var + EPS)
        return r1 * lax.rsqrt(var * r1 * r1 + EPS)

    def inv_norm(blk, rr):
        buf, lc, gc = where(blk)
        for sl in range(20):
            hb[16 * sl:16 * (sl + 1), gc] = _pk(buf[32 * sl:32 * (sl + 1), lc] * rr)

    def col_inv_up():
        def up(t):
            kc = pl.ds(t * CH, CH)
            d = _dot_t(w1[F0:F, kc], _bf(hb[:, kc]))
            if t == 0:
                uat[...] = d
            else:
                uat[...] += d

        v = inv_dots(0)
        scale = {}
        done = 0
        for blk in range(17):
            if blk < 16:
                vn = inv_dots(blk + 1) if blk + 1 < 16 else None
                scale[blk] = inv_post(blk, v)
                v = vn
            if blk >= 1:
                inv_norm(blk - 1, scale[blk - 1])
            while 2 * done + 4 <= blk:
                up(done)
                done += 1
        for t in range(done, NCH):
            up(t)

    def mlp_up(l):
        def body(j, c):
            @pl.when(l == 0)
            def _():
                w1_copy(j + 1).wait()

            off = jnp.minimum(j * 384, D - 384)
            for i in range(UN // 256):
                cols = _cols(j * UN + 256 * i, 256)
                u = _dot_t(_bf(hb[:, 0:S]), w1[cols, 0:S]) + b1f[:, cols]
                gb[:, cols] = _pk(_gelu(u))
                if i == 0:
                    u = uat[:, pl.ds(pl.multiple_of(off, 128), 384)].T
                    gb[pl.ds(pl.multiple_of(off // 2, 64), 192), F0:F] = _pk(_gelu(u + b1f[:, F0:F]))
            return c
        lax.fori_loop(0, NU, body, 0)

    def mlp_down_mid():
        def step(cur, loff, goff, prev, ploff, pgoff, slot):
            lc, gc = _cols(loff, CH), _cols(goff, CH)
            acc = row0 = None
            for b in range(2):
                y = _dot(_bf(gb[160 * b:160 * (b + 1), :]), w2[:, gc])
                if b == 0:
                    row0 = cur[0:1, lc] + y[0:1]
                for sl in range(20):
                    rows = slice(320 * b + 16 * sl, 320 * b + 16 * (sl + 1))
                    xn = cur[rows, lc] + (y[16 * sl:16 * (sl + 1)] - row0)
                    cur[rows, lc] = xn
                    acc = _acc_stats(acc, xn)
                if b == 0:
                    col_pre(prev, ploff, pgoff, slot, CH, LATE)
            col_dft(pgoff, slot, LATE)
            col_dft(pgoff + 128, slot + 1, LATE)
            dlt, var = _fin_stats(acc)
            st[0:1, gc] = st[0:1, gc] + row0 + b2f[:, gc]
            st[1:2, gc] = dlt
            st[2:3, gc] = var

        def body(i, c):
            ip = (i + 3) % 4
            step(xa, i * CH, 2 * i * CH, xb, ip * CH, (2 * ip + 1) * CH, 0)
            step(xb, i * CH, (2 * i + 1) * CH, xa, i * CH, 2 * i * CH, 2)
            return c
        lax.fori_loop(0, NCH // 2, body, 0)
        col_fwd(xb, 3 * CH, 7 * CH, 0, LATE)

    def mlp_down_last():
        def step(cur, loff, j):
            y = _dot(_bf(gb[...]), w2[:, _cols(j * CH, CH)])
            for h in range(2):
                gc = _cols(j * CH + 128 * h, 128)
                xn = (cur[:, _cols(loff + 128 * h, 128)] + y[:, 128 * h:128 * (h + 1)]
                      + (st[0:1, gc] + b2f[:, gc]))
                ost[gc, :] = xn.T.astype(BF16)
                o_copy(2 * j + h).start()

        def body(i, c):
            step(xa, i * CH, 2 * i)
            step(xb, i * CH, 2 * i + 1)
            return c
        lax.fori_loop(0, NCH // 2, body, 0)

    def load_chunk(j):
        buf, lc, gc = (xa, xb)[j % 2], pl.ds((j // 2) * CH, CH), pl.ds(j * CH, CH)
        xt = xin[gc, :].astype(F32).T
        pilot = xt[0:1]
        acc = None
        for sl in range(40):
            rows = slice(16 * sl, 16 * (sl + 1))
            xn = xt[rows] - pilot
            buf[rows, lc] = xn
            acc = _acc_stats(acc, xn)
        dlt, var = _fin_stats(acc)
        st[0:1, gc] = pilot
        st[1:2, gc] = dlt
        st[2:3, gc] = var

    def first_fwd(j):
        col_fwd((xa, xb)[j % 2], (j // 2) * CH, j * CH, 2 * (j % 2), 5)

    ft_copy.wait()
    for m1 in range(16):
        gen_g(m1)
    for j in range(NCH):
        x_copy(j).wait()
        if j == 1:
            fwd_copy.wait()
        if j in (5, 7):
            for cp in w_half[j // 6]:
                cp.start()
        block(_run_all(([(first_fwd, j - 1)] if j else []) + [(load_chunk, j)]))
    block(lambda: first_fwd(NCH - 1))

    def layer(l, c):
        pl.when(l == 0)(spectral_head_first)
        pl.when(l == 1)(spectral_head_second)
        block(inv_pass(B, [(ri, g) for g in _groups(*A)]))
        block(_run_all(_merge([(ri, g) for g in _groups(*B)], [(inv_early, b) for b in range(16)])))
        col_inv_up()

        @pl.when(l == 0)
        def _():
            w2_copy.start()

        mlp_up(l)

        @pl.when(l == 0)
        def _():
            w2_copy.wait()
            mlp_down_mid()

        pl.when(l == 1)(mlp_down_last)
        return c

    lax.fori_loop(0, 2, layer, 0)
    pltpu.make_async_copy(ost, out_hbm, sem_o.at[0]).wait()


@jax.jit
def pallas_interleave_layers__spectral_gfnet__mixer_token_mlp__prompt_kernel(A_x, A_w_r, A_w_i, B_x, B_w1, B_b1, B_w2, B_b2):
    del B_x
    fwd, inv, ft = _tables()
    hbm = pl.BlockSpec(memory_space=pltpu.HBM)
    out = pl.pallas_call(
        _kernel,
        out_shape=jax.ShapeDtypeStruct((S, D), BF16),
        in_specs=[hbm] * 10,
        out_specs=hbm,
        scratch_shapes=[
            pltpu.VMEM((S, D), BF16),
            pltpu.VMEM((672, S), BF16),
            pltpu.VMEM((2, 1, S), BF16),
            pltpu.VMEM((3, 128 * WP, 128), U32),
            pltpu.VMEM((F, S + PAD), BF16),
            pltpu.VMEM((F, S + PAD), BF16),
            pltpu.VMEM((F,), BF16),
            pltpu.VMEM((S,), BF16),
            pltpu.VMEM(fwd.shape, U32),
            pltpu.VMEM(inv.shape, U32),
            pltpu.VMEM(ft.shape, F32),
            pltpu.VMEM((1, F), F32),
            pltpu.VMEM((1, S), F32),
            pltpu.VMEM((8, S), F32),
            pltpu.VMEM((D, S // 2 + PAD), F32),
            pltpu.VMEM((D, S // 2 + PAD), F32),
            pltpu.VMEM((320, 512), U32),
            pltpu.VMEM((64 * (5 - LATE), S + PAD), U32),
            pltpu.VMEM((R, S), F32),
            pltpu.VMEM((R, S), F32),
            pltpu.VMEM((16, R, 384), BF16),
            pltpu.VMEM((16, R, 256), F32),
            pltpu.VMEM((D // 2, S + PAD), U32),
            pltpu.VMEM((D // 2, S + PAD), U32),
            pltpu.VMEM((D // 2, F), U32),
            pltpu.VMEM((128 * EARLY, S + PAD), F32),
            pltpu.VMEM((F - F0, D), F32),
            pltpu.VMEM((16, R, 128), U32),
            pltpu.VMEM((64, 48 * 128), U32),
            pltpu.VMEM((S, D), BF16),
            pltpu.SMEM((1,), jnp.int32),
            pltpu.SemaphoreType.DMA((NCH,)),
            pltpu.SemaphoreType.DMA((6,)),
            pltpu.SemaphoreType.DMA((NU + 2,)),
            pltpu.SemaphoreType.DMA((1,)),
            pltpu.SemaphoreType.DMA((5,)),
        ],
        compiler_params=pltpu.CompilerParams(
            vmem_limit_bytes=110 * 1024 * 1024,
            disable_bounds_checks=True,
            disable_semaphore_checks=True),
    )(A_x.reshape(S, D), A_w_r.T, A_w_i.T, B_w1.T, B_b1, B_w2, B_b2,
      jnp.asarray(fwd), jnp.asarray(inv), jnp.asarray(ft))
    return out.reshape(1, S, D)
```

```python
import numpy as np
import jax
import jax.numpy as jnp
from jax import lax
import jax.experimental.pallas as pl
import jax.experimental.pallas.tpu as pltpu

S, D, F = 2048, 640, 1728
R = 336
CH = 256
NCH = S // CH
PAD = 128
EPS = 1e-5
F32 = jnp.float32
BF16 = jnp.bfloat16
U32 = jnp.uint32

SPLIT = 176
LATE = 3
EARLY = 2
F0 = 1536
NU = 2
WP = 24
UN = F0 // NU
W1_PIECES = ((F0, F - F0),) + tuple((UN * i, UN) for i in range(NU))

_S1 = float(np.sin(2 * np.pi / 5))
_S2 = float(np.sin(4 * np.pi / 5))
_C5 = float((np.cos(2 * np.pi / 5) - np.cos(4 * np.pi / 5)) / 2)
_RHO = _S2 / _S1
_RH = float(np.sqrt(0.5))
_TILE_CLASS = ((4, -1), (2, 1), (1, 1), (3, -1))
_PAIRS = ((0, 5), (2, 7), (4, 9), (6, 1), (8, 3))

_PIECES = []
for _k in (0, 5, None) + tuple(v for c, _ in _TILE_CLASS for v in (c, 10 - c)):
    _r0 = _PIECES[-1][0] + _PIECES[-1][1] if _PIECES else 0
    _PIECES.append((_r0, 16, None, None) if _k is None else (_r0, 32, _k // 2, _k % 2))


def _pack_rows(a):
    u = np.ascontiguousarray(a, np.float32).view(np.uint32)
    u = (u + 0x7FFF + ((u >> 16) & 1)) >> 16
    return (u[0::2] | (u[1::2] << 16)).astype(np.uint32)


_DC_SCALE = float((_pack_rows(np.full((2, 1), 1.0 / (D * S))) << 16).view(np.float32)[0, 0])


def _tables():
    q = np.arange(64)
    j10 = 10 * np.arange(32)

    def cs(k):
        th = 2 * np.pi * np.outer(k, q) / D
        return np.cos(th), np.sin(th)

    sc = 2.0 / (D * S)
    z = np.zeros((32, 64))
    c0, s0 = cs(j10)
    c5, s5 = cs(5 + j10)
    nyq = np.zeros((16, 128))
    nyq[0, :64] = cs(np.array([D // 2]))[0][0]
    m0 = np.block([[c0, z], [z, c5], [-s0, z], [z, -s5]])
    i0 = m0.T * sc
    i0[:, 0] *= 0.5
    i0[:, 64] = nyq[0] * 0.5 * sc
    fwd, inv = [nyq, m0], [i0]
    for c, sgn in _TILE_CLASS:
        cA, sA = cs(c + j10)
        cB, sB = cs(10 - c + j10)
        m = np.block([[cA, sA], [cB, -sB], [-sA, cA], [-sB, -cB]])
        scale = np.concatenate([np.ones(64), sgn * _S1 * np.ones(64)])
        fwd.append(m * np.concatenate([np.ones(64), -scale[64:]])[None, :])
        inv.append(m.T * sc * scale[:, None])
    kperm = np.arange(128).reshape(2, 8, 8).transpose(1, 0, 2).reshape(-1)
    b = np.arange(128)
    th = 2 * np.pi * np.outer(b, b) / 128
    tt = 2 * np.pi * np.outer(np.arange(16), b) / S
    ft = np.concatenate([np.cos(th), -np.sin(th), np.cos(tt), -np.sin(tt)])
    return (_pack_rows(np.concatenate(fwd)[:, kperm]), _pack_rows(np.concatenate(inv)[:, kperm]),
            ft.astype(np.float32))


def _bfly4(a, b, c, d):
    s0r, s0i = a[0] + c[0], a[1] + c[1]
    d0r, d0i = a[0] - c[0], a[1] - c[1]
    s1r, s1i = b[0] + d[0], b[1] + d[1]
    d1r, d1i = b[0] - d[0], b[1] - d[1]
    return ((s0r + s1r, s0i + s1i), (d0r + d1i, d0i - d1r),
            (s0r - s1r, s0i - s1i), (d0r - d1i, d0i + d1r))


def _tw16(z, e):
    r, i = z
    if e == 0:
        return z
    if e == 4:
        return (i, -r)
    if e == 2:
        return ((r + i) * _RH, (i - r) * _RH)
    if e == 6:
        return ((i - r) * _RH, (r + i) * (-_RH))
    c, s = float(np.cos(2 * np.pi * e / 16)), float(np.sin(2 * np.pi * e / 16))
    return (r * c + i * s, i * c - r * s)


def _dft16(x):
    t = []
    for a0 in range(4):
        o = _bfly4(x[a0], x[4 + a0], x[8 + a0], x[12 + a0])
        t.append([_tw16(o[r0], a0 * r0) for r0 in range(4)])
    out = [None] * 16
    for r0 in range(4):
        o = _bfly4(t[0][r0], t[1][r0], t[2][r0], t[3][r0])
        for r1 in range(4):
            out[r0 + 4 * r1] = o[r1]
    return out


def _dot(a, b):
    return jnp.dot(a, b, preferred_element_type=F32)


def _dot_t(a, b):
    return lax.dot_general(a, b, (((1,), (1,)), ((), ())), preferred_element_type=F32)


def _gelu(u):
    return 0.5 * u * (1.0 + jnp.tanh(0.7978845608028654 * (u + 0.044715 * (u * u * u))))


def _cols(off, width):
    if isinstance(off, int):
        return pl.ds(off, width)
    return pl.ds(pl.multiple_of(off, 128), width)


def _bf(u):
    return pltpu.bitcast(u, BF16)


def _pk(v):
    return pltpu.bitcast(v.astype(BF16), U32)


def _pk2(lo, hi):
    return _pk(jnp.concatenate([lo, hi], axis=0))


def _half(v, h):
    return pltpu.bitcast(v << 16 if h == 0 else v & jnp.uint32(0xFFFF0000), F32)


def _fold8(v):
    out = v[0:8]
    for i in range(1, v.shape[0] // 8):
        out = out + v[8 * i:8 * (i + 1)]
    return out


def _acc_stats(acc, xn):
    a1, a2 = _fold8(xn), _fold8(xn * xn)
    return (a1, a2) if acc is None else (acc[0] + a1, acc[1] + a2)


def _fin_stats(acc):
    dlt = jnp.sum(acc[0], axis=0, keepdims=True) * (1.0 / D)
    msq = jnp.sum(acc[1], axis=0, keepdims=True) * (1.0 / D)
    return dlt, jnp.maximum(msq - dlt * dlt, 0.0)


def _rows(r0, n):
    p = r0 + 8 * (r0 // 64)
    return slice(p, p + n)


def _groups(lo, hi):
    return [g for g in range(lo // 8, hi // 8) if g != 9]


def _merge(a, b):
    keyed = ([((i + 0.5) / len(b), 0, w) for i, w in enumerate(b)]
             + [((i + 0.75) / len(a), 1, w) for i, w in enumerate(a)])
    return [w for _, _, w in sorted(keyed, key=lambda t: t[:2])]


def _run_all(work):
    def fn():
        for f, arg in work:
            f(arg)
    return fn


def _spread(work, m1):
    n = len(work)
    for fn, arg in work[(m1 * n) // 16:((m1 + 1) * n) // 16]:
        fn(arg)


def _kernel(x_hbm, wr_hbm, wi_hbm, w1_hbm, b1_hbm, w2_hbm, b2_hbm, fwd_hbm, inv_hbm, ft_hbm,
            out_hbm,
            xin, wraw, wnyq, wn, w1, w2, b1_ref, b2_ref, fwd_ref, inv_ref, ft_ref,
            b1f, b2f, st, xa, xb, ab, al, yr, yi, tb, tp, yb, hb, gb, vraw, uat, wt, g3, ost, flag,
            sem_x, sem_w, sem_m, sem_o, sem_c):

    def x_copy(j):
        return pltpu.make_async_copy(x_hbm.at[pl.ds(j * CH, CH), :], xin.at[pl.ds(j * CH, CH), :], sem_x.at[j])

    def o_copy(k):
        return pltpu.make_async_copy(ost.at[pl.ds(k * 128, 128), :], out_hbm.at[pl.ds(k * 128, 128), :],
                                     sem_o.at[0])

    w_half = [[], []]
    for ri, src in enumerate((wr_hbm, wi_hbm)):
        for h in range(2):
            w_half[h].append(pltpu.make_async_copy(
                src.at[pl.ds(0, 320), pl.ds(1024 * h, 1024)],
                wraw.at[pl.ds(320 * ri, 320), pl.ds(1024 * h, 1024)], sem_w.at[3 * ri + h]))
        w_half[0].append(pltpu.make_async_copy(src.at[pl.ds(320, 1), :], wnyq.at[ri], sem_w.at[3 * ri + 2]))

    def w1_copy(i):
        if isinstance(i, int):
            rows = pl.ds(*W1_PIECES[i])
        else:
            rows = pl.ds(pl.multiple_of((i - 1) * UN, 128), UN)
        return pltpu.make_async_copy(w1_hbm.at[rows, :], w1.at[rows, pl.ds(0, S)], sem_m.at[i])

    w2_copy = pltpu.make_async_copy(w2_hbm, w2.at[:, pl.ds(0, S)], sem_m.at[NU + 1])
    fwd_copy = pltpu.make_async_copy(fwd_hbm, fwd_ref, sem_c.at[0])
    ft_copy = pltpu.make_async_copy(ft_hbm, ft_ref, sem_c.at[1])
    misc_copies = [pltpu.make_async_copy(a, b, sem_c.at[2 + i])
                   for i, (a, b) in enumerate(((inv_hbm, inv_ref), (b1_hbm, b1_ref), (b2_hbm, b2_ref)))]

    ft_copy.start()

    def start_x(j, c):
        x_copy(j).start()

        @pl.when(j == 0)
        def _():
            fwd_copy.start()
        return c
    lax.fori_loop(0, NCH, start_x, 0)

    flag[0] = 1
    yi[64:80, :] = jnp.zeros((16, S), F32)
    tb[:, 64:80, :] = jnp.zeros((16, 16, 384), BF16)
    wn[2, :, 80:128] = jnp.zeros((128 * WP, 48), U32)

    def block(fn):
        pl.when(flag[0] == 1)(fn)

    def col_pre(buf, loff, goff, slot, width, late):
        lc, gc, ac = _cols(loff, width), _cols(goff, width), pl.ds(128 * slot, width)
        r = lax.rsqrt(st[2:3, gc] + EPS)
        rc, rr, d10 = r * _C5, r * _RHO, st[1:2, gc] * r * 10.0

        def radix5(x0, x1, x2, x3, x4):
            t1, t2, t3, t4 = x1 + x4, x2 + x3, x1 - x4, x2 - x3
            u = (t1 + t2) * r
            x0 = x0 * r
            m = x0 - 0.25 * u
            n = (t1 - t2) * rc
            return x0 + u, m + n, t3 * r + t4 * rr, m - n, t3 * rr - t4 * r

        for sl in range(8):
            sm, df = [], []
            for pa, pb in _PAIRS:
                va = buf[_rows(64 * pa + 8 * sl, 8), lc]
                vb = buf[_rows(64 * pb + 8 * sl, 8), lc]
                sm.append(va + vb)
                df.append(va - vb)
            s0, s1r, s1i, s2r, s2i = radix5(*sm)
            d0, d1r, d1i, d2r, d2i = radix5(*df)
            for t, pair in enumerate(((s0 - d10, d0), (s1r, s1i), (s2r, s2i), (d1r, d1i), (d2r, d2i))):
                if t < late:
                    ab[64 * t + 8 * sl:64 * t + 8 * (sl + 1), ac] = _pk2(*pair)
                else:
                    al[64 * (t - LATE) + 8 * sl:64 * (t - LATE) + 8 * (sl + 1), gc] = _pk2(*pair)

    def dft_tile(t, cols, operand):
        o = _dot(_bf(fwd_ref[8 + 64 * t:72 + 64 * t, :]), _bf(operand))
        yr[16 + 64 * t:80 + 64 * t, cols] = o[0:64]
        yi[16 + 64 * t:80 + 64 * t, cols] = o[64:128]

    def col_dft(goff, slot, late):
        cols, ac = _cols(goff, 128), pl.ds(128 * slot, 128)
        o = _dot(_bf(fwd_ref[0:72, :]), _bf(ab[0:64, ac]))
        yr[64:80, cols] = o[0:16]
        yr[0:64, cols] = o[16:80]
        yi[0:64, cols] = o[80:144]
        for t in range(1, late):
            dft_tile(t, cols, ab[64 * t:64 * (t + 1), ac])

    def dft_late(blk):
        cols = pl.ds(128 * blk, 128)
        for t in range(LATE, 5):
            dft_tile(t, cols, al[64 * (t - LATE):64 * (t - LATE + 1), cols])

    def col_fwd(buf, loff, goff, slot, late):
        for h in range(2):
            col_pre(buf, loff + 128 * h, goff + 128 * h, slot + h, 128, late)
            col_dft(goff + 128 * h, slot + h, late)

    def rf(g):
        rows = pl.ds(g * 8, 8)
        o = _dft16([(yr[rows, 128 * a:128 * (a + 1)], yi[rows, 128 * a:128 * (a + 1)]) for a in range(16)])
        for m1 in range(16):
            tb[m1, rows, :] = jnp.concatenate([o[m1][0] + o[m1][1], o[m1][0], o[m1][1]], axis=1).astype(BF16)

    def idft(g):
        rows = pl.ds(g * 8, 8)
        o = _dft16([(tp[m1, rows, 128:256], tp[m1, rows, 0:128]) for m1 in range(16)])
        return [o[a][1] for a in range(16)], [o[a][0] for a in range(16)]

    def ri(g):
        if g == 8:
            return
        re, im = idft(g)
        if g == 0:
            ren, _ = idft(8)
            first = lax.broadcasted_iota(jnp.int32, (8, 128), 0) == 0
            im = [jnp.where(first, a, b) for a, b in zip(ren, im)]
        gg = g if g < 8 else g - 2
        for a in range(16):
            yb[pl.ds(8 * gg, 8), 128 * a:128 * (a + 1)] = _pk2(re[a], im[a])

    def gen_g(m1):
        tr, ti = ft_ref[256 + m1:257 + m1, :], ft_ref[272 + m1:273 + m1, :]
        fr, fi = ft_ref[0:128, :], ft_ref[128:256, :]
        gr = fr * tr - fi * ti
        gi = fr * ti + fi * tr
        g3[:, 384 * m1:384 * (m1 + 1)] = _pk(jnp.concatenate([gr, gi - gr, gr + gi], axis=1))

    def gmat(m1, i):
        return _bf(g3[:, 128 * (3 * m1 + i):128 * (3 * m1 + i + 1)])

    def load_wt(m1, lo, hi):
        res = []
        for c in range(2):
            ps = []
            for (r0, n, w0, h) in _PIECES:
                a, b = max(lo, r0), min(hi, r0 + n)
                if a >= b:
                    continue
                if w0 is None:
                    ps.append(_half(wt[m1, 320 + a - r0:320 + b - r0, :], c))
                else:
                    ps.append(_half(wt[m1, pl.ds(160 * c + w0 + 5 * (a - r0), b - a, stride=5), :], h))
            res.append(jnp.concatenate(ps, axis=0))
        return res

    def prep1(j):
        cols = pl.ds(j * 128, 128)
        for blk, (r0, r1) in enumerate(((0, 256), (256, 512), (512, 672))):
            v = pltpu.bitcast(wraw[r0:r1, cols], U32).T
            for t in range(8):
                wn[blk, pl.ds(WP * (8 * j + t), 16), 0:(r1 - r0) // 2] = v[16 * t:16 * (t + 1)]

    def prep2(m1):
        wt[m1, 0:128, :] = wn[0, pl.ds(m1, 128, stride=WP), :].T
        wt[m1, 128:256, :] = wn[1, pl.ds(m1, 128, stride=WP), :].T
        wt[m1, 256:336, :] = wn[2, pl.ds(m1, 128, stride=WP), :].T[0:80]

    def fwd_pass(rows, side):
        lo, hi = rows

        def fn():
            for m1 in range(16):
                _spread(side, m1)
                k1, k2, k3 = [_dot_t(tb[m1, lo:hi, 128 * i:128 * (i + 1)], gmat(m1, i)) for i in range(3)]
                tp[m1, lo:hi, 0:128] = k1 - k3
                tp[m1, lo:hi, 128:256] = k1 + k2
        return fn

    def inv_pass(rows, side, pre=()):
        lo, hi = rows

        def fn():
            for m1 in range(16):
                if m1 in pre:
                    prep2(m1)
                xr, xi = tp[m1, lo:hi, 0:128], tp[m1, lo:hi, 128:256]
                wr_, wi_ = load_wt(m1, lo, hi)
                zr = xr * wr_ - xi * wi_
                zi = xr * wi_ + xi * wr_
                q1, q2, q3 = [_dot(z.astype(BF16), gmat(m1, i)) for i, z in enumerate((zr + zi, zi, zr))]
                tp[m1, lo:hi, 0:128] = q1 + q2
                tp[m1, lo:hi, 128:256] = q1 - q3
                _spread(side, m1)
        return fn

    A, B = (0, SPLIT), (SPLIT, R)
    rf_a, rf_b = [(rf, g) for g in _groups(*A)], [(rf, g) for g in _groups(*B)]

    def spectral_head_first():
        block(_run_all(rf_a))
        for cp in w_half[0]:
            cp.wait()
        for cp in misc_copies:
            cp.start()
        w1_copy(0).start()
        wraw[640:672, :] = jnp.concatenate(
            [wnyq[0].astype(F32), wnyq[1].astype(F32), jnp.zeros((30, S), F32)], axis=0).astype(BF16)
        block(fwd_pass(A, _merge(rf_b, [(prep1, j) for j in range(8)])))
        for cp in w_half[1]:
            cp.wait()
        w1_copy(1).start()
        block(fwd_pass(B, [(prep1, j) for j in range(8, 16)] + [(prep2, m) for m in range(5)]))
        block(inv_pass(A, [], range(5, 16)))
        w1_copy(2).start()
        for cp in misc_copies:
            cp.wait()
        w1_copy(0).wait()
        b1f[...] = b1_ref[...].reshape(1, F).astype(F32)
        b2f[...] = b2_ref[...].reshape(1, S).astype(F32)

    def spectral_head_second():
        block(_run_all(_merge(rf_a, [(dft_late, b) for b in range(16)])))
        block(fwd_pass(A, rf_b))

        def rest():
            fwd_pass(B, [])()
            inv_pass(A, [])()
        block(rest)

    def inv_dot(t, cols):
        return _dot(_bf(inv_ref[64 * t:64 * (t + 1), :]), _bf(yb[64 * t:64 * (t + 1), cols]))

    def inv_early(blk):
        cols = pl.ds(128 * blk, 128)
        for t in range(EARLY):
            vraw[128 * t:128 * (t + 1), cols] = inv_dot(t, cols)

    def inv_dots(blk):
        return [None if t < EARLY else inv_dot(t, pl.ds(128 * blk, 128)) for t in range(5)]

    def where(blk):
        j = blk // 2
        return (xa, xb)[j % 2], pl.ds((j // 2) * CH + 128 * (blk % 2), 128), pl.ds(128 * blk, 128)

    def inv_post(blk, v):
        buf, lc, gc = where(blk)
        shift = st[1:2, gc] + _half(yb[0:1, gc], 0) * _DC_SCALE
        st[0:1, gc] = st[0:1, gc] + shift

        def get(t, r0):
            if t < EARLY:
                return vraw[128 * t + r0:128 * t + r0 + 8, gc]
            return v[t][r0:r0 + 8]

        def iradix5(v0, v1r, v1i, v2r, v2i):
            t1 = v1r + v2r
            m = v0 - 0.25 * t1
            n = _C5 * (v1r - v2r)
            a, b = m + n, m - n
            cc = v1i + _RHO * v2i
            dd = _RHO * v1i - v2i
            return v0 + t1, a - cc, b - dd, b + dd, a + cc

        acc = None
        for sl in range(8):
            lo, hi = 8 * sl, 64 + 8 * sl
            ys = iradix5(get(0, lo) - shift, get(1, lo), get(1, hi), get(2, lo), get(2, hi))
            yd = iradix5(get(0, hi), get(3, lo), get(3, hi), get(4, lo), get(4, hi))
            for (pa, pb), a, b in zip(_PAIRS, ys, yd):
                for p, y in ((pa, a + b), (pb, a - b)):
                    rows = _rows(64 * p + lo, 8)
                    xn = buf[rows, lc] + y
                    buf[rows, lc] = xn
                    acc = xn * xn if acc is None else acc + xn * xn
        var = jnp.sum(acc, axis=0, keepdims=True) * (1.0 / D)
        r1 = lax.rsqrt(var + EPS)
        return r1 * lax.rsqrt(var * r1 * r1 + EPS)

    def inv_norm(blk, rr):
        buf, lc, gc = where(blk)
        for sl in range(20):
            hb[16 * sl:16 * (sl + 1), gc] = _pk(buf[_rows(32 * sl, 32), lc] * rr)

    def col_inv_up():
        def up(t):
            kc = pl.ds(t * CH, CH)
            d = _dot_t(w1[F0:F, kc], _bf(hb[:, kc]))
            if t == 0:
                uat[...] = d
            else:
                uat[...] += d

        v = inv_dots(0)
        scale = {}
        done = 0
        for blk in range(17):
            if blk < 16:
                vn = inv_dots(blk + 1) if blk + 1 < 16 else None
                scale[blk] = inv_post(blk, v)
                v = vn
            if blk >= 1:
                inv_norm(blk - 1, scale[blk - 1])
            while 2 * done + 4 <= blk:
                up(done)
                done += 1
        for t in range(done, NCH):
            up(t)

    def mlp_up(l):
        def body(j, c):
            @pl.when(l == 0)
            def _():
                w1_copy(j + 1).wait()

            off = jnp.minimum(j * 384, D - 384)
            for i in range(UN // 256):
                cols = _cols(j * UN + 256 * i, 256)
                u = _dot_t(_bf(hb[:, 0:S]), w1[cols, 0:S]) + b1f[:, cols]
                gb[:, cols] = _pk(_gelu(u))
                if i == 0:
                    u = uat[:, pl.ds(pl.multiple_of(off, 128), 384)].T
                    gb[pl.ds(pl.multiple_of(off // 2, 64), 192), F0:F] = _pk(_gelu(u + b1f[:, F0:F]))
            return c
        lax.fori_loop(0, NU, body, 0)

    def mlp_down_mid():
        def step(cur, loff, goff, prev, ploff, pgoff, slot):
            lc, gc = _cols(loff, CH), _cols(goff, CH)
            acc = row0 = None
            for b in range(2):
                y = _dot(_bf(gb[160 * b:160 * (b + 1), :]), w2[:, gc])
                if b == 0:
                    row0 = cur[0:1, lc] + y[0:1]
                for sl in range(20):
                    rows = _rows(320 * b + 16 * sl, 16)
                    xn = cur[rows, lc] + (y[16 * sl:16 * (sl + 1)] - row0)
                    cur[rows, lc] = xn
                    acc = _acc_stats(acc, xn)
                if b == 0:
                    col_pre(prev, ploff, pgoff, slot, CH, LATE)
            col_dft(pgoff, slot, LATE)
            col_dft(pgoff + 128, slot + 1, LATE)
            dlt, var = _fin_stats(acc)
            st[0:1, gc] = st[0:1, gc] + row0 + b2f[:, gc]
            st[1:2, gc] = dlt
            st[2:3, gc] = var

        def body(i, c):
            ip = (i + 3) % 4
            step(xa, i * CH, 2 * i * CH, xb, ip * CH, (2 * ip + 1) * CH, 0)
            step(xb, i * CH, (2 * i + 1) * CH, xa, i * CH, 2 * i * CH, 2)
            return c
        lax.fori_loop(0, NCH // 2, body, 0)
        col_fwd(xb, 3 * CH, 7 * CH, 0, LATE)

    def mlp_down_last():
        def step(cur, loff, j):
            y = _dot(_bf(gb[...]), w2[:, _cols(j * CH, CH)])
            for h in range(2):
                gc = _cols(j * CH + 128 * h, 128)
                lc = _cols(loff + 128 * h, 128)
                xc = jnp.concatenate([cur[_rows(64 * p, 64), lc] for p in range(10)], axis=0)
                xn = xc + y[:, 128 * h:128 * (h + 1)] + (st[0:1, gc] + b2f[:, gc])
                ost[gc, :] = xn.T.astype(BF16)
                o_copy(2 * j + h).start()

        def body(i, c):
            step(xa, i * CH, 2 * i)
            step(xb, i * CH, 2 * i + 1)
            return c
        lax.fori_loop(0, NCH // 2, body, 0)

    def load_chunk(j):
        buf, lc, gc = (xa, xb)[j % 2], pl.ds((j // 2) * CH, CH), pl.ds(j * CH, CH)
        xt = xin[gc, :].astype(F32).T
        pilot = xt[0:1]
        acc = None
        for sl in range(40):
            xn = xt[16 * sl:16 * (sl + 1)] - pilot
            buf[_rows(16 * sl, 16), lc] = xn
            acc = _acc_stats(acc, xn)
        dlt, var = _fin_stats(acc)
        st[0:1, gc] = pilot
        st[1:2, gc] = dlt
        st[2:3, gc] = var

    def first_fwd(j):
        col_fwd((xa, xb)[j % 2], (j // 2) * CH, j * CH, 2 * (j % 2), 5)

    ft_copy.wait()
    for m1 in range(16):
        gen_g(m1)
    for j in range(NCH):
        x_copy(j).wait()
        if j == 1:
            fwd_copy.wait()
        if j in (5, 7):
            for cp in w_half[j // 6]:
                cp.start()
        block(_run_all(([(first_fwd, j - 1)] if j else []) + [(load_chunk, j)]))
    block(lambda: first_fwd(NCH - 1))

    def layer(l, c):
        pl.when(l == 0)(spectral_head_first)
        pl.when(l == 1)(spectral_head_second)
        block(inv_pass(B, [(ri, g) for g in _groups(*A)]))
        block(_run_all(_merge([(ri, g) for g in _groups(*B)], [(inv_early, b) for b in range(16)])))
        col_inv_up()

        @pl.when(l == 0)
        def _():
            w2_copy.start()

        mlp_up(l)

        @pl.when(l == 0)
        def _():
            w2_copy.wait()
            mlp_down_mid()

        pl.when(l == 1)(mlp_down_last)
        return c

    lax.fori_loop(0, 2, layer, 0)
    pltpu.make_async_copy(ost, out_hbm, sem_o.at[0]).wait()


@jax.jit
def pallas_interleave_layers__spectral_gfnet__mixer_token_mlp__prompt_kernel(A_x, A_w_r, A_w_i, B_x, B_w1, B_b1, B_w2, B_b2):
    del B_x
    fwd, inv, ft = _tables()
    hbm = pl.BlockSpec(memory_space=pltpu.HBM)
    out = pl.pallas_call(
        _kernel,
        out_shape=jax.ShapeDtypeStruct((S, D), BF16),
        in_specs=[hbm] * 10,
        out_specs=hbm,
        scratch_shapes=[
            pltpu.VMEM((S, D), BF16),
            pltpu.VMEM((672, S), BF16),
            pltpu.VMEM((2, 1, S), BF16),
            pltpu.VMEM((3, 128 * WP, 128), U32),
            pltpu.VMEM((F, S + PAD), BF16),
            pltpu.VMEM((F, S + PAD), BF16),
            pltpu.VMEM((F,), BF16),
            pltpu.VMEM((S,), BF16),
            pltpu.VMEM(fwd.shape, U32),
            pltpu.VMEM(inv.shape, U32),
            pltpu.VMEM(ft.shape, F32),
            pltpu.VMEM((1, F), F32),
            pltpu.VMEM((1, S), F32),
            pltpu.VMEM((8, S), F32),
            pltpu.VMEM((720, S // 2 + PAD), F32),
            pltpu.VMEM((720, S // 2 + PAD), F32),
            pltpu.VMEM((320, 512), U32),
            pltpu.VMEM((64 * (5 - LATE), S + PAD), U32),
            pltpu.VMEM((R, S), F32),
            pltpu.VMEM((R, S), F32),
            pltpu.VMEM((16, R, 384), BF16),
            pltpu.VMEM((16, R, 256), F32),
            pltpu.VMEM((D // 2, S + PAD), U32),
            pltpu.VMEM((D // 2, S + PAD), U32),
            pltpu.VMEM((D // 2, F), U32),
            pltpu.VMEM((128 * EARLY, S + PAD), F32),
            pltpu.VMEM((F - F0, D), F32),
            pltpu.VMEM((16, R, 128), U32),
            pltpu.VMEM((64, 48 * 128), U32),
            pltpu.VMEM((S, D), BF16),
            pltpu.SMEM((1,), jnp.int32),
            pltpu.SemaphoreType.DMA((NCH,)),
            pltpu.SemaphoreType.DMA((6,)),
            pltpu.SemaphoreType.DMA((NU + 2,)),
            pltpu.SemaphoreType.DMA((1,)),
            pltpu.SemaphoreType.DMA((5,)),
        ],
        compiler_params=pltpu.CompilerParams(
            vmem_limit_bytes=110 * 1024 * 1024,
            disable_bounds_checks=True,
            disable_semaphore_checks=True),
    )(A_x.reshape(S, D), A_w_r.T, A_w_i.T, B_w1.T, B_b1, B_w2, B_b2,
      jnp.asarray(fwd), jnp.asarray(inv), jnp.asarray(ft))
    return out.reshape(1, S, D)
```

```python
import numpy as np
import jax
import jax.numpy as jnp
from jax import lax
import jax.experimental.pallas as pl
import jax.experimental.pallas.tpu as pltpu

S, D, F = 2048, 640, 1728
R = 336
CH = 256
NCH = S // CH
PAD = 128
EPS = 1e-5
F32 = jnp.float32
BF16 = jnp.bfloat16
U32 = jnp.uint32

SPLIT = 176
LATE = 3
EARLY = 2
F0 = 1536
NU = 2
WP = 24
UN = F0 // NU
W1_PIECES = ((F0, F - F0),) + tuple((UN * i, UN) for i in range(NU))

_S1 = float(np.sin(2 * np.pi / 5))
_S2 = float(np.sin(4 * np.pi / 5))
_C5 = float((np.cos(2 * np.pi / 5) - np.cos(4 * np.pi / 5)) / 2)
_RHO = _S2 / _S1
_RH = float(np.sqrt(0.5))
_TILE_CLASS = ((4, -1), (2, 1), (1, 1), (3, -1))
_PAIRS = ((0, 5), (2, 7), (4, 9), (6, 1), (8, 3))

_PIECES = []
for _k in (0, 5, None) + tuple(v for c, _ in _TILE_CLASS for v in (c, 10 - c)):
    _r0 = _PIECES[-1][0] + _PIECES[-1][1] if _PIECES else 0
    _PIECES.append((_r0, 16, None, None) if _k is None else (_r0, 32, _k // 2, _k % 2))


def _pack_rows(a):
    u = np.ascontiguousarray(a, np.float32).view(np.uint32)
    u = (u + 0x7FFF + ((u >> 16) & 1)) >> 16
    return (u[0::2] | (u[1::2] << 16)).astype(np.uint32)


_DC_SCALE = float((_pack_rows(np.full((2, 1), 1.0 / (D * S))) << 16).view(np.float32)[0, 0])


def _tables():
    q = np.arange(64)
    j10 = 10 * np.arange(32)

    def cs(k):
        th = 2 * np.pi * np.outer(k, q) / D
        return np.cos(th), np.sin(th)

    sc = 2.0 / (D * S)
    z = np.zeros((32, 64))
    c0, s0 = cs(j10)
    c5, s5 = cs(5 + j10)
    nyq = np.zeros((16, 128))
    nyq[0, :64] = cs(np.array([D // 2]))[0][0]
    m0 = np.block([[c0, z], [z, c5], [-s0, z], [z, -s5]])
    i0 = m0.T * sc
    i0[:, 0] *= 0.5
    i0[:, 64] = nyq[0] * 0.5 * sc
    fwd, inv = [nyq, m0], [i0]
    for c, sgn in _TILE_CLASS:
        cA, sA = cs(c + j10)
        cB, sB = cs(10 - c + j10)
        m = np.block([[cA, sA], [cB, -sB], [-sA, cA], [-sB, -cB]])
        scale = np.concatenate([np.ones(64), sgn * _S1 * np.ones(64)])
        fwd.append(m * np.concatenate([np.ones(64), -scale[64:]])[None, :])
        inv.append(m.T * sc * scale[:, None])
    kperm = np.arange(128).reshape(2, 8, 8).transpose(1, 0, 2).reshape(-1)
    return _pack_rows(np.concatenate(fwd)[:, kperm]), _pack_rows(np.concatenate(inv)[:, kperm])


def _bfly4(a, b, c, d):
    s0r, s0i = a[0] + c[0], a[1] + c[1]
    d0r, d0i = a[0] - c[0], a[1] - c[1]
    s1r, s1i = b[0] + d[0], b[1] + d[1]
    d1r, d1i = b[0] - d[0], b[1] - d[1]
    return ((s0r + s1r, s0i + s1i), (d0r + d1i, d0i - d1r),
            (s0r - s1r, s0i - s1i), (d0r - d1i, d0i + d1r))


def _tw16(z, e):
    r, i = z
    if e == 0:
        return z
    if e == 4:
        return (i, -r)
    if e == 2:
        return ((r + i) * _RH, (i - r) * _RH)
    if e == 6:
        return ((i - r) * _RH, (r + i) * (-_RH))
    c, s = float(np.cos(2 * np.pi * e / 16)), float(np.sin(2 * np.pi * e / 16))
    return (r * c + i * s, i * c - r * s)


def _dft16(x):
    t = []
    for a0 in range(4):
        o = _bfly4(x[a0], x[4 + a0], x[8 + a0], x[12 + a0])
        t.append([_tw16(o[r0], a0 * r0) for r0 in range(4)])
    out = [None] * 16
    for r0 in range(4):
        o = _bfly4(t[0][r0], t[1][r0], t[2][r0], t[3][r0])
        for r1 in range(4):
            out[r0 + 4 * r1] = o[r1]
    return out


def _dot(a, b):
    return jnp.dot(a, b, preferred_element_type=F32)


def _dot_t(a, b):
    return lax.dot_general(a, b, (((1,), (1,)), ((), ())), preferred_element_type=F32)


def _gelu(u):
    return 0.5 * u * (1.0 + jnp.tanh(0.7978845608028654 * (u + 0.044715 * (u * u * u))))


def _cols(off, width):
    if isinstance(off, int):
        return pl.ds(off, width)
    return pl.ds(pl.multiple_of(off, 128), width)


def _bf(u):
    return pltpu.bitcast(u, BF16)


def _pk(v):
    return pltpu.bitcast(v.astype(BF16), U32)


def _pk2(lo, hi):
    return _pk(jnp.concatenate([lo, hi], axis=0))


def _half(v, h):
    return pltpu.bitcast(v << 16 if h == 0 else v & jnp.uint32(0xFFFF0000), F32)


def _fold8(v):
    out = v[0:8]
    for i in range(1, v.shape[0] // 8):
        out = out + v[8 * i:8 * (i + 1)]
    return out


def _acc_stats(acc, xn):
    a1, a2 = _fold8(xn), _fold8(xn * xn)
    return (a1, a2) if acc is None else (acc[0] + a1, acc[1] + a2)


def _fin_stats(acc):
    dlt = jnp.sum(acc[0], axis=0, keepdims=True) * (1.0 / D)
    msq = jnp.sum(acc[1], axis=0, keepdims=True) * (1.0 / D)
    return dlt, jnp.maximum(msq - dlt * dlt, 0.0)


def _rows(r0, n):
    p = r0 + 8 * (r0 // 64)
    return slice(p, p + n)


def _groups(lo, hi):
    return [g for g in range(lo // 8, hi // 8) if g != 9]


def _merge(a, b):
    keyed = ([((i + 0.5) / len(b), 0, w) for i, w in enumerate(b)]
             + [((i + 0.75) / len(a), 1, w) for i, w in enumerate(a)])
    return [w for _, _, w in sorted(keyed, key=lambda t: t[:2])]


def _run_all(work):
    def fn():
        for f, arg in work:
            f(arg)
    return fn


def _spread(work, m1):
    n = len(work)
    for fn, arg in work[(m1 * n) // 16:((m1 + 1) * n) // 16]:
        fn(arg)


def _kernel(x_hbm, wr_hbm, wi_hbm, w1_hbm, b1_hbm, w2_hbm, b2_hbm, fwd_hbm, inv_hbm,
            out_hbm,
            xin, wraw, wnyq, wn, w1, w2, b1_ref, b2_ref, fwd_ref, inv_ref, ft_ref,
            b1f, b2f, st, xa, xb, ab, al, yr, yi, tb, tp, yb, hb, gb, vraw, uat, wt, g3, ost, flag,
            sem_x, sem_w, sem_m, sem_o, sem_c):

    def x_copy(j):
        return pltpu.make_async_copy(x_hbm.at[pl.ds(j * CH, CH), :], xin.at[pl.ds(j * CH, CH), :], sem_x.at[j])

    def o_copy(k):
        return pltpu.make_async_copy(ost.at[pl.ds(k * 128, 128), :], out_hbm.at[pl.ds(k * 128, 128), :],
                                     sem_o.at[0])

    w_half = [[], []]
    for ri, src in enumerate((wr_hbm, wi_hbm)):
        for h in range(2):
            w_half[h].append(pltpu.make_async_copy(
                src.at[pl.ds(0, 320), pl.ds(1024 * h, 1024)],
                wraw.at[pl.ds(320 * ri, 320), pl.ds(1024 * h, 1024)], sem_w.at[3 * ri + h]))
        w_half[0].append(pltpu.make_async_copy(src.at[pl.ds(320, 1), :], wnyq.at[ri], sem_w.at[3 * ri + 2]))

    def w1_copy(i):
        if isinstance(i, int):
            rows = pl.ds(*W1_PIECES[i])
        else:
            rows = pl.ds(pl.multiple_of((i - 1) * UN, 128), UN)
        return pltpu.make_async_copy(w1_hbm.at[rows, :], w1.at[rows, pl.ds(0, S)], sem_m.at[i])

    w2_copy = pltpu.make_async_copy(w2_hbm, w2.at[:, pl.ds(0, S)], sem_m.at[NU + 1])
    fwd_copy = pltpu.make_async_copy(fwd_hbm, fwd_ref, sem_c.at[0])
    misc_copies = [pltpu.make_async_copy(a, b, sem_c.at[1 + i])
                   for i, (a, b) in enumerate(((inv_hbm, inv_ref), (b1_hbm, b1_ref), (b2_hbm, b2_ref)))]

    def start_x(j, c):
        x_copy(j).start()

        @pl.when(j == 0)
        def _():
            fwd_copy.start()
        return c
    lax.fori_loop(0, NCH, start_x, 0)

    flag[0] = 1

    def block(fn):
        pl.when(flag[0] == 1)(fn)

    def col_pre(buf, loff, goff, slot, width, late):
        lc, gc, ac = _cols(loff, width), _cols(goff, width), pl.ds(128 * slot, width)
        r = lax.rsqrt(st[2:3, gc] + EPS)
        rc, rr, d10 = r * _C5, r * _RHO, st[1:2, gc] * r * 10.0

        def radix5(x0, x1, x2, x3, x4):
            t1, t2, t3, t4 = x1 + x4, x2 + x3, x1 - x4, x2 - x3
            u = (t1 + t2) * r
            x0 = x0 * r
            m = x0 - 0.25 * u
            n = (t1 - t2) * rc
            return x0 + u, m + n, t3 * r + t4 * rr, m - n, t3 * rr - t4 * r

        for sl in range(8):
            sm, df = [], []
            for pa, pb in _PAIRS:
                va = buf[_rows(64 * pa + 8 * sl, 8), lc]
                vb = buf[_rows(64 * pb + 8 * sl, 8), lc]
                sm.append(va + vb)
                df.append(va - vb)
            s0, s1r, s1i, s2r, s2i = radix5(*sm)
            d0, d1r, d1i, d2r, d2i = radix5(*df)
            for t, pair in enumerate(((s0 - d10, d0), (s1r, s1i), (s2r, s2i), (d1r, d1i), (d2r, d2i))):
                if t < late:
                    ab[64 * t + 8 * sl:64 * t + 8 * (sl + 1), ac] = _pk2(*pair)
                else:
                    al[64 * (t - LATE) + 8 * sl:64 * (t - LATE) + 8 * (sl + 1), gc] = _pk2(*pair)

    def dft_tile(t, cols, operand):
        o = _dot(_bf(fwd_ref[8 + 64 * t:72 + 64 * t, :]), _bf(operand))
        yr[16 + 64 * t:80 + 64 * t, cols] = o[0:64]
        yi[16 + 64 * t:80 + 64 * t, cols] = o[64:128]

    def col_dft(goff, slot, late):
        cols, ac = _cols(goff, 128), pl.ds(128 * slot, 128)
        o = _dot(_bf(fwd_ref[0:72, :]), _bf(ab[0:64, ac]))
        yr[64:80, cols] = o[0:16]
        yr[0:64, cols] = o[16:80]
        yi[0:64, cols] = o[80:144]
        for t in range(1, late):
            dft_tile(t, cols, ab[64 * t:64 * (t + 1), ac])

    def dft_late(blk):
        cols = pl.ds(128 * blk, 128)
        for t in range(LATE, 5):
            dft_tile(t, cols, al[64 * (t - LATE):64 * (t - LATE + 1), cols])

    def col_fwd(buf, loff, goff, slot, late):
        for h in range(2):
            col_pre(buf, loff + 128 * h, goff + 128 * h, slot + h, 128, late)
            col_dft(goff + 128 * h, slot + h, late)

    def rf(g):
        rows = pl.ds(g * 8, 8)
        o = _dft16([(yr[rows, 128 * a:128 * (a + 1)], yi[rows, 128 * a:128 * (a + 1)]) for a in range(16)])
        for m1 in range(16):
            tb[m1, rows, :] = jnp.concatenate([o[m1][0] + o[m1][1], o[m1][0], o[m1][1]], axis=1).astype(BF16)

    def idft(g):
        rows = pl.ds(g * 8, 8)
        o = _dft16([(tp[m1, rows, 128:256], tp[m1, rows, 0:128]) for m1 in range(16)])
        return [o[a][1] for a in range(16)], [o[a][0] for a in range(16)]

    def ri(g):
        if g == 8:
            return
        re, im = idft(g)
        if g == 0:
            ren, _ = idft(8)
            first = lax.broadcasted_iota(jnp.int32, (8, 128), 0) == 0
            im = [jnp.where(first, a, b) for a, b in zip(ren, im)]
        gg = g if g < 8 else g - 2
        for a in range(16):
            yb[pl.ds(8 * gg, 8), 128 * a:128 * (a + 1)] = _pk2(re[a], im[a])

    def gen_g(m1):
        tr, ti = ft_ref[0, 128 + m1:129 + m1, :], ft_ref[1, 128 + m1:129 + m1, :]
        fr, fi = ft_ref[0, 0:128, :], ft_ref[1, 0:128, :]
        gr = fr * tr - fi * ti
        gi = fr * ti + fi * tr
        g3[:, 384 * m1:384 * (m1 + 1)] = _pk(jnp.concatenate([gr, gi - gr, gr + gi], axis=1))

    def gmat(m1, i):
        return _bf(g3[:, 128 * (3 * m1 + i):128 * (3 * m1 + i + 1)])

    def load_wt(m1, lo, hi):
        res = []
        for c in range(2):
            ps = []
            for (r0, n, w0, h) in _PIECES:
                a, b = max(lo, r0), min(hi, r0 + n)
                if a >= b:
                    continue
                if w0 is None:
                    ps.append(_half(wt[m1, 320 + a - r0:320 + b - r0, :], c))
                else:
                    ps.append(_half(wt[m1, pl.ds(160 * c + w0 + 5 * (a - r0), b - a, stride=5), :], h))
            res.append(jnp.concatenate(ps, axis=0))
        return res

    def prep1(j):
        cols = pl.ds(j * 128, 128)
        for blk, (r0, r1) in enumerate(((0, 256), (256, 512), (512, 672))):
            v = pltpu.bitcast(wraw[r0:r1, cols], U32).T
            if blk == 2:
                v = jnp.concatenate([v, jnp.zeros((128, 48), U32)], axis=1)
            for t in range(8):
                wn[blk, pl.ds(WP * (8 * j + t), 16), :] = v[16 * t:16 * (t + 1)]

    def prep2(m1):
        wt[m1, 0:128, :] = wn[0, pl.ds(m1, 128, stride=WP), :].T
        wt[m1, 128:256, :] = wn[1, pl.ds(m1, 128, stride=WP), :].T
        wt[m1, 256:336, :] = wn[2, pl.ds(m1, 128, stride=WP), :].T[0:80]

    def fwd_pass(rows, side):
        lo, hi = rows

        def fn():
            for m1 in range(16):
                _spread(side, m1)
                k1, k2, k3 = [_dot_t(tb[m1, lo:hi, 128 * i:128 * (i + 1)], gmat(m1, i)) for i in range(3)]
                tp[m1, lo:hi, 0:128] = k1 - k3
                tp[m1, lo:hi, 128:256] = k1 + k2
        return fn

    def inv_pass(rows, side, pre=()):
        lo, hi = rows

        def fn():
            for m1 in range(16):
                if m1 in pre:
                    prep2(m1)
                xr, xi = tp[m1, lo:hi, 0:128], tp[m1, lo:hi, 128:256]
                wr_, wi_ = load_wt(m1, lo, hi)
                zr = xr * wr_ - xi * wi_
                zi = xr * wi_ + xi * wr_
                q1, q2, q3 = [_dot(z.astype(BF16), gmat(m1, i)) for i, z in enumerate((zr + zi, zi, zr))]
                tp[m1, lo:hi, 0:128] = q1 + q2
                tp[m1, lo:hi, 128:256] = q1 - q3
                _spread(side, m1)
        return fn

    A, B = (0, SPLIT), (SPLIT, R)
    rf_a, rf_b = [(rf, g) for g in _groups(*A)], [(rf, g) for g in _groups(*B)]

    def spectral_head_first():
        block(_run_all(rf_a))
        for cp in w_half[0]:
            cp.wait()
        for cp in misc_copies:
            cp.start()
        w1_copy(0).start()
        wraw[640:672, :] = jnp.concatenate(
            [wnyq[0].astype(F32), wnyq[1].astype(F32), jnp.zeros((30, S), F32)], axis=0).astype(BF16)
        block(fwd_pass(A, _merge(rf_b, [(prep1, j) for j in range(8)])))
        for cp in w_half[1]:
            cp.wait()
        w1_copy(1).start()
        block(fwd_pass(B, [(prep1, j) for j in range(8, 16)] + [(prep2, m) for m in range(5)]))
        block(inv_pass(A, [], range(5, 16)))
        w1_copy(2).start()
        for cp in misc_copies:
            cp.wait()
        w1_copy(0).wait()
        b1f[...] = b1_ref[...].reshape(1, F).astype(F32)
        b2f[...] = b2_ref[...].reshape(1, S).astype(F32)

    def spectral_head_second():
        block(_run_all(_merge(rf_a, [(dft_late, b) for b in range(16)])))
        block(fwd_pass(A, rf_b))

        def rest():
            fwd_pass(B, [])()
            inv_pass(A, [])()
        block(rest)

    def inv_dot(t, cols):
        return _dot(_bf(inv_ref[64 * t:64 * (t + 1), :]), _bf(yb[64 * t:64 * (t + 1), cols]))

    def inv_early(blk):
        cols = pl.ds(128 * blk, 128)
        for t in range(EARLY):
            vraw[128 * t:128 * (t + 1), cols] = inv_dot(t, cols)

    def inv_dots(blk):
        return [None if t < EARLY else inv_dot(t, pl.ds(128 * blk, 128)) for t in range(5)]

    def where(blk):
        j = blk // 2
        return (xa, xb)[j % 2], pl.ds((j // 2) * CH + 128 * (blk % 2), 128), pl.ds(128 * blk, 128)

    def inv_post(blk, v):
        buf, lc, gc = where(blk)
        shift = st[1:2, gc] + _half(yb[0:1, gc], 0) * _DC_SCALE
        st[0:1, gc] = st[0:1, gc] + shift

        def get(t, r0):
            if t < EARLY:
                return vraw[128 * t + r0:128 * t + r0 + 8, gc]
            return v[t][r0:r0 + 8]

        def iradix5(v0, v1r, v1i, v2r, v2i):
            t1 = v1r + v2r
            m = v0 - 0.25 * t1
            n = _C5 * (v1r - v2r)
            a, b = m + n, m - n
            cc = v1i + _RHO * v2i
            dd = _RHO * v1i - v2i
            return v0 + t1, a - cc, b - dd, b + dd, a + cc

        acc = None
        for sl in range(8):
            lo, hi = 8 * sl, 64 + 8 * sl
            ys = iradix5(get(0, lo) - shift, get(1, lo), get(1, hi), get(2, lo), get(2, hi))
            yd = iradix5(get(0, hi), get(3, lo), get(3, hi), get(4, lo), get(4, hi))
            for (pa, pb), a, b in zip(_PAIRS, ys, yd):
                for p, y in ((pa, a + b), (pb, a - b)):
                    rows = _rows(64 * p + lo, 8)
                    xn = buf[rows, lc] + y
                    buf[rows, lc] = xn
                    acc = xn * xn if acc is None else acc + xn * xn
        var = jnp.sum(acc, axis=0, keepdims=True) * (1.0 / D)
        r1 = lax.rsqrt(var + EPS)
        return r1 * lax.rsqrt(var * r1 * r1 + EPS)

    def inv_norm(blk, rr):
        buf, lc, gc = where(blk)
        for sl in range(20):
            hb[16 * sl:16 * (sl + 1), gc] = _pk(buf[_rows(32 * sl, 32), lc] * rr)

    def col_inv_up():
        def up(t):
            kc = pl.ds(t * CH, CH)
            d = _dot_t(w1[F0:F, kc], _bf(hb[:, kc]))
            if t == 0:
                uat[...] = d
            else:
                uat[...] += d

        v = inv_dots(0)
        scale = {}
        done = 0
        for blk in range(17):
            if blk < 16:
                vn = inv_dots(blk + 1) if blk + 1 < 16 else None
                scale[blk] = inv_post(blk, v)
                v = vn
            if blk >= 1:
                inv_norm(blk - 1, scale[blk - 1])
            while 2 * done + 4 <= blk:
                up(done)
                done += 1
        for t in range(done, NCH):
            up(t)

    def mlp_up(l):
        def body(j, c):
            @pl.when(l == 0)
            def _():
                w1_copy(j + 1).wait()

            off = jnp.minimum(j * 384, D - 384)
            for i in range(UN // 256):
                cols = _cols(j * UN + 256 * i, 256)
                u = _dot_t(_bf(hb[:, 0:S]), w1[cols, 0:S]) + b1f[:, cols]
                gb[:, cols] = _pk(_gelu(u))
                if i == 0:
                    u = uat[:, pl.ds(pl.multiple_of(off, 128), 384)].T
                    gb[pl.ds(pl.multiple_of(off // 2, 64), 192), F0:F] = _pk(_gelu(u + b1f[:, F0:F]))
            return c
        lax.fori_loop(0, NU, body, 0)

    def mlp_down_mid():
        def step(cur, loff, goff, prev, ploff, pgoff, slot):
            lc, gc = _cols(loff, CH), _cols(goff, CH)
            acc = row0 = None
            for b in range(2):
                y = _dot(_bf(gb[160 * b:160 * (b + 1), :]), w2[:, gc])
                if b == 0:
                    row0 = cur[0:1, lc] + y[0:1]
                for sl in range(20):
                    rows = _rows(320 * b + 16 * sl, 16)
                    xn = cur[rows, lc] + (y[16 * sl:16 * (sl + 1)] - row0)
                    cur[rows, lc] = xn
                    acc = _acc_stats(acc, xn)
                if b == 0:
                    col_pre(prev, ploff, pgoff, slot, CH, LATE)
            col_dft(pgoff, slot, LATE)
            col_dft(pgoff + 128, slot + 1, LATE)
            dlt, var = _fin_stats(acc)
            st[0:1, gc] = st[0:1, gc] + row0 + b2f[:, gc]
            st[1:2, gc] = dlt
            st[2:3, gc] = var

        def body(i, c):
            ip = (i + 3) % 4
            step(xa, i * CH, 2 * i * CH, xb, ip * CH, (2 * ip + 1) * CH, 0)
            step(xb, i * CH, (2 * i + 1) * CH, xa, i * CH, 2 * i * CH, 2)
            return c
        lax.fori_loop(0, NCH // 2, body, 0)
        col_fwd(xb, 3 * CH, 7 * CH, 0, LATE)

    def mlp_down_last():
        def step(cur, loff, j):
            y = _dot(_bf(gb[...]), w2[:, _cols(j * CH, CH)])
            for h in range(2):
                gc = _cols(j * CH + 128 * h, 128)
                lc = _cols(loff + 128 * h, 128)
                xc = jnp.concatenate([cur[_rows(64 * p, 64), lc] for p in range(10)], axis=0)
                xn = xc + y[:, 128 * h:128 * (h + 1)] + (st[0:1, gc] + b2f[:, gc])
                ost[gc, :] = xn.T.astype(BF16)
                o_copy(2 * j + h).start()

        def body(i, c):
            step(xa, i * CH, 2 * i)
            step(xb, i * CH, 2 * i + 1)
            return c
        lax.fori_loop(0, NCH // 2, body, 0)

    def load_chunk(j):
        buf, lc, gc = (xa, xb)[j % 2], pl.ds((j // 2) * CH, CH), pl.ds(j * CH, CH)
        xt = xin[gc, :].astype(F32).T
        pilot = xt[0:1]
        acc = None
        for sl in range(40):
            xn = xt[16 * sl:16 * (sl + 1)] - pilot
            buf[_rows(16 * sl, 16), lc] = xn
            acc = _acc_stats(acc, xn)
        dlt, var = _fin_stats(acc)
        st[0:1, gc] = pilot
        st[1:2, gc] = dlt
        st[2:3, gc] = var

    def zero_pads(_):
        yi[64:80, :] = jnp.zeros((16, S), F32)
        tb[:, 64:80, :] = jnp.zeros((16, 16, 384), BF16)

    def first_fwd(j):
        col_fwd((xa, xb)[j % 2], (j // 2) * CH, j * CH, 2 * (j % 2), 5)

    row = lax.broadcasted_iota(jnp.int32, (144, 128), 0)
    lane = lax.broadcasted_iota(jnp.int32, (144, 128), 1)
    turns = jnp.where(row < 128, 16 * row * lane, (row - 128) * lane) & (S - 1)
    ang = jnp.where(turns >= S // 2, turns - S, turns).astype(F32) * (2.0 * np.pi / S)
    ft_ref[0] = jnp.cos(ang)
    ft_ref[1] = -jnp.sin(ang)
    for m1 in range(16):
        gen_g(m1)
    for j in range(NCH):
        x_copy(j).wait()
        if j == 1:
            fwd_copy.wait()
        if j in (5, 7):
            for cp in w_half[j // 6]:
                cp.start()
        block(_run_all([(first_fwd, j - 1) if j else (zero_pads, None), (load_chunk, j)]))
    block(lambda: first_fwd(NCH - 1))

    def layer(l, c):
        pl.when(l == 0)(spectral_head_first)
        pl.when(l == 1)(spectral_head_second)
        block(inv_pass(B, [(ri, g) for g in _groups(*A)]))
        block(_run_all(_merge([(ri, g) for g in _groups(*B)], [(inv_early, b) for b in range(16)])))
        col_inv_up()

        @pl.when(l == 0)
        def _():
            w2_copy.start()

        mlp_up(l)

        @pl.when(l == 0)
        def _():
            w2_copy.wait()
            mlp_down_mid()

        pl.when(l == 1)(mlp_down_last)
        return c

    lax.fori_loop(0, 2, layer, 0)
    pltpu.make_async_copy(ost, out_hbm, sem_o.at[0]).wait()


@jax.jit
def pallas_interleave_layers__spectral_gfnet__mixer_token_mlp__prompt_kernel(A_x, A_w_r, A_w_i, B_x, B_w1, B_b1, B_w2, B_b2):
    del B_x
    fwd, inv = _tables()
    hbm = pl.BlockSpec(memory_space=pltpu.HBM)
    out = pl.pallas_call(
        _kernel,
        out_shape=jax.ShapeDtypeStruct((S, D), BF16),
        in_specs=[hbm] * 9,
        out_specs=hbm,
        scratch_shapes=[
            pltpu.VMEM((S, D), BF16),
            pltpu.VMEM((672, S), BF16),
            pltpu.VMEM((2, 1, S), BF16),
            pltpu.VMEM((3, 128 * WP, 128), U32),
            pltpu.VMEM((F, S + PAD), BF16),
            pltpu.VMEM((F, S + PAD), BF16),
            pltpu.VMEM((F,), BF16),
            pltpu.VMEM((S,), BF16),
            pltpu.VMEM(fwd.shape, U32),
            pltpu.VMEM(inv.shape, U32),
            pltpu.VMEM((2, 144, 128), F32),
            pltpu.VMEM((1, F), F32),
            pltpu.VMEM((1, S), F32),
            pltpu.VMEM((8, S), F32),
            pltpu.VMEM((720, S // 2 + PAD), F32),
            pltpu.VMEM((720, S // 2 + PAD), F32),
            pltpu.VMEM((320, 512), U32),
            pltpu.VMEM((64 * (5 - LATE), S + PAD), U32),
            pltpu.VMEM((R, S), F32),
            pltpu.VMEM((R, S), F32),
            pltpu.VMEM((16, R, 384), BF16),
            pltpu.VMEM((16, R, 256), F32),
            pltpu.VMEM((D // 2, S + PAD), U32),
            pltpu.VMEM((D // 2, S + PAD), U32),
            pltpu.VMEM((D // 2, F), U32),
            pltpu.VMEM((128 * EARLY, S + PAD), F32),
            pltpu.VMEM((F - F0, D), F32),
            pltpu.VMEM((16, R, 128), U32),
            pltpu.VMEM((64, 48 * 128), U32),
            pltpu.VMEM((S, D), BF16),
            pltpu.SMEM((1,), jnp.int32),
            pltpu.SemaphoreType.DMA((NCH,)),
            pltpu.SemaphoreType.DMA((6,)),
            pltpu.SemaphoreType.DMA((NU + 2,)),
            pltpu.SemaphoreType.DMA((1,)),
            pltpu.SemaphoreType.DMA((4,)),
        ],
        compiler_params=pltpu.CompilerParams(
            vmem_limit_bytes=110 * 1024 * 1024,
            disable_bounds_checks=True,
            disable_semaphore_checks=True),
    )(A_x.reshape(S, D), A_w_r.T, A_w_i.T, B_w1.T, B_b1, B_w2, B_b2,
      jnp.asarray(fwd), jnp.asarray(inv))
    return out.reshape(1, S, D)
```

```python
import numpy as np
import jax
import jax.numpy as jnp
from jax import lax
import jax.experimental.pallas as pl
import jax.experimental.pallas.tpu as pltpu

S, D, F = 2048, 640, 1728
R = 336
CH = 256
NCH = S // CH
PAD = 128
EPS = 1e-5
F32 = jnp.float32
BF16 = jnp.bfloat16
U32 = jnp.uint32

SPLIT_F = 144
SPLIT = 176
LATE = 2
EARLY = 2
F0 = 1536
NU = 2
WP = 24
UN = F0 // NU
W1_PIECES = ((F0, F - F0),) + tuple((UN * i, UN) for i in range(NU))

_S1 = float(np.sin(2 * np.pi / 5))
_S2 = float(np.sin(4 * np.pi / 5))
_C5 = float((np.cos(2 * np.pi / 5) - np.cos(4 * np.pi / 5)) / 2)
_RHO = _S2 / _S1
_RH = float(np.sqrt(0.5))
_TILE_CLASS = ((4, -1), (2, 1), (1, 1), (3, -1))
_PAIRS = ((0, 5), (2, 7), (4, 9), (6, 1), (8, 3))

_PIECES = []
for _k in (0, 5, None) + tuple(v for c, _ in _TILE_CLASS for v in (c, 10 - c)):
    _r0 = _PIECES[-1][0] + _PIECES[-1][1] if _PIECES else 0
    _PIECES.append((_r0, 16, None, None) if _k is None else (_r0, 32, _k // 2, _k % 2))


def _pack_rows(a):
    u = np.ascontiguousarray(a, np.float32).view(np.uint32)
    u = (u + 0x7FFF + ((u >> 16) & 1)) >> 16
    return (u[0::2] | (u[1::2] << 16)).astype(np.uint32)


_DC_SCALE = float((_pack_rows(np.full((2, 1), 1.0 / (D * S))) << 16).view(np.float32)[0, 0])


def _tables():
    q = np.arange(64)
    j10 = 10 * np.arange(32)

    def cs(k):
        th = 2 * np.pi * np.outer(k, q) / D
        return np.cos(th), np.sin(th)

    sc = 2.0 / (D * S)
    z = np.zeros((32, 64))
    c0, s0 = cs(j10)
    c5, s5 = cs(5 + j10)
    nyq = np.zeros((16, 128))
    nyq[0, :64] = cs(np.array([D // 2]))[0][0]
    m0 = np.block([[c0, z], [z, c5], [-s0, z], [z, -s5]])
    i0 = m0.T * sc
    i0[:, 0] *= 0.5
    i0[:, 64] = nyq[0] * 0.5 * sc
    fwd, inv = [nyq, m0], [i0]
    for c, sgn in _TILE_CLASS:
        cA, sA = cs(c + j10)
        cB, sB = cs(10 - c + j10)
        m = np.block([[cA, sA], [cB, -sB], [-sA, cA], [-sB, -cB]])
        scale = np.concatenate([np.ones(64), sgn * _S1 * np.ones(64)])
        fwd.append(m * np.concatenate([np.ones(64), -scale[64:]])[None, :])
        inv.append(m.T * sc * scale[:, None])
    kperm = np.arange(128).reshape(2, 8, 8).transpose(1, 0, 2).reshape(-1)
    return _pack_rows(np.concatenate(fwd)[:, kperm]), _pack_rows(np.concatenate(inv)[:, kperm])


def _bfly4(a, b, c, d):
    s0r, s0i = a[0] + c[0], a[1] + c[1]
    d0r, d0i = a[0] - c[0], a[1] - c[1]
    s1r, s1i = b[0] + d[0], b[1] + d[1]
    d1r, d1i = b[0] - d[0], b[1] - d[1]
    return ((s0r + s1r, s0i + s1i), (d0r + d1i, d0i - d1r),
            (s0r - s1r, s0i - s1i), (d0r - d1i, d0i + d1r))


def _tw16(z, e):
    r, i = z
    if e == 0:
        return z
    if e == 4:
        return (i, -r)
    if e == 2:
        return ((r + i) * _RH, (i - r) * _RH)
    if e == 6:
        return ((i - r) * _RH, (r + i) * (-_RH))
    c, s = float(np.cos(2 * np.pi * e / 16)), float(np.sin(2 * np.pi * e / 16))
    return (r * c + i * s, i * c - r * s)


def _dft16(x):
    t = []
    for a0 in range(4):
        o = _bfly4(x[a0], x[4 + a0], x[8 + a0], x[12 + a0])
        t.append([_tw16(o[r0], a0 * r0) for r0 in range(4)])
    out = [None] * 16
    for r0 in range(4):
        o = _bfly4(t[0][r0], t[1][r0], t[2][r0], t[3][r0])
        for r1 in range(4):
            out[r0 + 4 * r1] = o[r1]
    return out


def _dft8(x):
    e = _bfly4(x[0], x[2], x[4], x[6])
    o = _bfly4(x[1], x[3], x[5], x[7])
    o = [_tw16(o[k], 2 * k) for k in range(4)]
    return ([(e[k][0] + o[k][0], e[k][1] + o[k][1]) for k in range(4)]
            + [(e[k][0] - o[k][0], e[k][1] - o[k][1]) for k in range(4)])


def _dot(a, b):
    return jnp.dot(a, b, preferred_element_type=F32)


def _dot_t(a, b):
    return lax.dot_general(a, b, (((1,), (1,)), ((), ())), preferred_element_type=F32)


def _gelu(u):
    return 0.5 * u * (1.0 + jnp.tanh(0.7978845608028654 * (u + 0.044715 * (u * u * u))))


def _cols(off, width):
    if isinstance(off, int):
        return pl.ds(off, width)
    return pl.ds(pl.multiple_of(off, 128), width)


def _bf(u):
    return pltpu.bitcast(u, BF16)


def _pk(v):
    return pltpu.bitcast(v.astype(BF16), U32)


def _pk2(lo, hi):
    return _pk(jnp.concatenate([lo, hi], axis=0))


def _half(v, h):
    return pltpu.bitcast(v << 16 if h == 0 else v & jnp.uint32(0xFFFF0000), F32)


def _fold8(v):
    out = v[0:8]
    for i in range(1, v.shape[0] // 8):
        out = out + v[8 * i:8 * (i + 1)]
    return out


def _acc_stats(acc, xn):
    a1, a2 = _fold8(xn), _fold8(xn * xn)
    return (a1, a2) if acc is None else (acc[0] + a1, acc[1] + a2)


def _fin_stats(acc):
    dlt = jnp.sum(acc[0], axis=0, keepdims=True) * (1.0 / D)
    msq = jnp.sum(acc[1], axis=0, keepdims=True) * (1.0 / D)
    return dlt, jnp.maximum(msq - dlt * dlt, 0.0)


def _rows(r0, n):
    p = r0 + 8 * (r0 // 64)
    return slice(p, p + n)


def _groups(lo, hi):
    return [g for g in range(lo // 8, hi // 8) if g != 9]


def _merge(a, b):
    keyed = ([((i + 0.5) / len(b), 0, w) for i, w in enumerate(b)]
             + [((i + 0.75) / len(a), 1, w) for i, w in enumerate(a)])
    return [w for _, _, w in sorted(keyed, key=lambda t: t[:2])]


def _run_all(work):
    def fn():
        for f, arg in work:
            f(arg)
    return fn


def _spread(work, m1):
    n = len(work)
    for fn, arg in work[(m1 * n) // 16:((m1 + 1) * n) // 16]:
        fn(arg)


def _kernel(x_hbm, wr_hbm, wi_hbm, w1_hbm, b1_hbm, w2_hbm, b2_hbm, fwd_hbm, inv_hbm,
            out_hbm,
            xin, wraw, wnyq, wn, w1, w2, b1_ref, b2_ref, fwd_ref, inv_ref, ft_ref,
            b1f, b2f, st, xa, xb, ab, al, yr, yi, tb, tp, yb, hb, gb, vraw, uat, wt, g3, ost, flag,
            sem_x, sem_w, sem_m, sem_o, sem_c):

    def x_copy(j):
        return pltpu.make_async_copy(x_hbm.at[pl.ds(j * CH, CH), :], xin.at[pl.ds(j * CH, CH), :], sem_x.at[j])

    def o_copy(k):
        return pltpu.make_async_copy(ost.at[pl.ds(k * 128, 128), :], out_hbm.at[pl.ds(k * 128, 128), :],
                                     sem_o.at[0])

    w_part = [[], []]
    for ri, src in enumerate((wr_hbm, wi_hbm)):
        for h, cols in enumerate((pl.ds(0, 256), pl.ds(256, S - 256))):
            w_part[h].append(pltpu.make_async_copy(
                src.at[pl.ds(0, 320), cols], wraw.at[pl.ds(320 * ri, 320), cols], sem_w.at[3 * ri + h]))
        w_part[0].append(pltpu.make_async_copy(src.at[pl.ds(320, 1), :], wnyq.at[ri], sem_w.at[3 * ri + 2]))

    def w1_copy(i):
        if isinstance(i, int):
            rows = pl.ds(*W1_PIECES[i])
        else:
            rows = pl.ds(pl.multiple_of((i - 1) * UN, 128), UN)
        return pltpu.make_async_copy(w1_hbm.at[rows, :], w1.at[rows, pl.ds(0, S)], sem_m.at[i])

    w2_copy = pltpu.make_async_copy(w2_hbm, w2.at[:, pl.ds(0, S)], sem_m.at[NU + 1])
    fwd_copy = pltpu.make_async_copy(fwd_hbm, fwd_ref, sem_c.at[0])
    misc_copies = [pltpu.make_async_copy(a, b, sem_c.at[1 + i])
                   for i, (a, b) in enumerate(((inv_hbm, inv_ref), (b1_hbm, b1_ref), (b2_hbm, b2_ref)))]

    def start_x(j, c):
        x_copy(j).start()

        @pl.when(j == 0)
        def _():
            fwd_copy.start()
        return c
    lax.fori_loop(0, NCH, start_x, 0)

    flag[0] = 1

    def block(fn):
        pl.when(flag[0] == 1)(fn)

    def col_pre(buf, loff, goff, slot, late):
        lc, gc, ac = _cols(loff, 128), _cols(goff, 128), pl.ds(128 * slot, 128)
        r = lax.rsqrt(st[2:3, gc] + EPS)
        rc, rr, d10 = r * _C5, r * _RHO, st[1:2, gc] * r * 10.0

        def radix5(x0, x1, x2, x3, x4):
            t1, t2, t3, t4 = x1 + x4, x2 + x3, x1 - x4, x2 - x3
            u = (t1 + t2) * r
            x0 = x0 * r
            m = x0 - 0.25 * u
            n = (t1 - t2) * rc
            return x0 + u, m + n, t3 * r + t4 * rr, m - n, t3 * rr - t4 * r

        for sl in range(8):
            sm, df = [], []
            for pa, pb in _PAIRS:
                va = buf[_rows(64 * pa + 8 * sl, 8), lc]
                vb = buf[_rows(64 * pb + 8 * sl, 8), lc]
                sm.append(va + vb)
                df.append(va - vb)
            s0, s1r, s1i, s2r, s2i = radix5(*sm)
            d0, d1r, d1i, d2r, d2i = radix5(*df)
            for t, pair in enumerate(((s0 - d10, d0), (s1r, s1i), (s2r, s2i), (d1r, d1i), (d2r, d2i))):
                if t < late:
                    ab[64 * t + 8 * sl:64 * t + 8 * (sl + 1), ac] = _pk2(*pair)
                else:
                    al[64 * (t - LATE) + 8 * sl:64 * (t - LATE) + 8 * (sl + 1), gc] = _pk2(*pair)

    def dft_tile(t, cols, operand):
        o = _dot(_bf(fwd_ref[8 + 64 * t:72 + 64 * t, :]), _bf(operand))
        yr[16 + 64 * t:80 + 64 * t, cols] = o[0:64]
        yi[16 + 64 * t:80 + 64 * t, cols] = o[64:128]

    def col_dft(goff, slot, late):
        cols, ac = _cols(goff, 128), pl.ds(128 * slot, 128)
        o = _dot(_bf(fwd_ref[0:72, :]), _bf(ab[0:64, ac]))
        yr[64:80, cols] = o[0:16]
        yr[0:64, cols] = o[16:80]
        yi[0:64, cols] = o[80:144]
        for t in range(1, late):
            dft_tile(t, cols, ab[64 * t:64 * (t + 1), ac])

    def dft_late(blk):
        cols = pl.ds(128 * blk, 128)
        for t in range(LATE, 5):
            dft_tile(t, cols, al[64 * (t - LATE):64 * (t - LATE + 1), cols])

    def col_fwd(buf, loff, goff, slot, late):
        for h in range(2):
            col_pre(buf, loff + 128 * h, goff + 128 * h, slot + h, late)
            col_dft(goff + 128 * h, slot + h, late)

    def rf_half(g, par):
        rows = pl.ds(16 * g, 16)
        t = []
        for a in range(8):
            lo, hi = slice(128 * a, 128 * (a + 1)), slice(128 * (a + 8), 128 * (a + 9))
            ar, ai, br, bi = yr[rows, lo], yi[rows, lo], yr[rows, hi], yi[rows, hi]
            t.append((ar + br, ai + bi) if par == 0 else _tw16((ar - br, ai - bi), a))
        for k, (re, im) in enumerate(_dft8(t)):
            m1 = 2 * k + par
            tb[8 * g:8 * (g + 1), 384 * m1:384 * (m1 + 1)] = _pk(jnp.concatenate([re + im, re, im], axis=1))

    def idft(g):
        rows = pl.ds(g * 8, 8)
        o = _dft16([(tp[m1, rows, 128:256], tp[m1, rows, 0:128]) for m1 in range(16)])
        return [o[a][1] for a in range(16)], [o[a][0] for a in range(16)]

    def ri(g):
        if g == 8:
            return
        re, im = idft(g)
        if g == 0:
            ren, _ = idft(8)
            first = lax.broadcasted_iota(jnp.int32, (8, 128), 0) == 0
            im = [jnp.where(first, a, b) for a, b in zip(ren, im)]
        gg = g if g < 8 else g - 2
        for a in range(16):
            yb[pl.ds(8 * gg, 8), 128 * a:128 * (a + 1)] = _pk2(re[a], im[a])

    def gen_g(m1):
        tr, ti = ft_ref[0, 128 + m1:129 + m1, :], ft_ref[1, 128 + m1:129 + m1, :]
        fr, fi = ft_ref[0, 0:128, :], ft_ref[1, 0:128, :]
        gr = fr * tr - fi * ti
        gi = fr * ti + fi * tr
        g3[:, 384 * m1:384 * (m1 + 1)] = _pk(jnp.concatenate([gr, gi - gr, gr + gi], axis=1))

    def gmat(m1, i):
        return _bf(g3[:, 128 * (3 * m1 + i):128 * (3 * m1 + i + 1)])

    def load_wt(m1, lo, hi):
        res = []
        for c in range(2):
            ps = []
            for (r0, n, w0, h) in _PIECES:
                a, b = max(lo, r0), min(hi, r0 + n)
                if a >= b:
                    continue
                if w0 is None:
                    ps.append(_half(wt[m1, 320 + a - r0:320 + b - r0, :], c))
                else:
                    ps.append(_half(wt[m1, pl.ds(160 * c + w0 + 5 * (a - r0), b - a, stride=5), :], h))
            res.append(jnp.concatenate(ps, axis=0))
        return res

    def prep1(j):
        cols = pl.ds(j * 128, 128)
        for blk, (r0, r1) in enumerate(((0, 256), (256, 512), (512, 672))):
            v = pltpu.bitcast(wraw[r0:r1, cols], U32).T
            if blk == 2:
                v = jnp.concatenate([v, jnp.zeros((128, 48), U32)], axis=1)
            for t in range(8):
                wn[blk, pl.ds(WP * (8 * j + t), 16), :] = v[16 * t:16 * (t + 1)]

    def prep2(m1):
        wt[m1, 0:128, :] = wn[0, pl.ds(m1, 128, stride=WP), :].T
        wt[m1, 128:256, :] = wn[1, pl.ds(m1, 128, stride=WP), :].T
        wt[m1, 256:336, :] = wn[2, pl.ds(m1, 128, stride=WP), :].T[0:80]

    def fwd_pass(rows, side):
        lo, hi = rows

        def fn():
            for m1 in range(16):
                _spread(side, m1)
                ks = [_dot_t(_bf(tb[lo // 2:hi // 2, 128 * (3 * m1 + i):128 * (3 * m1 + i + 1)]), gmat(m1, i))
                      for i in range(3)]
                if lo == 0:
                    for i in range(3):
                        tp[m1, lo:hi, 128 * i:128 * (i + 1)] = ks[i]
                else:
                    tp[m1, lo:hi, 0:128] = ks[0] - ks[2]
                    tp[m1, lo:hi, 128:256] = ks[0] + ks[1]
        return fn

    def inv_pass(rows, side, pre=()):
        lo, hi = rows

        def fn():
            for m1 in range(16):
                if m1 in pre:
                    prep2(m1)
                xr, xi = tp[m1, lo:hi, 0:128], tp[m1, lo:hi, 128:256]
                if lo == 0:
                    k = SPLIT_F
                    xr, xi = xr[0:k] - tp[m1, 0:k, 256:384], xr[0:k] + xi[0:k]
                    if k < hi:
                        xr = jnp.concatenate([xr, tp[m1, k:hi, 0:128]], axis=0)
                        xi = jnp.concatenate([xi, tp[m1, k:hi, 128:256]], axis=0)
                wr_, wi_ = load_wt(m1, lo, hi)
                zr = xr * wr_ - xi * wi_
                zi = xr * wi_ + xi * wr_
                q1, q2, q3 = [_dot(z.astype(BF16), gmat(m1, i)) for i, z in enumerate((zr + zi, zi, zr))]
                tp[m1, lo:hi, 0:128] = q1 + q2
                tp[m1, lo:hi, 128:256] = q1 - q3
                _spread(side, m1)
        return fn

    def rf_pair(arg):
        rf_half(arg[0], 0)
        rf_half(arg[1], 1)

    na, nb = SPLIT_F // 16, (R - SPLIT_F) // 16
    rf_a = [(lambda a: rf_half(*a), (g, par)) for par in range(2) for g in range(na)]
    rf_b = [(rf_pair, (na + i, na + (i + nb // 2) % nb)) for i in range(nb)]
    AF, BF = (0, SPLIT_F), (SPLIT_F, R)
    A, B = (0, SPLIT), (SPLIT, R)

    def spectral_head_first():
        block(_run_all(rf_a))
        for cp in w_part[0]:
            cp.wait()
        wraw[640:672, :] = jnp.concatenate(
            [wnyq[0].astype(F32), wnyq[1].astype(F32), jnp.zeros((30, S), F32)], axis=0).astype(BF16)
        block(fwd_pass(AF, _merge(rf_b, [(prep1, j) for j in range(2)])))
        for cp in w_part[1]:
            cp.wait()
        for cp in misc_copies:
            cp.start()
        w1_copy(0).start()
        block(fwd_pass(BF, [(prep1, j) for j in range(2, 16)] + [(prep2, m) for m in range(4)]))
        w1_copy(1).start()
        block(inv_pass(A, [], range(4, 16)))
        w1_copy(2).start()
        for cp in misc_copies:
            cp.wait()
        w1_copy(0).wait()
        b1f[...] = b1_ref[...].reshape(1, F).astype(F32)
        b2f[...] = b2_ref[...].reshape(1, S).astype(F32)

    def spectral_head_second():
        block(_run_all(_merge([(dft_late, b) for b in range(16)], rf_a)))
        block(fwd_pass(AF, rf_b))

        def rest():
            fwd_pass(BF, [])()
            inv_pass(A, [])()
        block(rest)

    def inv_dot(t, cols):
        return _dot(_bf(inv_ref[64 * t:64 * (t + 1), :]), _bf(yb[64 * t:64 * (t + 1), cols]))

    def inv_early(blk):
        cols = pl.ds(128 * blk, 128)
        for t in range(EARLY):
            vraw[128 * t:128 * (t + 1), cols] = inv_dot(t, cols)

    def inv_dots(blk):
        return [None if t < EARLY else inv_dot(t, pl.ds(128 * blk, 128)) for t in range(5)]

    def where(blk):
        j = blk // 2
        return (xa, xb)[j % 2], pl.ds((j // 2) * CH + 128 * (blk % 2), 128), pl.ds(128 * blk, 128)

    def inv_post(blk, v):
        buf, lc, gc = where(blk)
        shift = st[1:2, gc] + _half(yb[0:1, gc], 0) * _DC_SCALE
        st[0:1, gc] = st[0:1, gc] + shift

        def get(t, r0):
            if t < EARLY:
                return vraw[128 * t + r0:128 * t + r0 + 8, gc]
            return v[t][r0:r0 + 8]

        def iradix5(v0, v1r, v1i, v2r, v2i):
            t1 = v1r + v2r
            m = v0 - 0.25 * t1
            n = _C5 * (v1r - v2r)
            a, b = m + n, m - n
            cc = v1i + _RHO * v2i
            dd = _RHO * v1i - v2i
            return v0 + t1, a - cc, b - dd, b + dd, a + cc

        acc = None
        for sl in range(8):
            lo, hi = 8 * sl, 64 + 8 * sl
            ys = iradix5(get(0, lo) - shift, get(1, lo), get(1, hi), get(2, lo), get(2, hi))
            yd = iradix5(get(0, hi), get(3, lo), get(3, hi), get(4, lo), get(4, hi))
            for (pa, pb), a, b in zip(_PAIRS, ys, yd):
                for p, y in ((pa, a + b), (pb, a - b)):
                    rows = _rows(64 * p + lo, 8)
                    xn = buf[rows, lc] + y
                    buf[rows, lc] = xn
                    acc = xn * xn if acc is None else acc + xn * xn
        var = jnp.sum(acc, axis=0, keepdims=True) * (1.0 / D)
        r1 = lax.rsqrt(var + EPS)
        return r1 * lax.rsqrt(var * r1 * r1 + EPS)

    def inv_norm(blk, rr):
        buf, lc, gc = where(blk)
        for sl in range(20):
            hb[16 * sl:16 * (sl + 1), gc] = _pk(buf[_rows(32 * sl, 32), lc] * rr)

    def col_inv_up():
        def up(t):
            kc = pl.ds(t * CH, CH)
            d = _dot_t(w1[F0:F, kc], _bf(hb[:, kc]))
            if t == 0:
                uat[...] = d
            else:
                uat[...] += d

        v = inv_dots(0)
        scale = {}
        done = 0
        for blk in range(17):
            if blk < 16:
                vn = inv_dots(blk + 1) if blk + 1 < 16 else None
                scale[blk] = inv_post(blk, v)
                v = vn
            if blk >= 1:
                inv_norm(blk - 1, scale[blk - 1])
            while 2 * done + 4 <= blk:
                up(done)
                done += 1
        for t in range(done, NCH):
            up(t)

    def mlp_up(l):
        def body(j, c):
            @pl.when(l == 0)
            def _():
                w1_copy(j + 1).wait()

            off = jnp.minimum(j * 384, D - 384)
            for i in range(UN // 256):
                cols = _cols(j * UN + 256 * i, 256)
                u = _dot_t(_bf(hb[:, 0:S]), w1[cols, 0:S]) + b1f[:, cols]
                gb[:, cols] = _pk(_gelu(u))
                if i == 0:
                    u = uat[:, pl.ds(pl.multiple_of(off, 128), 384)].T
                    gb[pl.ds(pl.multiple_of(off // 2, 64), 192), F0:F] = _pk(_gelu(u + b1f[:, F0:F]))
            return c
        lax.fori_loop(0, NU, body, 0)

    def mlp_down_mid():
        def unit(cur, loff, goff):
            lc, gc = _cols(loff, 128), _cols(goff, 128)
            y = _dot(_bf(gb[...]), w2[:, gc])
            row0 = cur[0:1, lc] + y[0:1]
            acc = None
            for sl in range(20):
                rows = _rows(32 * sl, 32)
                xn = cur[rows, lc] + (y[32 * sl:32 * (sl + 1)] - row0)
                cur[rows, lc] = xn
                acc = _acc_stats(acc, xn)
            dlt, var = _fin_stats(acc)
            st[0:1, gc] = st[0:1, gc] + row0 + b2f[:, gc]
            st[1:2, gc] = dlt
            st[2:3, gc] = var

        def pos(i, k):
            return (xa, xb)[k // 2], i * CH + 128 * (k % 2), 2 * i * CH + 128 * k

        def body(i, c):
            ip = (i + 3) % 4
            prev = [pos(ip, 2), pos(ip, 3), pos(i, 0), pos(i, 1)]
            for k in range(4):
                col_pre(*prev[k], k, LATE)
                unit(*pos(i, k))
                if k:
                    col_dft(prev[k - 1][2], k - 1, LATE)
            col_dft(prev[3][2], 3, LATE)
            return c
        lax.fori_loop(0, NCH // 2, body, 0)
        col_fwd(xb, 3 * CH, 7 * CH, 0, LATE)

    def mlp_down_last():
        def step(cur, loff, j):
            for h in range(2):
                gc = _cols(j * CH + 128 * h, 128)
                y = _dot(_bf(gb[...]), w2[:, gc])
                lc = _cols(loff + 128 * h, 128)
                xc = jnp.concatenate([cur[_rows(64 * p, 64), lc] for p in range(10)], axis=0)
                xn = xc + y + (st[0:1, gc] + b2f[:, gc])
                ost[gc, :] = xn.T.astype(BF16)
                o_copy(2 * j + h).start()

        def body(i, c):
            step(xa, i * CH, 2 * i)
            step(xb, i * CH, 2 * i + 1)
            return c
        lax.fori_loop(0, NCH // 2, body, 0)

    def load_chunk(j):
        buf, lc, gc = (xa, xb)[j % 2], pl.ds((j // 2) * CH, CH), pl.ds(j * CH, CH)
        xt = xin[gc, :].astype(F32).T
        pilot = xt[0:1]
        acc = None
        for sl in range(40):
            xn = xt[16 * sl:16 * (sl + 1)] - pilot
            buf[_rows(16 * sl, 16), lc] = xn
            acc = _acc_stats(acc, xn)
        dlt, var = _fin_stats(acc)
        st[0:1, gc] = pilot
        st[1:2, gc] = dlt
        st[2:3, gc] = var

    def zero_pads(_):
        yi[64:80, :] = jnp.zeros((16, S), F32)

    def first_fwd(j):
        col_fwd((xa, xb)[j % 2], (j // 2) * CH, j * CH, 2 * (j % 2), 5)

    row = lax.broadcasted_iota(jnp.int32, (144, 128), 0)
    lane = lax.broadcasted_iota(jnp.int32, (144, 128), 1)
    turns = jnp.where(row < 128, 16 * row * lane, (row - 128) * lane) & (S - 1)
    ang = jnp.where(turns >= S // 2, turns - S, turns).astype(F32) * (2.0 * np.pi / S)
    ft_ref[0] = jnp.cos(ang)
    ft_ref[1] = -jnp.sin(ang)
    for m1 in range(16):
        gen_g(m1)
    for j in range(NCH):
        x_copy(j).wait()
        if j == 1:
            fwd_copy.wait()
        if j in (5, 6):
            for cp in w_part[j - 5]:
                cp.start()
        block(_run_all([(first_fwd, j - 1) if j else (zero_pads, None), (load_chunk, j)]))
    block(lambda: first_fwd(NCH - 1))

    def layer(l, c):
        pl.when(l == 0)(spectral_head_first)
        pl.when(l == 1)(spectral_head_second)
        block(inv_pass(B, [(ri, g) for g in _groups(*A)]))
        block(_run_all(_merge([(ri, g) for g in _groups(*B)], [(inv_early, b) for b in range(16)])))
        col_inv_up()

        @pl.when(l == 0)
        def _():
            w2_copy.start()

        mlp_up(l)

        @pl.when(l == 0)
        def _():
            w2_copy.wait()
            mlp_down_mid()

        pl.when(l == 1)(mlp_down_last)
        return c

    lax.fori_loop(0, 2, layer, 0)
    pltpu.make_async_copy(ost, out_hbm, sem_o.at[0]).wait()


@jax.jit
def pallas_interleave_layers__spectral_gfnet__mixer_token_mlp__prompt_kernel(A_x, A_w_r, A_w_i, B_x, B_w1, B_b1, B_w2, B_b2):
    del B_x
    fwd, inv = _tables()
    hbm = pl.BlockSpec(memory_space=pltpu.HBM)
    out = pl.pallas_call(
        _kernel,
        out_shape=jax.ShapeDtypeStruct((S, D), BF16),
        in_specs=[hbm] * 9,
        out_specs=hbm,
        scratch_shapes=[
            pltpu.VMEM((S, D), BF16),
            pltpu.VMEM((672, S), BF16),
            pltpu.VMEM((2, 1, S), BF16),
            pltpu.VMEM((3, 128 * WP, 128), U32),
            pltpu.VMEM((F, S + PAD), BF16),
            pltpu.VMEM((F, S + PAD), BF16),
            pltpu.VMEM((F,), BF16),
            pltpu.VMEM((S,), BF16),
            pltpu.VMEM(fwd.shape, U32),
            pltpu.VMEM(inv.shape, U32),
            pltpu.VMEM((2, 144, 128), F32),
            pltpu.VMEM((1, F), F32),
            pltpu.VMEM((1, S), F32),
            pltpu.VMEM((8, S), F32),
            pltpu.VMEM((720, S // 2 + PAD), F32),
            pltpu.VMEM((720, S // 2 + PAD), F32),
            pltpu.VMEM((320, 512), U32),
            pltpu.VMEM((64 * (5 - LATE), S + PAD), U32),
            pltpu.VMEM((R, S), F32),
            pltpu.VMEM((R, S), F32),
            pltpu.VMEM((R // 2, 48 * 128 + PAD), U32),
            pltpu.VMEM((16, R, 384), F32),
            pltpu.VMEM((D // 2, S + PAD), U32),
            pltpu.VMEM((D // 2, S + PAD), U32),
            pltpu.VMEM((D // 2, F), U32),
            pltpu.VMEM((128 * EARLY, S + PAD), F32),
            pltpu.VMEM((F - F0, D), F32),
            pltpu.VMEM((16, R, 128), U32),
            pltpu.VMEM((64, 48 * 128), U32),
            pltpu.VMEM((S, D), BF16),
            pltpu.SMEM((1,), jnp.int32),
            pltpu.SemaphoreType.DMA((NCH,)),
            pltpu.SemaphoreType.DMA((6,)),
            pltpu.SemaphoreType.DMA((NU + 2,)),
            pltpu.SemaphoreType.DMA((1,)),
            pltpu.SemaphoreType.DMA((4,)),
        ],
        compiler_params=pltpu.CompilerParams(
            vmem_limit_bytes=110 * 1024 * 1024,
            disable_bounds_checks=True,
            disable_semaphore_checks=True),
    )(A_x.reshape(S, D), A_w_r.T, A_w_i.T, B_w1.T, B_b1, B_w2, B_b2,
      jnp.asarray(fwd), jnp.asarray(inv))
    return out.reshape(1, S, D)
```
